```python
import jax
import jax.numpy as jnp

def _softmax(x, axis=-1):
    return jax.nn.softmax(x, axis=axis)

def _gelu(x):
    return jax.nn.gelu(x, approximate=True)

def _silu(x):
    return jax.nn.silu(x)

def _sigmoid(x):
    return jax.nn.sigmoid(x)

def _layernorm(x, axis=-1, eps=1e-05):
    m = jnp.mean(x, axis=axis, keepdims=True)
    v = jnp.var(x, axis=axis, keepdims=True)
    return (x - m) / jnp.sqrt(v + eps)

def _scatter_add(tgt, idx, src, axis=0):
    return tgt.at[idx].add(src)

def _segment_sum(src, seg, n):
    return jax.ops.segment_sum(src, seg, n)

class _Rng:

    def __init__(self, key):
        self._k = key

    def _next(self):
        self._k, sub = jax.random.split(self._k)
        return sub

    def normal(self, shape):
        return jax.random.normal(self._next(), shape, dtype=jnp.bfloat16)

    def randint(self, lo, hi, shape):
        return jax.random.randint(self._next(), shape, lo, hi, dtype=jnp.int32)

    def uniform(self, shape, lo=0.0, hi=1.0):
        return jax.random.uniform(self._next(), shape, jnp.bfloat16, lo, hi)

    def permutation(self, n):
        return jax.random.permutation(self._next(), n)
kernel_name = 'interleave_layers__memory_aug_recurrent_mem_tr__linear_kernel_hedgehog__prompt'

def setup_inputs():
    _rng = _Rng(jax.random.key(int.from_bytes(__import__("os").urandom(4), "little")))
    _w = lambda a: (lambda t: t.astype(jnp.bfloat16) if jnp.issubdtype(t.dtype, jnp.floating) else t)(jnp.asarray(a))

    def _A_setup():
        B, S, Dm = (1, 2048, 640)
        H, Dh = (32, 192)
        M, seg = (8, 32)
        seg = min(seg, S)
        S = S // seg * seg
        return {'x': _w((lambda *s: _rng.normal(s) * 0.05)(B, S, Dm)), 'mem0': _w((lambda *s: _rng.normal(s) * 0.05)(B, M, Dm)), 'Wq': _w((lambda *s: _rng.normal(s) * 0.05)(Dm, H, Dh) * Dm ** (-0.5)), 'Wk': _w((lambda *s: _rng.normal(s) * 0.05)(Dm, H, Dh) * Dm ** (-0.5)), 'Wv': _w((lambda *s: _rng.normal(s) * 0.05)(Dm, H, Dh) * Dm ** (-0.5)), 'Wo': _w((lambda *s: _rng.normal(s) * 0.05)(H, Dh, Dm) * (H * Dh) ** (-0.5)), 'seg_len': seg}
    _A_in = _A_setup()

    def _B_setup():
        B, S, D, H = (1, 2048, 640, 32)
        Dh = D // H
        return {'x': _w((lambda *s: _rng.normal(s) * 0.05)(B, S, D)), 'wqkv': _w((lambda *s: _rng.normal(s) * 0.05)(D, 3 * D)), 'w_phi': _w((lambda *s: _rng.normal(s) * 0.05)(H, Dh, Dh) * Dh ** (-0.5)), 'wo': _w((lambda *s: _rng.normal(s) * 0.05)(D, D))}
    _B_in = _B_setup()
    return {'A_x': _A_in['x'], 'A_mem0': _A_in['mem0'], 'A_Wq': _A_in['Wq'], 'A_Wk': _A_in['Wk'], 'A_Wv': _A_in['Wv'], 'A_Wo': _A_in['Wo'], 'A_seg_len': _A_in['seg_len'], 'B_x': _B_in['x'], 'B_wqkv': _B_in['wqkv'], 'B_w_phi': _B_in['w_phi'], 'B_wo': _B_in['wo']}

def reference(A_x, A_mem0, A_Wq, A_Wk, A_Wv, A_Wo, A_seg_len, B_x, B_wqkv, B_w_phi, B_wo):

    def _A_ref(x, mem0, Wq, Wk, Wv, Wo, seg_len):
        B, S, Dm = x.shape
        H, Dh = (Wq.shape[1], Wq.shape[2])
        M = mem0.shape[1]
        scale = Dh ** (-0.5)
        n_seg = S // seg_len
        L = M + seg_len
        idx = jnp.arange(L)
        mask = (idx[:, None] < M) | (idx[:, None] >= idx[None, :])
        mem = mem0
        outs = []
        for s in range(n_seg):
            xs = x[:, s * seg_len:(s + 1) * seg_len, :].copy()
            h = jnp.concatenate([mem, xs], axis=1)
            q = jnp.einsum('btd,dhe->bhte', h, Wq)
            k = jnp.einsum('btd,dhe->bhte', h, Wk)
            v = jnp.einsum('btd,dhe->bhte', h, Wv)
            scores = jnp.einsum('bhqe,bhke->bhqk', q, k) * scale
            scores = jnp.where(mask[None, None], scores, -1000000000.0)
            p = _softmax(scores, axis=-1)
            o = jnp.einsum('bhqk,bhke->bhqe', p, v)
            o = jnp.einsum('bhte,hed->btd', o, Wo)
            mem = o[:, :M, :].copy()
            outs.append(o[:, M:, :])
        return jnp.concatenate(outs, axis=1)

    def _B_ref(x, wqkv, w_phi, wo):
        B, S, D = x.shape
        H = 32
        Dh = D // H
        qkv = (lambda x, *d: x.transpose(*d))((x @ wqkv).reshape(B, S, 3, H, Dh), 2, 0, 3, 1, 4)
        q, k, v = (qkv[0], qkv[1], qkv[2])
        pq = jnp.einsum('bhsd,hdf->bhsf', q, w_phi)
        pk = jnp.einsum('bhsd,hdf->bhsf', k, w_phi)
        phi_q = jnp.concatenate([_softmax(pq, axis=-1), _softmax(-pq, axis=-1)], axis=-1)
        phi_k = jnp.concatenate([_softmax(pk, axis=-1), _softmax(-pk, axis=-1)], axis=-1)
        kv = jnp.einsum('bhsf,bhsd->bhfd', phi_k, v)
        z = jnp.einsum('bhsf->bhf', phi_k)
        num = jnp.einsum('bhqf,bhfd->bhqd', phi_q, kv)
        den = jnp.einsum('bhqf,bhf->bhq', phi_q, z)[..., None] + 1e-06
        o = num / den
        return (lambda x, *d: x.transpose(*d))(o, 0, 2, 1, 3).reshape(B, S, D) @ wo
    x = A_x
    x = x + _A_ref(_layernorm(x, axis=-1), A_mem0, A_Wq, A_Wk, A_Wv, A_Wo, A_seg_len)
    x = x + _B_ref(_layernorm(x, axis=-1), B_wqkv, B_w_phi, B_wo)
    x = x + _A_ref(_layernorm(x, axis=-1), A_mem0, A_Wq, A_Wk, A_Wv, A_Wo, A_seg_len)
    x = x + _B_ref(_layernorm(x, axis=-1), B_wqkv, B_w_phi, B_wo)
    return x
```

```python
import functools

import jax
import jax.numpy as jnp
from jax import lax
import jax.experimental.pallas as pl
import jax.experimental.pallas.tpu as pltpu

F32 = jnp.float32
BF16 = jnp.bfloat16
LANES = 128
SUB = 8


def _dot(a, b):
    return lax.dot_general(a, b, (((1,), (0,)), ((), ())), preferred_element_type=F32)


def _dot_nt(a, b):
    return lax.dot_general(a, b, (((1,), (1,)), ((), ())), preferred_element_type=F32)


def _layernorm(x):
    inv_n = 1.0 / x.shape[-1]
    c = x - jnp.sum(x, axis=-1, keepdims=True) * inv_n
    var = jnp.sum(c * c, axis=-1, keepdims=True) * inv_n
    return c * lax.rsqrt(var + 1e-5)


def _iota(shape, dim):
    return lax.broadcasted_iota(jnp.int32, shape, dim)


def _div20(n):
    return (n * 3277) >> 16


def _make_kernel(S, D, H, DH, M, SEG, HB, *, HG, TB, NBUF):
    L = M + SEG
    G = H // 2
    PW = 2 * DH
    NSEG = S // SEG
    DB = D // HB
    NG = HB // HG
    GR = DB * HG
    LOG_HG = HG.bit_length() - 1
    NCH = S // TB
    scale = DH ** -0.5
    assert PW == 3 * LANES and 2 * L <= LANES and DB == 20 and D < 1024
    assert L % SUB == 0 and M % SUB == 0 and GR % SUB == 0 and S % TB == 0

    def kernel(x_hbm, mem_ref, wq_hbm, wk_hbm, wv_hbm, wo_hbm, bw_hbm, phi_ref, bwo_hbm,
               out_hbm,
               w_ref, wo_ref, stage_ref, xb_ref, x_ref, xn_ref, h_ref, o_ref,
               bw_ref, bwo_in_ref, bt_ref, bwo_ref, kv_ref, ot_ref,
               stage_sem, misc_sem, out_sem):

        srcs = (wq_hbm, wk_hbm, wv_hbm)

        def stage_copy(g, j):
            slot = g % NBUF
            return pltpu.make_async_copy(
                srcs[j].at[pl.ds(pl.multiple_of(g * PW, PW), PW), :],
                stage_ref.at[slot, j], stage_sem.at[slot, j])

        x_copy = pltpu.make_async_copy(x_hbm, xb_ref, misc_sem.at[0])
        wo_copy = pltpu.make_async_copy(wo_hbm, wo_ref, misc_sem.at[1])
        bw_copy = pltpu.make_async_copy(bw_hbm, bw_ref, misc_sem.at[2])
        bwo_copy = pltpu.make_async_copy(bwo_hbm, bwo_in_ref, misc_sem.at[3])

        x_copy.start()
        bw_copy.start()
        bwo_copy.start()
        for g in range(NBUF):
            for j in range(3):
                stage_copy(g, j).start()

        x_copy.wait()

        def ln_body(c, carry):
            rows = pl.ds(pl.multiple_of(c * TB, TB), TB)
            x = xb_ref[rows, :].astype(F32)
            x_ref[rows, :] = x
            xn_ref[rows, :] = _layernorm(x)
            return carry

        lax.fori_loop(0, NCH, ln_body, 0)

        n = _iota((D, D), 0)
        c = _iota((D, D), 1)
        nf = n >> LOG_HG
        grp = _div20(nf)
        feat = nf - DB * grp
        head = (grp << LOG_HG) + (n & (HG - 1))
        perm = jnp.where(c == head * DB + feat, 1.0, 0.0).astype(BF16)
        eh = _iota((HB, D), 0) * DB
        ec = _iota((HB, D), 1)
        phi_flat = None
        for d in range(DB):
            t = _dot(phi_ref[d], jnp.where(ec == eh + d, 1.0, 0.0).astype(BF16))
            phi_flat = t if phi_flat is None else phi_flat + t
        nf1 = _iota((D, DB), 0) >> LOG_HG
        sel = jnp.where(nf1 - DB * _div20(nf1) == _iota((D, DB), 1), 1.0, 0.0)
        phi_t = jnp.where(_div20(c) == head,
                          _dot(sel.astype(BF16), phi_flat.astype(BF16)), 0.0).astype(BF16)
        bw_copy.wait()
        bt_ref[0] = _dot_nt(phi_t, bw_ref[:, 0:D]).astype(BF16)
        bt_ref[1] = _dot_nt(phi_t, bw_ref[:, D:2 * D]).astype(BF16)
        bt_ref[2] = _dot_nt(perm, bw_ref[:, 2 * D:3 * D]).astype(BF16)
        bwo_copy.wait()
        bwo_ref[...] = _dot(perm, bwo_in_ref[...]).astype(BF16)

        def tr_body(g, carry):
            for j in range(3):
                stage_copy(g, j).wait()
            for j in range(3):
                w_ref[g, :, j * PW:(j + 1) * PW] = stage_ref[g % NBUF, j].T

            @pl.when(g + NBUF < G)
            def _():
                for j in range(3):
                    stage_copy(g + NBUF, j).start()

            @pl.when(g + NBUF == G)
            def _():
                wo_copy.start()

            return carry

        lax.fori_loop(0, G, tr_body, 0)
        wo_copy.wait()

        def layer_a():
            row = _iota((L, 2 * L), 0)
            col = _iota((L, 2 * L), 1)
            first = col < L
            visible = (row < M) | (row >= jnp.where(first, col, col - L))
            low = _iota((L, LANES), 1) < DH - LANES
            zero = jnp.zeros((L, LANES), F32)

            def block_diag(t):
                t0, t1, t2 = t[:, :LANES], t[:, LANES:2 * LANES], t[:, 2 * LANES:]
                top = jnp.concatenate([t0, jnp.where(low, t1, 0.0), zero], axis=1)
                bot = jnp.concatenate([zero, jnp.where(low, 0.0, t1), t2], axis=1)
                return jnp.concatenate([top, bot], axis=0).astype(BF16)

            h_ref[0:M, :] = mem_ref[...].astype(F32)

            def step(s, carry):
                rows = pl.ds(pl.multiple_of(s * SEG, SEG), SEG)
                h_ref[M:L, :] = xn_ref[rows, :]
                st = {}
                acc = [None]

                def project(g):
                    qkv = _dot(h_ref[...], w_ref[g])
                    st[g] = [qkv[:, :PW], block_diag(qkv[:, PW:2 * PW]),
                             block_diag(qkv[:, 2 * PW:])]

                def attend(g):
                    sc = jnp.where(visible, _dot_nt(st[g][0], st[g][1]) * scale, -1e9)
                    m0 = jnp.max(jnp.where(first, sc, -jnp.inf), axis=1, keepdims=True)
                    m1 = jnp.max(jnp.where(first, -jnp.inf, sc), axis=1, keepdims=True)
                    e = jnp.exp(sc - jnp.where(first, m0, m1))
                    s0 = jnp.sum(jnp.where(first, e, 0.0), axis=1, keepdims=True)
                    s1 = jnp.sum(jnp.where(first, 0.0, e), axis=1, keepdims=True)
                    st[g][0] = e / jnp.where(first, s0, s1)

                def mix(g):
                    o_ref[:, g * PW:(g + 1) * PW] = _dot(st[g][0], st[g][2])

                def out_proj(g):
                    r = _dot(o_ref[:, g * PW:(g + 1) * PW], wo_ref[g * PW:(g + 1) * PW, :])
                    acc[0] = r if acc[0] is None else acc[0] + r

                done = 0
                for i in range(G + 2):
                    if i < G:
                        project(i)
                    else:
                        for _ in range(3):
                            out_proj(done)
                            done += 1
                    if 0 <= i - 1 < G:
                        attend(i - 1)
                    if 0 <= i - 2 < G:
                        mix(i - 2)
                for g in range(done, G):
                    out_proj(g)
                h_ref[0:M, :] = acc[0][0:M]
                x_ref[rows, :] = x_ref[rows, :] + acc[0][M:L]
                return carry

            lax.fori_loop(0, NSEG, step, 0)

        def over_features(op, p):
            r = p[0:SUB]
            for i in range(1, GR // SUB):
                r = op(r, p[i * SUB:(i + 1) * SUB])
            shift = SUB // 2
            while shift >= HG:
                r = op(r, pltpu.roll(r, shift, 0))
                shift //= 2
            return r

        def spread(r):
            return jnp.concatenate([r] * (GR // SUB), axis=0)

        def features(p):
            ep = jnp.exp(p - spread(over_features(jnp.maximum, p)))
            en = jnp.exp(spread(over_features(jnp.minimum, p)) - p)
            fp = ep * spread(1.0 / over_features(jnp.add, ep))
            fn = en * spread(1.0 / over_features(jnp.add, en))
            return jnp.concatenate([fp, fn], axis=0).astype(BF16)

        def out_copy(c):
            rows = pl.ds(pl.multiple_of(c * TB, TB), TB)
            return pltpu.make_async_copy(xb_ref.at[rows, :], out_hbm.at[rows, :], out_sem.at[c])

        def layer_b(last):
            kv_ref[...] = jnp.zeros(kv_ref.shape, F32)

            def keys(c, carry):
                rows = pl.ds(pl.multiple_of(c * TB, TB), TB)
                xb_ref[rows, :] = _layernorm(x_ref[rows, :]).astype(BF16)
                xn = xb_ref[rows, :]
                pk = _dot_nt(bt_ref[1], xn)
                v = _dot_nt(bt_ref[2], xn)
                ones = jnp.ones((SUB, TB), F32)
                for j in range(NG):
                    vj = jnp.concatenate([v[j * GR:(j + 1) * GR], ones], axis=0)
                    kv_ref[j] += _dot_nt(vj, features(pk[j * GR:(j + 1) * GR]))
                return carry

            lax.fori_loop(0, NCH, keys, 0)

            shape = (GR + SUB, 2 * GR)
            same_head = (_iota(shape, 0) & (HG - 1)) == (_iota(shape, 1) & (HG - 1))
            for j in range(NG):
                kv_ref[j] = jnp.where(same_head, kv_ref[j], 0.0)

            def queries(c, carry):
                rows = pl.ds(pl.multiple_of(c * TB, TB), TB)
                pq = _dot_nt(bt_ref[0], xb_ref[rows, :])
                for j in range(NG):
                    nd = _dot(kv_ref[j], features(pq[j * GR:(j + 1) * GR]))
                    ot_ref[j * GR:(j + 1) * GR, :] = (
                        nd[:GR] * spread(1.0 / (nd[GR:] + 1e-6)))
                o = ot_ref[...].astype(BF16).T
                x = x_ref[rows, :] + _dot(o, bwo_ref[...])
                x_ref[rows, :] = x
                xn_ref[rows, :] = _layernorm(x)
                xb_ref[rows, :] = x.astype(BF16)

                @pl.when(last)
                def _():
                    out_copy(c).start()

                return carry

            lax.fori_loop(0, NCH, queries, 0)

        def layer(i, carry):
            layer_a()
            layer_b(i == 1)
            return carry

        lax.fori_loop(0, 2, layer, 0)
        for c in range(NCH):
            out_copy(c).wait()

    scratch = [
        pltpu.VMEM((G, D, 3 * PW), BF16),
        pltpu.VMEM((H * DH, D), BF16),
        pltpu.VMEM((NBUF, 3, PW, D), BF16),
        pltpu.VMEM((S, D), BF16),
        pltpu.VMEM((S, D), F32),
        pltpu.VMEM((S, D), F32),
        pltpu.VMEM((L, D), F32),
        pltpu.VMEM((L, H * DH), F32),
        pltpu.VMEM((D, 3 * D), BF16),
        pltpu.VMEM((D, D), BF16),
        pltpu.VMEM((3, D, D), BF16),
        pltpu.VMEM((D, D), BF16),
        pltpu.VMEM((NG, GR + SUB, 2 * GR), F32),
        pltpu.VMEM((D, TB), F32),
        pltpu.SemaphoreType.DMA((NBUF, 3)),
        pltpu.SemaphoreType.DMA((4,)),
        pltpu.SemaphoreType.DMA((NCH,)),
    ]
    return kernel, scratch


@functools.partial(jax.jit, static_argnames=("A_seg_len",))
def pallas_interleave_layers__memory_aug_recurrent_mem_tr__linear_kernel_hedgehog__prompt_kernel(
    A_x: jax.Array,
    A_mem0: jax.Array,
    A_Wq: jax.Array,
    A_Wk: jax.Array,
    A_Wv: jax.Array,
    A_Wo: jax.Array,
    A_seg_len: int,
    B_x: jax.Array,
    B_wqkv: jax.Array,
    B_w_phi: jax.Array,
    B_wo: jax.Array,
):
    del B_x
    B, S, D = A_x.shape
    M = A_mem0.shape[1]
    _, H, DH = A_Wq.shape
    HB = B_w_phi.shape[0]
    assert B == 1

    kernel, scratch = _make_kernel(S, D, H, DH, M, A_seg_len, HB, HG=4, TB=256, NBUF=4)

    def head_major(w):
        return w.transpose(1, 2, 0).reshape(H * DH, D)

    hbm = pl.BlockSpec(memory_space=pltpu.HBM)
    vmem = pl.BlockSpec(memory_space=pltpu.VMEM)
    out = pl.pallas_call(
        kernel,
        out_shape=jax.ShapeDtypeStruct((S, D), A_x.dtype),
        in_specs=[hbm, vmem, hbm, hbm, hbm, hbm, hbm, vmem, hbm],
        out_specs=hbm,
        scratch_shapes=scratch,
        compiler_params=pltpu.CompilerParams(vmem_limit_bytes=110 * 1024 * 1024),
    )(
        A_x.reshape(S, D), A_mem0.reshape(M, D),
        head_major(A_Wq), head_major(A_Wk), head_major(A_Wv), A_Wo.reshape(H * DH, D),
        B_wqkv, B_w_phi.transpose(1, 2, 0), B_wo,
    )
    return out.reshape(B, S, D)
```

```python
import functools

import jax
import jax.numpy as jnp
from jax import lax
import jax.experimental.pallas as pl
import jax.experimental.pallas.tpu as pltpu

F32 = jnp.float32
BF16 = jnp.bfloat16
LANES = 128
SUB = 8


def _dot(a, b):
    return lax.dot_general(a, b, (((1,), (0,)), ((), ())), preferred_element_type=F32)


def _dot_nt(a, b):
    return lax.dot_general(a, b, (((1,), (1,)), ((), ())), preferred_element_type=F32)


def _layernorm(x):
    inv_n = 1.0 / x.shape[-1]
    c = x - jnp.sum(x, axis=-1, keepdims=True) * inv_n
    var = jnp.sum(c * c, axis=-1, keepdims=True) * inv_n
    return c * lax.rsqrt(var + 1e-5)


def _iota(shape, dim):
    return lax.broadcasted_iota(jnp.int32, shape, dim)


def _div20(n):
    return (n * 3277) >> 16


def _make_kernel(S, D, H, DH, M, SEG, HB, *, HG, TB, NBUF, NPRE):
    L = M + SEG
    G = H // 2
    PW = 2 * DH
    NSEG = S // SEG
    XC = S // G
    PRE = SUB
    DB = D // HB
    NG = HB // HG
    GR = DB * HG
    FR = 4 * DB
    LOG_HG = HG.bit_length() - 1
    NCH = S // TB
    scale = DH ** -0.5
    assert PW == 3 * LANES and 2 * L <= LANES and DB == 20 and D < 1024
    assert L % SUB == 0 and M % SUB == 0 and GR % SUB == 0 and 4 % HG == 0
    assert S % TB == 0 and S % G == 0 and NPRE <= NSEG and NBUF + 3 <= G

    def kernel(x_hbm, mem_ref, wq_hbm, wk_hbm, wv_hbm, wo_hbm, bw_hbm, phi_ref, bwo_hbm,
               out_hbm,
               w_ref, wo_ref, stage_ref, xin_ref, xp_ref, hp_ref, pre_ref,
               xb_ref, x_ref, xn_ref, h_ref, hb_ref, o_ref,
               bw_ref, bwo_in_ref, bt_ref, bwo_ref, kv_ref, ot_ref,
               stage_sem, misc_sem, out_sem):

        def stage_copies(g):
            slot = g % NBUF
            rows = pl.ds(pl.multiple_of(g * PW, PW), PW)
            copies = [
                pltpu.make_async_copy(src.at[rows, :],
                                      stage_ref.at[slot, pl.ds(j * PW, PW), :],
                                      stage_sem.at[slot, j])
                for j, src in enumerate((wq_hbm, wk_hbm, wv_hbm))]
            copies.append(pltpu.make_async_copy(
                x_hbm.at[pl.ds(g * (XC // SEG), XC // SEG)], xin_ref.at[slot],
                stage_sem.at[slot, 3]))
            return copies

        xp_copy = pltpu.make_async_copy(
            x_hbm.at[pl.ds(0, NPRE), pl.ds(SEG - PRE, PRE), :], xp_ref, misc_sem.at[0])
        bw_copy = pltpu.make_async_copy(bw_hbm, bw_ref, misc_sem.at[1])
        bwo_copy = pltpu.make_async_copy(bwo_hbm, bwo_in_ref, misc_sem.at[2])
        wo_copy = pltpu.make_async_copy(wo_hbm, wo_ref, misc_sem.at[3])

        xp_copy.start()
        for cp in stage_copies(0):
            cp.start()
        xp_copy.wait()
        for g in range(1, NBUF):
            for cp in stage_copies(g):
                cp.start()
        hp_ref[...] = _layernorm(
            xp_ref[...].astype(F32).reshape(NPRE * PRE, D)).astype(BF16)

        def load_body(g, carry):
            slot = g % NBUF
            for cp in stage_copies(g):
                cp.wait()
            pre_ref[g] = _dot_nt(hp_ref[...], stage_ref[slot])
            w_ref[g] = pltpu.bitcast(stage_ref[slot].T, jnp.uint32)
            rows = pl.ds(pl.multiple_of(g * XC, XC), XC)
            x = xin_ref[slot].astype(F32).reshape(XC, D)
            x_ref[rows, :] = x
            xn_ref[rows, :] = _layernorm(x)

            @pl.when(g + NBUF < G)
            def _():
                for cp in stage_copies(g + NBUF):
                    cp.start()

            @pl.when(g + NBUF == G)
            def _():
                bw_copy.start()
                bwo_copy.start()

            @pl.when(g + NBUF == G + 1)
            def _():
                wo_copy.start()

            return carry

        lax.fori_loop(0, G, load_body, 0)

        eh = _iota((HB, D), 0) * DB
        ec = _iota((HB, D), 1)
        phi_flat = None
        for d in range(DB):
            t = _dot(phi_ref[d], jnp.where(ec == eh + d, 1.0, 0.0).astype(BF16))
            phi_flat = t if phi_flat is None else phi_flat + t
        nf = _iota((FR, DB), 0) >> LOG_HG
        sel = jnp.where(nf - DB * _div20(nf) == _iota((FR, DB), 1), 1.0, 0.0)
        phi_rows = _dot(sel.astype(BF16), phi_flat.astype(BF16))
        bw_copy.wait()
        bwo_copy.wait()
        for r0 in range(0, D, FR):
            c0 = r0 // LANES * LANES
            c1 = pl.cdiv(r0 + FR, LANES) * LANES
            n = _iota((FR, c1 - c0), 0) + r0
            c = _iota((FR, c1 - c0), 1) + c0
            grp = _div20(n >> LOG_HG)
            feat = (n >> LOG_HG) - DB * grp
            head = (grp << LOG_HG) + (n & (HG - 1))
            perm = jnp.where(c == head * DB + feat, 1.0, 0.0).astype(BF16)
            fold = jnp.where(_div20(c) == head, phi_rows[:, c0:c1], 0.0).astype(BF16)
            for j, lhs in enumerate((fold, fold, perm)):
                bt_ref[j, r0:r0 + FR, :] = _dot_nt(
                    lhs, bw_ref[:, j * D + c0:j * D + c1]).astype(BF16)
            bwo_ref[r0:r0 + FR, :] = _dot(perm, bwo_in_ref[c0:c1, :]).astype(BF16)
        wo_copy.wait()

        def layer_a(start, stop, pre):
            row = _iota((L, 2 * L), 0)
            col = _iota((L, 2 * L), 1)
            first = col < L
            visible = (row < M) | (row >= jnp.where(first, col, col - L))
            low = _iota((L, LANES), 1) < DH - LANES
            zero = jnp.zeros((L, LANES), F32)

            def block_diag(t):
                t0, t1, t2 = t[:, :LANES], t[:, LANES:2 * LANES], t[:, 2 * LANES:]
                top = jnp.concatenate([t0, jnp.where(low, t1, 0.0), zero], axis=1)
                bot = jnp.concatenate([zero, jnp.where(low, 0.0, t1), t2], axis=1)
                return jnp.concatenate([top, bot], axis=0).astype(BF16)

            def step(s, carry):
                r0 = pl.multiple_of(s * SEG, SEG)
                rows = pl.ds(r0, SEG)
                if pre:
                    hb_ref[...] = jnp.concatenate(
                        [h_ref[0:M, :], xn_ref[pl.ds(r0, SEG - PRE), :]], axis=0).astype(BF16)
                else:
                    h_ref[M:L, :] = xn_ref[rows, :]
                st = {}
                acc = [None]

                def project(g):
                    w = pltpu.bitcast(w_ref[g], BF16)
                    if pre:
                        qkv = jnp.concatenate(
                            [_dot(hb_ref[...], w),
                             pre_ref[g, pl.ds(pl.multiple_of(s * PRE, PRE), PRE), :]], axis=0)
                    else:
                        qkv = _dot(h_ref[...], w)
                    st[g] = [qkv[:, :PW], block_diag(qkv[:, PW:2 * PW]),
                             block_diag(qkv[:, 2 * PW:])]

                def attend(g):
                    sc = jnp.where(visible, _dot_nt(st[g][0], st[g][1]) * scale, -1e9)
                    m0 = jnp.max(jnp.where(first, sc, -jnp.inf), axis=1, keepdims=True)
                    m1 = jnp.max(jnp.where(first, -jnp.inf, sc), axis=1, keepdims=True)
                    e = jnp.exp(sc - jnp.where(first, m0, m1))
                    s0 = jnp.sum(jnp.where(first, e, 0.0), axis=1, keepdims=True)
                    s1 = jnp.sum(jnp.where(first, 0.0, e), axis=1, keepdims=True)
                    st[g][0] = e / jnp.where(first, s0, s1)

                def mix(g):
                    o_ref[:, g * PW:(g + 1) * PW] = _dot(st[g][0], st[g][2])

                def out_proj(g):
                    r = _dot(o_ref[:, g * PW:(g + 1) * PW], wo_ref[g * PW:(g + 1) * PW, :])
                    acc[0] = r if acc[0] is None else acc[0] + r

                done = 0
                for i in range(G + 2):
                    if i < G:
                        project(i)
                    else:
                        for _ in range(3):
                            out_proj(done)
                            done += 1
                    if 0 <= i - 1 < G:
                        attend(i - 1)
                    if 0 <= i - 2 < G:
                        mix(i - 2)
                for g in range(done, G):
                    out_proj(g)
                h_ref[0:M, :] = acc[0][0:M]
                x_ref[rows, :] = x_ref[rows, :] + acc[0][M:L]
                return carry

            lax.fori_loop(start, stop, step, 0)

        def over_features(op, p):
            r = p[0:SUB]
            for i in range(1, GR // SUB):
                r = op(r, p[i * SUB:(i + 1) * SUB])
            shift = SUB // 2
            while shift >= HG:
                r = op(r, pltpu.roll(r, shift, 0))
                shift //= 2
            return r

        def spread(r):
            return jnp.concatenate([r] * (GR // SUB), axis=0)

        def features(p):
            ep = jnp.exp(p - spread(over_features(jnp.maximum, p)))
            en = jnp.exp(spread(over_features(jnp.minimum, p)) - p)
            fp = ep * spread(1.0 / over_features(jnp.add, ep))
            fn = en * spread(1.0 / over_features(jnp.add, en))
            return jnp.concatenate([fp, fn], axis=0).astype(BF16)

        def out_copy(c):
            rows = pl.ds(pl.multiple_of(c * TB, TB), TB)
            return pltpu.make_async_copy(xb_ref.at[rows, :], out_hbm.at[rows, :], out_sem.at[c])

        def layer_b(last):
            kv_ref[...] = jnp.zeros(kv_ref.shape, F32)

            def keys(c, carry):
                rows = pl.ds(pl.multiple_of(c * TB, TB), TB)
                xb_ref[rows, :] = _layernorm(x_ref[rows, :]).astype(BF16)
                xn = xb_ref[rows, :]
                pk = _dot_nt(bt_ref[1], xn)
                v = _dot_nt(bt_ref[2], xn)
                ones = jnp.ones((SUB, TB), F32)
                for j in range(NG):
                    vj = jnp.concatenate([v[j * GR:(j + 1) * GR], ones], axis=0)
                    kv_ref[j] += _dot_nt(vj, features(pk[j * GR:(j + 1) * GR]))
                return carry

            lax.fori_loop(0, NCH, keys, 0)

            shape = (GR + SUB, 2 * GR)
            same_head = (_iota(shape, 0) & (HG - 1)) == (_iota(shape, 1) & (HG - 1))
            for j in range(NG):
                kv_ref[j] = jnp.where(same_head, kv_ref[j], 0.0)

            def queries(c, carry):
                rows = pl.ds(pl.multiple_of(c * TB, TB), TB)
                pq = _dot_nt(bt_ref[0], xb_ref[rows, :])
                for j in range(NG):
                    nd = _dot(kv_ref[j], features(pq[j * GR:(j + 1) * GR]))
                    ot_ref[j * GR:(j + 1) * GR, :] = (
                        nd[:GR] * spread(1.0 / (nd[GR:] + 1e-6)))
                o = ot_ref[...].astype(BF16).T
                x = x_ref[rows, :] + _dot(o, bwo_ref[...])
                x_ref[rows, :] = x
                xn_ref[rows, :] = _layernorm(x)
                xb_ref[rows, :] = x.astype(BF16)

                @pl.when(last)
                def _():
                    out_copy(c).start()

                return carry

            lax.fori_loop(0, NCH, queries, 0)

        def layer(i, carry):
            layer_a(jnp.where(i == 0, NPRE, 0), NSEG, pre=False)
            h_ref[0:M, :] = mem_ref[...].astype(F32)
            layer_b(i == 1)
            return carry

        h_ref[0:M, :] = mem_ref[...].astype(F32)
        layer_a(0, NPRE, pre=True)
        lax.fori_loop(0, 2, layer, 0)
        for c in range(NCH):
            out_copy(c).wait()

    scratch = [
        pltpu.VMEM((G, D // 2, 3 * PW), jnp.uint32),
        pltpu.VMEM((H * DH, D), BF16),
        pltpu.VMEM((NBUF, 3 * PW, D), BF16),
        pltpu.VMEM((NBUF, XC // SEG, SEG, D), BF16),
        pltpu.VMEM((NPRE, PRE, D), BF16),
        pltpu.VMEM((NPRE * PRE, D), BF16),
        pltpu.VMEM((G, NPRE * PRE, 3 * PW), F32),
        pltpu.VMEM((S, D), BF16),
        pltpu.VMEM((S, D), F32),
        pltpu.VMEM((S, D), F32),
        pltpu.VMEM((L, D), F32),
        pltpu.VMEM((L - PRE, D), BF16),
        pltpu.VMEM((L, H * DH), F32),
        pltpu.VMEM((D, 3 * D), BF16),
        pltpu.VMEM((D, D), BF16),
        pltpu.VMEM((3, D, D), BF16),
        pltpu.VMEM((D, D), BF16),
        pltpu.VMEM((NG, GR + SUB, 2 * GR), F32),
        pltpu.VMEM((D, TB), F32),
        pltpu.SemaphoreType.DMA((NBUF, 4)),
        pltpu.SemaphoreType.DMA((4,)),
        pltpu.SemaphoreType.DMA((NCH,)),
    ]
    return kernel, scratch


@functools.partial(jax.jit, static_argnames=("A_seg_len",))
def pallas_interleave_layers__memory_aug_recurrent_mem_tr__linear_kernel_hedgehog__prompt_kernel(
    A_x: jax.Array,
    A_mem0: jax.Array,
    A_Wq: jax.Array,
    A_Wk: jax.Array,
    A_Wv: jax.Array,
    A_Wo: jax.Array,
    A_seg_len: int,
    B_x: jax.Array,
    B_wqkv: jax.Array,
    B_w_phi: jax.Array,
    B_wo: jax.Array,
):
    del B_x
    B, S, D = A_x.shape
    M = A_mem0.shape[1]
    _, H, DH = A_Wq.shape
    HB = B_w_phi.shape[0]
    assert B == 1

    kernel, scratch = _make_kernel(S, D, H, DH, M, A_seg_len, HB,
                                   HG=2, TB=512, NBUF=3, NPRE=40)

    def head_major(w):
        return w.transpose(1, 2, 0).reshape(H * DH, D)

    hbm = pl.BlockSpec(memory_space=pltpu.HBM)
    vmem = pl.BlockSpec(memory_space=pltpu.VMEM)
    out = pl.pallas_call(
        kernel,
        out_shape=jax.ShapeDtypeStruct((S, D), A_x.dtype),
        in_specs=[hbm, vmem, hbm, hbm, hbm, hbm, hbm, vmem, hbm],
        out_specs=hbm,
        scratch_shapes=scratch,
        compiler_params=pltpu.CompilerParams(vmem_limit_bytes=110 * 1024 * 1024),
    )(
        A_x.reshape(S // A_seg_len, A_seg_len, D), A_mem0.reshape(M, D),
        head_major(A_Wq), head_major(A_Wk), head_major(A_Wv), A_Wo.reshape(H * DH, D),
        B_wqkv, B_w_phi.transpose(1, 2, 0), B_wo,
    )
    return out.reshape(B, S, D)
```

```python
import functools

import jax
import jax.numpy as jnp
from jax import lax
import jax.experimental.pallas as pl
import jax.experimental.pallas.tpu as pltpu

F32 = jnp.float32
BF16 = jnp.bfloat16
LANES = 128
SUB = 8


def _dot(a, b):
    return lax.dot_general(a, b, (((1,), (0,)), ((), ())), preferred_element_type=F32)


def _dot_nt(a, b):
    return lax.dot_general(a, b, (((1,), (1,)), ((), ())), preferred_element_type=F32)


def _layernorm(x):
    inv_n = 1.0 / x.shape[-1]
    c = x - jnp.sum(x, axis=-1, keepdims=True) * inv_n
    var = jnp.sum(c * c, axis=-1, keepdims=True) * inv_n
    return c * lax.rsqrt(var + 1e-5)


def _iota(shape, dim):
    return lax.broadcasted_iota(jnp.int32, shape, dim)


def _div20(n):
    return (n * 3277) >> 16


def _make_kernel(S, D, H, DH, M, SEG, HB, *, HG, TB, NBUF, NPRE, UNROLL, UNROLL_PRE):
    L = M + SEG
    G = H // 2
    PW = 2 * DH
    NSEG = S // SEG
    XC = S // G
    PRE = SUB
    DB = D // HB
    NG = HB // HG
    GR = DB * HG
    FR = 4 * DB
    LOG_HG = HG.bit_length() - 1
    NCH = S // TB
    scale = DH ** -0.5
    assert PW == 3 * LANES and 2 * L <= LANES and DB == 20 and D < 1024
    assert L % SUB == 0 and M % SUB == 0 and GR % SUB == 0 and 4 % HG == 0
    assert S % TB == 0 and S % G == 0 and NPRE <= NSEG and NBUF < G and G >= 14
    assert NSEG % UNROLL == 0 and NPRE % UNROLL == 0 and NPRE % UNROLL_PRE == 0

    def kernel(x_hbm, mem_ref, wq_hbm, wk_hbm, wv_hbm, wo_hbm, bw_hbm, phi_ref, bwo_hbm,
               out_hbm,
               w_ref, wo_ref, stage_ref, xin_ref, xp_ref, hp_ref, pre_ref,
               xb_ref, x_ref, h_ref, hb_ref,
               bw_ref, bwo_in_ref, phi_rows_ref, bt_ref, bwo_ref, kv_ref,
               stage_sem, wo_sem, misc_sem, out_sem):

        def stage_copies(g):
            slot = g % NBUF
            rows = pl.ds(pl.multiple_of(g * PW, PW), PW)
            copies = [
                pltpu.make_async_copy(src.at[rows, :],
                                      stage_ref.at[slot, pl.ds(j * PW, PW), :],
                                      stage_sem.at[slot, j])
                for j, src in enumerate((wq_hbm, wk_hbm, wv_hbm))]
            copies.append(pltpu.make_async_copy(
                x_hbm.at[pl.ds(g * (XC // SEG), XC // SEG)], xin_ref.at[slot],
                stage_sem.at[slot, 3]))
            return copies

        xp_copy = pltpu.make_async_copy(
            x_hbm.at[pl.ds(0, NPRE), pl.ds(SEG - PRE, PRE), :], xp_ref, misc_sem.at[0])
        bw_copy = pltpu.make_async_copy(bw_hbm, bw_ref, misc_sem.at[1])
        bwo_copy = pltpu.make_async_copy(bwo_hbm, bwo_in_ref, misc_sem.at[2])

        def wo_copy(g):
            rows = pl.ds(pl.multiple_of(g * PW, PW), PW)
            return pltpu.make_async_copy(wo_hbm.at[rows, :], wo_ref.at[rows, :], wo_sem.at[g])

        xp_copy.start()
        for cp in stage_copies(0):
            cp.start()

        eh = _iota((HB, D), 0) * DB
        ec = _iota((HB, D), 1)
        phi_flat = None
        for d in range(DB):
            t = _dot(phi_ref[d], jnp.where(ec == eh + d, 1.0, 0.0).astype(BF16))
            phi_flat = t if phi_flat is None else phi_flat + t
        nf = _iota((FR, DB), 0) >> LOG_HG
        sel = jnp.where(nf - DB * _div20(nf) == _iota((FR, DB), 1), 1.0, 0.0)
        phi_rows_ref[...] = _dot(sel.astype(BF16), phi_flat.astype(BF16))

        xp_copy.wait()
        for g in range(1, NBUF):
            for cp in stage_copies(g):
                cp.start()
        hp_ref[...] = _layernorm(
            xp_ref[...].astype(F32).reshape(NPRE * PRE, D)).astype(BF16)

        def load_body(g, carry):
            slot = g % NBUF
            for cp in stage_copies(g):
                cp.wait()
            pre_ref[g] = _dot_nt(hp_ref[...], stage_ref[slot])
            w_ref[g] = pltpu.bitcast(stage_ref[slot].T, jnp.uint32)
            rows = pl.ds(pl.multiple_of(g * XC, XC), XC)
            x_ref[rows, :] = xin_ref[slot].astype(F32).reshape(XC, D)

            @pl.when(g + NBUF < G)
            def _():
                for cp in stage_copies(g + NBUF):
                    cp.start()
                wo_copy(g).start()

            @pl.when(g + NBUF == G)
            def _():
                for k in range(G - NBUF, G):
                    wo_copy(k).start()

            return carry

        lax.fori_loop(0, G, load_body, 0)
        bw_copy.start()
        bwo_copy.start()

        def layer_a(start, stop, pre, unroll):
            row = _iota((L, 2 * L), 0)
            col = _iota((L, 2 * L), 1)
            first = col < L
            visible = (row < M) | (row >= jnp.where(first, col, col - L))
            low = _iota((L, LANES), 1) < DH - LANES
            zero = jnp.zeros((L, LANES), F32)

            def block_diag(t):
                t0, t1, t2 = t[:, :LANES], t[:, LANES:2 * LANES], t[:, 2 * LANES:]
                top = jnp.concatenate([t0, jnp.where(low, t1, 0.0), zero], axis=1)
                bot = jnp.concatenate([zero, jnp.where(low, 0.0, t1), t2], axis=1)
                return jnp.concatenate([top, bot], axis=0).astype(BF16)

            def step(s, h):
                rows = seg_rows(s)
                chained = h is not None
                if not chained:
                    h = h_ref[...]
                if pre:
                    h = h[:L - PRE].astype(BF16)
                    hb_ref[...] = h
                elif chained:
                    h_ref[...] = h
                st = {}
                acc = [None]

                def project(g):
                    w = pltpu.bitcast(w_ref[g], BF16)
                    if g == 0 and chained:
                        k = D - LANES
                        qkv = _dot(h[:, :k], w[:k]) + _dot(h[:, k:], w[k:])
                    else:
                        qkv = _dot((hb_ref if pre else h_ref)[...], w)
                    if pre:
                        qkv = jnp.concatenate(
                            [qkv, pre_ref[g, pl.ds(pl.multiple_of(s * PRE, PRE), PRE), :]],
                            axis=0)
                    st[g] = [qkv[:, :PW], block_diag(qkv[:, PW:2 * PW]),
                             block_diag(qkv[:, 2 * PW:])]

                def attend(g):
                    sc = jnp.where(visible, _dot_nt(st[g][0], st[g][1]) * scale, -1e9)
                    m0 = jnp.max(jnp.where(first, sc, -jnp.inf), axis=1, keepdims=True)
                    m1 = jnp.max(jnp.where(first, -jnp.inf, sc), axis=1, keepdims=True)
                    e = jnp.exp(sc - jnp.where(first, m0, m1))
                    s0 = jnp.sum(jnp.where(first, e, 0.0), axis=1, keepdims=True)
                    s1 = jnp.sum(jnp.where(first, 0.0, e), axis=1, keepdims=True)
                    st[g][0] = e / jnp.where(first, s0, s1)

                def mix(g):
                    st[g] = _dot(st[g][0], st[g][2])

                def out_proj(g0, g1):
                    o = jnp.concatenate([st[g] for g in range(g0, g1)], axis=1)
                    r = _dot(o, wo_ref[g0 * PW:g1 * PW, :])
                    acc[0] = r if acc[0] is None else acc[0] + r

                for i in range(G + 2):
                    if i < G:
                        project(i)
                    else:
                        for g in range(4 * (i - G), 4 * (i - G + 1)):
                            out_proj(g, g + 1)
                    if 0 <= i - 1 < G:
                        attend(i - 1)
                    if 0 <= i - 2 < G:
                        mix(i - 2)
                    if i == 1:
                        normalise_output(jnp.maximum(s - 1, 0))
                    if i == 3:
                        xn_next = _layernorm(
                            x_ref[seg_rows(jnp.minimum(s + 1, NSEG - 1)), :])
                for g in range(8, G - 4):
                    out_proj(g, g + 1)
                out_proj(G - 4, G)
                x_ref[rows, :] = x_ref[rows, :] + acc[0][M:L]
                return jnp.concatenate([acc[0][0:M], xn_next], axis=0)

            def steps(i, carry):
                h = None
                for u in range(unroll):
                    h = step(i * unroll + u, h)
                h_ref[...] = h
                return carry

            lax.fori_loop(start // unroll, stop // unroll, steps, 0)

        def seg_rows(s):
            return pl.ds(s * SEG if isinstance(s, int) else pl.multiple_of(s * SEG, SEG), SEG)

        def normalise_output(s):
            xb_ref[seg_rows(s), :] = _layernorm(x_ref[seg_rows(s), :]).astype(BF16)

        def reset_memory():
            h_ref[0:M, :] = mem_ref[...].astype(F32)
            h_ref[M:L, :] = _layernorm(x_ref[0:SEG, :])

        def fold_hedgehog_weights():
            bw_copy.wait()
            bwo_copy.wait()
            for r0 in range(0, D, FR):
                c0 = r0 // LANES * LANES
                c1 = pl.cdiv(r0 + FR, LANES) * LANES
                n = _iota((FR, c1 - c0), 0) + r0
                c = _iota((FR, c1 - c0), 1) + c0
                grp = _div20(n >> LOG_HG)
                feat = (n >> LOG_HG) - DB * grp
                head = (grp << LOG_HG) + (n & (HG - 1))
                perm = jnp.where(c == head * DB + feat, 1.0, 0.0).astype(BF16)
                fold = jnp.where(_div20(c) == head, phi_rows_ref[:, c0:c1], 0.0).astype(BF16)
                for j, lhs in enumerate((fold, fold, perm)):
                    bt_ref[j, r0:r0 + FR, :] = _dot_nt(
                        lhs, bw_ref[:, j * D + c0:j * D + c1]).astype(BF16)
                bwo_ref[r0:r0 + FR, :] = _dot(perm, bwo_in_ref[c0:c1, :]).astype(BF16)

        def over_features(op, p):
            r = p[0:SUB]
            for i in range(1, GR // SUB):
                r = op(r, p[i * SUB:(i + 1) * SUB])
            shift = SUB // 2
            while shift >= HG:
                r = op(r, pltpu.roll(r, shift, 0))
                shift //= 2
            return r

        def spread(r):
            return jnp.concatenate([r] * (GR // SUB), axis=0)

        def features(p):
            ep = jnp.exp(p - spread(over_features(jnp.maximum, p)))
            en = jnp.exp(spread(over_features(jnp.minimum, p)) - p)
            fp = ep * spread(1.0 / over_features(jnp.add, ep))
            fn = en * spread(1.0 / over_features(jnp.add, en))
            return jnp.concatenate([fp, fn], axis=0).astype(BF16)

        def out_copy(c):
            rows = pl.ds(pl.multiple_of(c * TB, TB), TB)
            return pltpu.make_async_copy(xb_ref.at[rows, :], out_hbm.at[rows, :], out_sem.at[c])

        def layer_b(last):
            kv_ref[...] = jnp.zeros(kv_ref.shape, F32)

            def keys(c, carry):
                rows = pl.ds(pl.multiple_of(c * TB, TB), TB)
                pk = _dot_nt(bt_ref[1], xb_ref[rows, :])
                v = _dot_nt(bt_ref[2], xb_ref[rows, :])
                ones = jnp.ones((SUB, TB), F32)
                for j in range(NG):
                    vj = jnp.concatenate([v[j * GR:(j + 1) * GR], ones], axis=0)
                    kv_ref[j] += _dot_nt(vj, features(pk[j * GR:(j + 1) * GR]))
                return carry

            lax.fori_loop(0, NCH, keys, 0)

            shape = (GR + SUB, 2 * GR)
            same_head = (_iota(shape, 0) & (HG - 1)) == (_iota(shape, 1) & (HG - 1))
            for j in range(NG):
                kv_ref[j] = jnp.where(same_head, kv_ref[j], 0.0)

            def queries(c, carry):
                rows = pl.ds(pl.multiple_of(c * TB, TB), TB)
                pq = _dot_nt(bt_ref[0], xb_ref[rows, :])
                o = []
                for j in range(NG):
                    nd = _dot(kv_ref[j], features(pq[j * GR:(j + 1) * GR]))
                    o.append(nd[:GR] * spread(1.0 / (nd[GR:] + 1e-6)))
                o = jnp.concatenate(o, axis=0).astype(BF16).T
                x = x_ref[rows, :] + _dot(o, bwo_ref[...])
                x_ref[rows, :] = x
                xb_ref[rows, :] = x.astype(BF16)

                @pl.when(last)
                def _():
                    out_copy(c).start()

                return carry

            lax.fori_loop(0, NCH, queries, 0)

        def layer(i, carry):
            layer_a(jnp.where(i == 0, NPRE, 0), NSEG, pre=False, unroll=UNROLL)
            normalise_output(NSEG - 1)
            layer_b(i == 1)
            reset_memory()
            return carry

        reset_memory()
        for g in range(G):
            wo_copy(g).wait()
        layer_a(0, NPRE, pre=True, unroll=UNROLL_PRE)
        fold_hedgehog_weights()
        lax.fori_loop(0, 2, layer, 0)
        for c in range(NCH):
            out_copy(c).wait()

    scratch = [
        pltpu.VMEM((G, D // 2, 3 * PW), jnp.uint32),
        pltpu.VMEM((H * DH, D), BF16),
        pltpu.VMEM((NBUF, 3 * PW, D), BF16),
        pltpu.VMEM((NBUF, XC // SEG, SEG, D), BF16),
        pltpu.VMEM((NPRE, PRE, D), BF16),
        pltpu.VMEM((NPRE * PRE, D), BF16),
        pltpu.VMEM((G, NPRE * PRE, 3 * PW), F32),
        pltpu.VMEM((S, D), BF16),
        pltpu.VMEM((S, D), F32),
        pltpu.VMEM((L, D), F32),
        pltpu.VMEM((L - PRE, D), BF16),
        pltpu.VMEM((D, 3 * D), BF16),
        pltpu.VMEM((D, D), BF16),
        pltpu.VMEM((FR, D), F32),
        pltpu.VMEM((3, D, D), BF16),
        pltpu.VMEM((D, D), BF16),
        pltpu.VMEM((NG, GR + SUB, 2 * GR), F32),
        pltpu.SemaphoreType.DMA((NBUF, 4)),
        pltpu.SemaphoreType.DMA((G,)),
        pltpu.SemaphoreType.DMA((3,)),
        pltpu.SemaphoreType.DMA((NCH,)),
    ]
    return kernel, scratch


@functools.partial(jax.jit, static_argnames=("A_seg_len",))
def pallas_interleave_layers__memory_aug_recurrent_mem_tr__linear_kernel_hedgehog__prompt_kernel(
    A_x: jax.Array,
    A_mem0: jax.Array,
    A_Wq: jax.Array,
    A_Wk: jax.Array,
    A_Wv: jax.Array,
    A_Wo: jax.Array,
    A_seg_len: int,
    B_x: jax.Array,
    B_wqkv: jax.Array,
    B_w_phi: jax.Array,
    B_wo: jax.Array,
):
    del B_x
    B, S, D = A_x.shape
    M = A_mem0.shape[1]
    _, H, DH = A_Wq.shape
    HB = B_w_phi.shape[0]
    assert B == 1

    kernel, scratch = _make_kernel(S, D, H, DH, M, A_seg_len, HB,
                                   HG=2, TB=512, NBUF=3, NPRE=44, UNROLL=2, UNROLL_PRE=1)

    def head_major(w):
        return w.transpose(1, 2, 0).reshape(H * DH, D)

    hbm = pl.BlockSpec(memory_space=pltpu.HBM)
    vmem = pl.BlockSpec(memory_space=pltpu.VMEM)
    out = pl.pallas_call(
        kernel,
        out_shape=jax.ShapeDtypeStruct((S, D), A_x.dtype),
        in_specs=[hbm, vmem, hbm, hbm, hbm, hbm, hbm, vmem, hbm],
        out_specs=hbm,
        scratch_shapes=scratch,
        compiler_params=pltpu.CompilerParams(vmem_limit_bytes=110 * 1024 * 1024),
    )(
        A_x.reshape(S // A_seg_len, A_seg_len, D), A_mem0.reshape(M, D),
        head_major(A_Wq), head_major(A_Wk), head_major(A_Wv), A_Wo.reshape(H * DH, D),
        B_wqkv, B_w_phi.transpose(1, 2, 0), B_wo,
    )
    return out.reshape(B, S, D)
```

```python
import functools

import jax
import jax.numpy as jnp
from jax import lax
import jax.experimental.pallas as pl
import jax.experimental.pallas.tpu as pltpu

F32 = jnp.float32
BF16 = jnp.bfloat16
LANES = 128
SUB = 8


def _dot(a, b):
    return lax.dot_general(a, b, (((1,), (0,)), ((), ())), preferred_element_type=F32)


def _dot_nt(a, b):
    return lax.dot_general(a, b, (((1,), (1,)), ((), ())), preferred_element_type=F32)


def _layernorm(x):
    inv_n = 1.0 / x.shape[-1]
    c = x - jnp.sum(x, axis=-1, keepdims=True) * inv_n
    var = jnp.sum(c * c, axis=-1, keepdims=True) * inv_n
    return c * lax.rsqrt(var + 1e-5)


def _iota(shape, dim):
    return lax.broadcasted_iota(jnp.int32, shape, dim)


def _div20(n):
    return (n * 3277) >> 16


def _make_kernel(S, D, H, DH, M, SEG, HB, *, HG, TB, NBUF, NPRE, UNROLL, UNROLL_PRE):
    L = M + SEG
    G = H // 2
    PW = 2 * DH
    NSEG = S // SEG
    XC = S // G
    PRE = SUB
    DB = D // HB
    NG = HB // HG
    GR = DB * HG
    FR = 4 * DB
    LOG_HG = HG.bit_length() - 1
    NCH = S // TB
    scale = DH ** -0.5
    assert PW == 3 * LANES and 2 * L <= LANES and DB == 20 and D < 1024
    assert L % SUB == 0 and M % SUB == 0 and GR % SUB == 0 and 4 % HG == 0
    assert S % TB == 0 and S % G == 0 and NPRE <= NSEG and NBUF < G and G >= 14
    assert NSEG % UNROLL == 0 and NPRE % UNROLL == 0 and NPRE % UNROLL_PRE == 0

    def kernel(x_hbm, mem_ref, wq_hbm, wk_hbm, wv_hbm, wo_hbm, bw_hbm, phi_ref, bwo_hbm,
               out_hbm,
               w_ref, wo_ref, stage_ref, xin_ref, xp_ref, hp_ref, pre_ref,
               xb_ref, x_ref, h_ref,
               bw_ref, bwo_in_ref, phi_rows_ref, bt_ref, bwo_ref, kv_ref,
               stage_sem, wo_sem, misc_sem, out_sem):

        def stage_copies(g):
            slot = g % NBUF
            rows = pl.ds(pl.multiple_of(g * PW, PW), PW)
            copies = [
                pltpu.make_async_copy(src.at[rows, :],
                                      stage_ref.at[slot, pl.ds(j * PW, PW), :],
                                      stage_sem.at[slot, j])
                for j, src in enumerate((wq_hbm, wk_hbm, wv_hbm))]
            copies.append(pltpu.make_async_copy(
                x_hbm.at[pl.ds(g * (XC // SEG), XC // SEG)], xin_ref.at[slot],
                stage_sem.at[slot, 3]))
            return copies

        xp_copy = pltpu.make_async_copy(
            x_hbm.at[pl.ds(0, NPRE), pl.ds(SEG - PRE, PRE), :], xp_ref, misc_sem.at[0])
        bw_copy = pltpu.make_async_copy(bw_hbm, bw_ref, misc_sem.at[1])
        bwo_copy = pltpu.make_async_copy(bwo_hbm, bwo_in_ref, misc_sem.at[2])

        def wo_copy(g):
            rows = pl.ds(pl.multiple_of(g * PW, PW), PW)
            return pltpu.make_async_copy(wo_hbm.at[rows, :], wo_ref.at[rows, :], wo_sem.at[g])

        xp_copy.start()
        for cp in stage_copies(0):
            cp.start()

        eh = _iota((HB, D), 0) * DB
        ec = _iota((HB, D), 1)
        phi_flat = None
        for d in range(DB):
            t = _dot(phi_ref[d], jnp.where(ec == eh + d, 1.0, 0.0).astype(BF16))
            phi_flat = t if phi_flat is None else phi_flat + t
        nf = _iota((FR, DB), 0) >> LOG_HG
        sel = jnp.where(nf - DB * _div20(nf) == _iota((FR, DB), 1), 1.0, 0.0)
        phi_rows_ref[...] = _dot(sel.astype(BF16), phi_flat.astype(BF16))

        xp_copy.wait()
        for g in range(1, NBUF):
            for cp in stage_copies(g):
                cp.start()
        hp_ref[...] = _layernorm(
            xp_ref[...].astype(F32).reshape(NPRE * PRE, D)).astype(BF16)

        def load_body(g, carry):
            slot = g % NBUF
            for cp in stage_copies(g):
                cp.wait()
            pre_ref[g] = _dot_nt(hp_ref[...], stage_ref[slot])
            w_ref[g] = pltpu.bitcast(stage_ref[slot].T, jnp.uint32)
            rows = pl.ds(pl.multiple_of(g * XC, XC), XC)
            x_ref[rows, :] = xin_ref[slot].astype(F32).reshape(XC, D)

            @pl.when(g + NBUF < G)
            def _():
                for cp in stage_copies(g + NBUF):
                    cp.start()
                wo_copy(g).start()

            @pl.when(g + NBUF == G)
            def _():
                for k in range(G - NBUF, G):
                    wo_copy(k).start()

            return carry

        lax.fori_loop(0, G, load_body, 0)
        bw_copy.start()
        bwo_copy.start()

        def layer_a(start, stop, pre, unroll):
            row = _iota((L, 2 * L), 0)
            col = _iota((L, 2 * L), 1)
            first = col < L
            visible = (row < M) | (row >= jnp.where(first, col, col - L))
            low = _iota((L, LANES), 1) < DH - LANES
            zero = jnp.zeros((L, LANES), F32)

            def block_diag(t):
                t0, t1, t2 = t[:, :LANES], t[:, LANES:2 * LANES], t[:, 2 * LANES:]
                top = jnp.concatenate([t0, jnp.where(low, t1, 0.0), zero], axis=1)
                bot = jnp.concatenate([zero, jnp.where(low, 0.0, t1), t2], axis=1)
                return jnp.concatenate([top, bot], axis=0).astype(BF16)

            def step(s, h):
                rows = seg_rows(s)
                chained = h is not None
                if not chained:
                    h = h_ref[...]
                if pre:
                    h = h[:L - PRE].astype(BF16)
                st = {}
                acc = [None]

                def project(g):
                    w = pltpu.bitcast(w_ref[g], BF16)
                    if g == 0 and chained:
                        qkv = functools.reduce(jnp.add, [
                            _dot(h[:, k:k + LANES], w[k:k + LANES])
                            for k in range(0, D, LANES)])
                    else:
                        qkv = _dot(h, w)
                    if pre:
                        qkv = jnp.concatenate(
                            [qkv, pre_ref[g, pl.ds(pl.multiple_of(s * PRE, PRE), PRE), :]],
                            axis=0)
                    st[g] = [qkv[:, :PW], block_diag(qkv[:, PW:2 * PW]),
                             block_diag(qkv[:, 2 * PW:])]

                def attend(g):
                    sc = jnp.where(visible, _dot_nt(st[g][0], st[g][1]) * scale, -1e9)
                    m0 = jnp.max(jnp.where(first, sc, -jnp.inf), axis=1, keepdims=True)
                    m1 = jnp.max(jnp.where(first, -jnp.inf, sc), axis=1, keepdims=True)
                    e = jnp.exp(sc - jnp.where(first, m0, m1))
                    s0 = jnp.sum(jnp.where(first, e, 0.0), axis=1, keepdims=True)
                    s1 = jnp.sum(jnp.where(first, 0.0, e), axis=1, keepdims=True)
                    st[g][0] = e / jnp.where(first, s0, s1)

                def mix(g):
                    st[g] = _dot(st[g][0], st[g][2])

                def out_proj(g0, g1):
                    o = jnp.concatenate([st[g] for g in range(g0, g1)], axis=1)
                    r = _dot(o, wo_ref[g0 * PW:g1 * PW, :])
                    acc[0] = r if acc[0] is None else acc[0] + r

                for i in range(G + 2):
                    if i < G:
                        project(i)
                    else:
                        for g in range(4 * (i - G), 4 * (i - G + 1)):
                            out_proj(g, g + 1)
                    if 0 <= i - 1 < G:
                        attend(i - 1)
                    if 0 <= i - 2 < G:
                        mix(i - 2)
                    if i == 1:
                        normalise_output(jnp.maximum(s - 1, 0))
                    if i == 3:
                        xn_next = _layernorm(
                            x_ref[seg_rows(jnp.minimum(s + 1, NSEG - 1)), :])
                for g in range(8, G - 4):
                    out_proj(g, g + 1)
                o = jnp.concatenate([st[g] for g in range(G - 4, G)], axis=1)
                y = jnp.concatenate([
                    acc[0][:, c:c + LANES]
                    + _dot(o, wo_ref[(G - 4) * PW:G * PW, c:c + LANES])
                    for c in range(0, D, LANES)], axis=1)
                x_ref[rows, :] = x_ref[rows, :] + y[M:L]
                return jnp.concatenate([y[0:M], xn_next], axis=0)

            def steps(i, carry):
                h = None
                for u in range(unroll):
                    h = step(i * unroll + u, h)
                h_ref[...] = h
                return carry

            lax.fori_loop(start // unroll, stop // unroll, steps, 0)

        def seg_rows(s):
            return pl.ds(s * SEG if isinstance(s, int) else pl.multiple_of(s * SEG, SEG), SEG)

        def normalise_output(s):
            xb_ref[seg_rows(s), :] = _layernorm(x_ref[seg_rows(s), :]).astype(BF16)

        def reset_memory():
            h_ref[0:M, :] = mem_ref[...].astype(F32)
            h_ref[M:L, :] = _layernorm(x_ref[0:SEG, :])

        def fold_hedgehog_weights():
            bw_copy.wait()
            bwo_copy.wait()
            for r0 in range(0, D, FR):
                c0 = r0 // LANES * LANES
                c1 = pl.cdiv(r0 + FR, LANES) * LANES
                n = _iota((FR, c1 - c0), 0) + r0
                c = _iota((FR, c1 - c0), 1) + c0
                grp = _div20(n >> LOG_HG)
                feat = (n >> LOG_HG) - DB * grp
                head = (grp << LOG_HG) + (n & (HG - 1))
                perm = jnp.where(c == head * DB + feat, 1.0, 0.0).astype(BF16)
                fold = jnp.where(_div20(c) == head, phi_rows_ref[:, c0:c1], 0.0).astype(BF16)
                for j, lhs in enumerate((fold, fold, perm)):
                    bt_ref[j, r0:r0 + FR, :] = _dot_nt(
                        lhs, bw_ref[:, j * D + c0:j * D + c1]).astype(BF16)
                bwo_ref[r0:r0 + FR, :] = _dot(perm, bwo_in_ref[c0:c1, :]).astype(BF16)

        def over_features(op, p):
            r = p[0:SUB]
            for i in range(1, GR // SUB):
                r = op(r, p[i * SUB:(i + 1) * SUB])
            shift = SUB // 2
            while shift >= HG:
                r = op(r, pltpu.roll(r, shift, 0))
                shift //= 2
            return r

        def spread(r):
            return jnp.concatenate([r] * (GR // SUB), axis=0)

        def features(p):
            ep = jnp.exp(p - spread(over_features(jnp.maximum, p)))
            en = jnp.exp(spread(over_features(jnp.minimum, p)) - p)
            fp = ep * spread(1.0 / over_features(jnp.add, ep))
            fn = en * spread(1.0 / over_features(jnp.add, en))
            return jnp.concatenate([fp, fn], axis=0).astype(BF16)

        def out_copy(c):
            rows = pl.ds(pl.multiple_of(c * TB, TB), TB)
            return pltpu.make_async_copy(xb_ref.at[rows, :], out_hbm.at[rows, :], out_sem.at[c])

        def layer_b(last):
            kv_ref[...] = jnp.zeros(kv_ref.shape, F32)

            def keys(c, carry):
                rows = pl.ds(pl.multiple_of(c * TB, TB), TB)
                pk = _dot_nt(bt_ref[1], xb_ref[rows, :])
                v = _dot_nt(bt_ref[2], xb_ref[rows, :])
                ones = jnp.ones((SUB, TB), F32)
                for j in range(NG):
                    vj = jnp.concatenate([v[j * GR:(j + 1) * GR], ones], axis=0)
                    kv_ref[j] += _dot_nt(vj, features(pk[j * GR:(j + 1) * GR]))
                return carry

            lax.fori_loop(0, NCH, keys, 0)

            shape = (GR + SUB, 2 * GR)
            same_head = (_iota(shape, 0) & (HG - 1)) == (_iota(shape, 1) & (HG - 1))
            for j in range(NG):
                kv_ref[j] = jnp.where(same_head, kv_ref[j], 0.0)

            def queries(c, carry):
                rows = pl.ds(pl.multiple_of(c * TB, TB), TB)
                pq = _dot_nt(bt_ref[0], xb_ref[rows, :])
                o = []
                for j in range(NG):
                    nd = _dot(kv_ref[j], features(pq[j * GR:(j + 1) * GR]))
                    o.append(nd[:GR] * spread(1.0 / (nd[GR:] + 1e-6)))
                o = jnp.concatenate(o, axis=0).astype(BF16).T
                x = x_ref[rows, :] + _dot(o, bwo_ref[...])
                x_ref[rows, :] = x
                xb_ref[rows, :] = x.astype(BF16)

                @pl.when(last)
                def _():
                    out_copy(c).start()

                return carry

            lax.fori_loop(0, NCH, queries, 0)

        def layer(i, carry):
            layer_a(jnp.where(i == 0, NPRE, 0), NSEG, pre=False, unroll=UNROLL)
            normalise_output(NSEG - 1)
            layer_b(i == 1)
            reset_memory()
            return carry

        reset_memory()
        for g in range(G):
            wo_copy(g).wait()
        layer_a(0, NPRE, pre=True, unroll=UNROLL_PRE)
        fold_hedgehog_weights()
        lax.fori_loop(0, 2, layer, 0)
        for c in range(NCH):
            out_copy(c).wait()

    scratch = [
        pltpu.VMEM((G, D // 2, 3 * PW), jnp.uint32),
        pltpu.VMEM((H * DH, D), BF16),
        pltpu.VMEM((NBUF, 3 * PW, D), BF16),
        pltpu.VMEM((NBUF, XC // SEG, SEG, D), BF16),
        pltpu.VMEM((NPRE, PRE, D), BF16),
        pltpu.VMEM((NPRE * PRE, D), BF16),
        pltpu.VMEM((G, NPRE * PRE, 3 * PW), F32),
        pltpu.VMEM((S, D), BF16),
        pltpu.VMEM((S, D), F32),
        pltpu.VMEM((L, D), F32),
        pltpu.VMEM((D, 3 * D), BF16),
        pltpu.VMEM((D, D), BF16),
        pltpu.VMEM((FR, D), F32),
        pltpu.VMEM((3, D, D), BF16),
        pltpu.VMEM((D, D), BF16),
        pltpu.VMEM((NG, GR + SUB, 2 * GR), F32),
        pltpu.SemaphoreType.DMA((NBUF, 4)),
        pltpu.SemaphoreType.DMA((G,)),
        pltpu.SemaphoreType.DMA((3,)),
        pltpu.SemaphoreType.DMA((NCH,)),
    ]
    return kernel, scratch


@functools.partial(jax.jit, static_argnames=("A_seg_len",))
def pallas_interleave_layers__memory_aug_recurrent_mem_tr__linear_kernel_hedgehog__prompt_kernel(
    A_x: jax.Array,
    A_mem0: jax.Array,
    A_Wq: jax.Array,
    A_Wk: jax.Array,
    A_Wv: jax.Array,
    A_Wo: jax.Array,
    A_seg_len: int,
    B_x: jax.Array,
    B_wqkv: jax.Array,
    B_w_phi: jax.Array,
    B_wo: jax.Array,
):
    del B_x
    B, S, D = A_x.shape
    M = A_mem0.shape[1]
    _, H, DH = A_Wq.shape
    HB = B_w_phi.shape[0]
    assert B == 1

    kernel, scratch = _make_kernel(S, D, H, DH, M, A_seg_len, HB,
                                   HG=2, TB=512, NBUF=3, NPRE=44, UNROLL=2, UNROLL_PRE=2)

    def head_major(w):
        return w.transpose(1, 2, 0).reshape(H * DH, D)

    hbm = pl.BlockSpec(memory_space=pltpu.HBM)
    vmem = pl.BlockSpec(memory_space=pltpu.VMEM)
    out = pl.pallas_call(
        kernel,
        out_shape=jax.ShapeDtypeStruct((S, D), A_x.dtype),
        in_specs=[hbm, vmem, hbm, hbm, hbm, hbm, hbm, vmem, hbm],
        out_specs=hbm,
        scratch_shapes=scratch,
        compiler_params=pltpu.CompilerParams(vmem_limit_bytes=110 * 1024 * 1024),
    )(
        A_x.reshape(S // A_seg_len, A_seg_len, D), A_mem0.reshape(M, D),
        head_major(A_Wq), head_major(A_Wk), head_major(A_Wv), A_Wo.reshape(H * DH, D),
        B_wqkv, B_w_phi.transpose(1, 2, 0), B_wo,
    )
    return out.reshape(B, S, D)
```

```python
import functools

import jax
import jax.numpy as jnp
from jax import lax
import jax.experimental.pallas as pl
import jax.experimental.pallas.tpu as pltpu

F32 = jnp.float32
BF16 = jnp.bfloat16
LANES = 128
SUB = 8


def _dot(a, b):
    return lax.dot_general(a, b, (((1,), (0,)), ((), ())), preferred_element_type=F32)


def _dot_nt(a, b):
    return lax.dot_general(a, b, (((1,), (1,)), ((), ())), preferred_element_type=F32)


def _layernorm(x):
    inv_n = 1.0 / x.shape[-1]
    c = x - jnp.sum(x, axis=-1, keepdims=True) * inv_n
    var = jnp.sum(c * c, axis=-1, keepdims=True) * inv_n
    return c * lax.rsqrt(var + 1e-5)


def _iota(shape, dim):
    return lax.broadcasted_iota(jnp.int32, shape, dim)


def _div20(n):
    return (n * 3277) >> 16


def _make_kernel(S, D, H, DH, M, SEG, HB, *, HG, TB, NBUF, NPRE, UNROLL, UNROLL_PRE):
    L = M + SEG
    G = H // 2
    PW = 2 * DH
    NSEG = S // SEG
    XC = S // G
    PRE = SUB
    DB = D // HB
    NG = HB // HG
    GR = DB * HG
    FR = 4 * DB
    LOG_HG = HG.bit_length() - 1
    NCH = S // TB
    scale = DH ** -0.5
    assert PW == 3 * LANES and 2 * L <= LANES and DB == 20 and D < 1024
    assert L % SUB == 0 and M % SUB == 0 and GR % SUB == 0 and HG == 2
    assert S % TB == 0 and S % G == 0 and NPRE <= NSEG and NBUF < G and G >= 14
    assert NSEG % UNROLL == 0 and NPRE % UNROLL == 0 and NPRE % UNROLL_PRE == 0

    def kernel(x_hbm, mem_ref, wq_hbm, wk_hbm, wv_hbm, wo_hbm, bw_hbm, phi_ref, bwo_hbm,
               out_hbm,
               w_ref, wo_ref, stage_ref, xin_ref, xp_ref, hp_ref, pre_ref,
               xb_ref, x_ref, h_ref,
               bw_ref, phi_rows_ref, bt_ref, bwo_ref, kv_ref,
               stage_sem, wo_sem, misc_sem, out_sem):

        def stage_copies(g):
            slot = g % NBUF
            rows = pl.ds(pl.multiple_of(g * PW, PW), PW)
            copies = [
                pltpu.make_async_copy(src.at[rows, :],
                                      stage_ref.at[slot, pl.ds(j * PW, PW), :],
                                      stage_sem.at[slot, j])
                for j, src in enumerate((wq_hbm, wk_hbm, wv_hbm))]
            copies.append(pltpu.make_async_copy(
                x_hbm.at[pl.ds(g * (XC // SEG), XC // SEG)], xin_ref.at[slot],
                stage_sem.at[slot, 3]))
            return copies

        xp_copy = pltpu.make_async_copy(
            x_hbm.at[pl.ds(0, NPRE), pl.ds(SEG - PRE, PRE), :], xp_ref, misc_sem.at[0])
        bw_copy = pltpu.make_async_copy(bw_hbm, bw_ref, misc_sem.at[1])
        bwo_copy = pltpu.make_async_copy(bwo_hbm, bwo_ref, misc_sem.at[2])

        def wo_copy(g):
            rows = pl.ds(pl.multiple_of(g * PW, PW), PW)
            return pltpu.make_async_copy(wo_hbm.at[rows, :], wo_ref.at[rows, :], wo_sem.at[g])

        xp_copy.start()
        for cp in stage_copies(0):
            cp.start()

        eh = _iota((HB, D), 0) * DB
        ec = _iota((HB, D), 1)
        phi_flat = None
        for d in range(DB):
            t = _dot(phi_ref[d], jnp.where(ec == eh + d, 1.0, 0.0).astype(BF16))
            phi_flat = t if phi_flat is None else phi_flat + t
        nf = _iota((FR, DB), 0) >> LOG_HG
        sel = jnp.where(nf - DB * _div20(nf) == _iota((FR, DB), 1), 1.0, 0.0)
        phi_rows_ref[...] = _dot(sel.astype(BF16), phi_flat.astype(BF16))

        xp_copy.wait()
        for g in range(1, NBUF):
            for cp in stage_copies(g):
                cp.start()
        hp_ref[...] = _layernorm(
            xp_ref[...].astype(F32).reshape(NPRE * PRE, D)).astype(BF16)

        def load_body(g, carry):
            slot = g % NBUF
            for cp in stage_copies(g):
                cp.wait()
            pre_ref[g] = _dot_nt(hp_ref[...], stage_ref[slot])
            w_ref[g] = pltpu.bitcast(stage_ref[slot].T, jnp.uint32)
            rows = pl.ds(pl.multiple_of(g * XC, XC), XC)
            x_ref[rows, :] = xin_ref[slot].astype(F32).reshape(XC, D)

            @pl.when(g + NBUF < G)
            def _():
                for cp in stage_copies(g + NBUF):
                    cp.start()
                wo_copy(g).start()

            @pl.when(g + NBUF == G)
            def _():
                for k in range(G - NBUF, G):
                    wo_copy(k).start()

            return carry

        lax.fori_loop(0, G, load_body, 0)
        bw_copy.start()
        bwo_copy.start()

        def layer_a(start, stop, pre, unroll, lag):
            row = _iota((L, 2 * L), 0)
            col = _iota((L, 2 * L), 1)
            first = col < L
            visible = (row < M) | (row >= jnp.where(first, col, col - L))
            low = _iota((L, LANES), 1) < DH - LANES
            zero = jnp.zeros((L, LANES), F32)

            def block_diag(t):
                t0, t1, t2 = t[:, :LANES], t[:, LANES:2 * LANES], t[:, 2 * LANES:]
                top = jnp.concatenate([t0, jnp.where(low, t1, 0.0), zero], axis=1)
                bot = jnp.concatenate([zero, jnp.where(low, 0.0, t1), t2], axis=1)
                return jnp.concatenate([top, bot], axis=0).astype(BF16)

            def step(s, h):
                rows = seg_rows(s)
                chained = h is not None
                if not chained:
                    h = h_ref[...]
                if pre:
                    h = h[:L - PRE].astype(BF16)
                st = {}
                acc = [None]

                def project(g):
                    w = pltpu.bitcast(w_ref[g], BF16)
                    if g == 0 and chained:
                        qkv = functools.reduce(jnp.add, [
                            _dot(h[:, k:k + LANES], w[k:k + LANES])
                            for k in range(0, D, LANES)])
                    else:
                        qkv = _dot(h, w)
                    if pre:
                        qkv = jnp.concatenate(
                            [qkv, pre_ref[g, pl.ds(pl.multiple_of(s * PRE, PRE), PRE), :]],
                            axis=0)
                    st[g] = [qkv[:, :PW], block_diag(qkv[:, PW:2 * PW]),
                             block_diag(qkv[:, 2 * PW:])]

                def attend(g):
                    sc = jnp.where(visible, _dot_nt(st[g][0], st[g][1]) * scale, -1e9)
                    m0 = jnp.max(jnp.where(first, sc, -jnp.inf), axis=1, keepdims=True)
                    m1 = jnp.max(jnp.where(first, -jnp.inf, sc), axis=1, keepdims=True)
                    e = jnp.exp(sc - jnp.where(first, m0, m1))
                    s0 = jnp.sum(jnp.where(first, e, 0.0), axis=1, keepdims=True)
                    s1 = jnp.sum(jnp.where(first, 0.0, e), axis=1, keepdims=True)
                    st[g][0] = e / jnp.where(first, s0, s1)

                def mix(g):
                    st[g] = _dot(st[g][0], st[g][2])

                def out_proj(g0, g1):
                    o = jnp.concatenate([st[g] for g in range(g0, g1)], axis=1)
                    r = _dot(o, wo_ref[g0 * PW:g1 * PW, :])
                    acc[0] = r if acc[0] is None else acc[0] + r

                done = 0
                for i in range(G + 2):
                    if i < G:
                        project(i)
                    while done < (i - lag if i < G else G - 4 * (G + 2 - i)):
                        out_proj(done, done + 1)
                        done += 1
                    if 0 <= i - 1 < G:
                        attend(i - 1)
                    if 0 <= i - 2 < G:
                        mix(i - 2)
                    if i == 1:
                        normalise_output(jnp.maximum(s - 1, 0))
                    if i == 3:
                        xn_next = _layernorm(
                            x_ref[seg_rows(jnp.minimum(s + 1, NSEG - 1)), :])
                o = jnp.concatenate([st[g] for g in range(G - 4, G)], axis=1)
                y = jnp.concatenate([
                    acc[0][:, c:c + LANES]
                    + _dot(o, wo_ref[(G - 4) * PW:G * PW, c:c + LANES])
                    for c in range(0, D, LANES)], axis=1)
                x_ref[rows, :] = x_ref[rows, :] + y[M:L]
                return jnp.concatenate([y[0:M], xn_next], axis=0)

            def steps(i, carry):
                h = None
                for u in range(unroll):
                    h = step(i * unroll + u, h)
                h_ref[...] = h
                return carry

            lax.fori_loop(start // unroll, stop // unroll, steps, 0)

        def seg_rows(s):
            return pl.ds(s * SEG if isinstance(s, int) else pl.multiple_of(s * SEG, SEG), SEG)

        def normalise_output(s):
            xb_ref[seg_rows(s), :] = _layernorm(x_ref[seg_rows(s), :]).astype(BF16)

        def reset_memory():
            h_ref[0:M, :] = mem_ref[...].astype(F32)
            h_ref[M:L, :] = _layernorm(x_ref[0:SEG, :])

        def fold_hedgehog_weights():
            bw_copy.wait()
            bwo_copy.wait()
            bt_ref[2] = bw_ref[:, 2 * D:3 * D].T
            for r0 in range(0, D, FR):
                c0 = r0 // LANES * LANES
                c1 = pl.cdiv(r0 + FR, LANES) * LANES
                n = _iota((FR, c1 - c0), 0) + r0
                c = _iota((FR, c1 - c0), 1) + c0
                grp = _div20(n >> LOG_HG)
                head = (grp << LOG_HG) + (n & (HG - 1))
                fold = jnp.where(_div20(c) == head, phi_rows_ref[:, c0:c1], 0.0).astype(BF16)
                for j in range(2):
                    bt_ref[j, r0:r0 + FR, :] = _dot_nt(
                        fold, bw_ref[:, j * D + c0:j * D + c1]).astype(BF16)

        def over_features(op, p):
            r = p[0:SUB]
            for i in range(1, GR // SUB):
                r = op(r, p[i * SUB:(i + 1) * SUB])
            shift = SUB // 2
            while shift >= HG:
                r = op(r, pltpu.roll(r, shift, 0))
                shift //= 2
            return r

        def spread(r):
            return jnp.concatenate([r] * (GR // SUB), axis=0)

        def features(p):
            ep = jnp.exp(p - spread(over_features(jnp.maximum, p)))
            en = jnp.exp(spread(over_features(jnp.minimum, p)) - p)
            fp = ep * spread(1.0 / over_features(jnp.add, ep))
            fn = en * spread(1.0 / over_features(jnp.add, en))
            return jnp.concatenate([fp, fn], axis=0).astype(BF16)

        def out_copy(c):
            rows = pl.ds(pl.multiple_of(c * TB, TB), TB)
            return pltpu.make_async_copy(xb_ref.at[rows, :], out_hbm.at[rows, :], out_sem.at[c])

        def layer_b(last):
            kv_ref[...] = jnp.zeros(kv_ref.shape, F32)

            def keys(c, carry):
                rows = pl.ds(pl.multiple_of(c * TB, TB), TB)
                pk = _dot_nt(bt_ref[1], xb_ref[rows, :])
                v = _dot_nt(bt_ref[2], xb_ref[rows, :])
                ones = jnp.ones((SUB, TB), F32)
                for j in range(NG):
                    vj = jnp.concatenate([v[j * GR:(j + 1) * GR], ones], axis=0)
                    kv_ref[j] += _dot_nt(vj, features(pk[j * GR:(j + 1) * GR]))
                return carry

            lax.fori_loop(0, NCH, keys, 0)

            shape = (GR + SUB, 2 * GR)
            r = _iota(shape, 0)
            second = ((r >= DB) & (r < GR)) | (r >= GR + SUB // 2)
            same_head = second.astype(jnp.int32) == (_iota(shape, 1) & 1)
            for j in range(NG):
                kv_ref[j] = jnp.where(same_head, kv_ref[j], 0.0)

            def queries(c, carry):
                rows = pl.ds(pl.multiple_of(c * TB, TB), TB)
                pq = _dot_nt(bt_ref[0], xb_ref[rows, :])
                top = _iota((SUB, TB), 0) < SUB // 2
                o = []
                for j in range(NG):
                    nd = _dot(kv_ref[j], features(pq[j * GR:(j + 1) * GR]))
                    inv = 1.0 / (nd[GR:] + 1e-6)
                    swapped = pltpu.roll(inv, SUB // 2, 0)
                    inv0, inv1 = jnp.where(top, inv, swapped), jnp.where(top, swapped, inv)
                    o.append(nd[:GR] * jnp.concatenate([inv0, inv0, inv, inv1, inv1], axis=0))
                o = jnp.concatenate(o, axis=0).astype(BF16).T
                x = x_ref[rows, :] + _dot(o, bwo_ref[...])
                x_ref[rows, :] = x
                xb_ref[rows, :] = x.astype(BF16)

                @pl.when(last)
                def _():
                    out_copy(c).start()

                return carry

            lax.fori_loop(0, NCH, queries, 0)

        def layer(i, carry):
            layer_a(jnp.where(i == 0, NPRE, 0), NSEG, pre=False, unroll=UNROLL, lag=99)
            normalise_output(NSEG - 1)
            layer_b(i == 1)
            reset_memory()
            return carry

        reset_memory()
        for g in range(G):
            wo_copy(g).wait()
        layer_a(0, NPRE, pre=True, unroll=UNROLL_PRE, lag=9)
        fold_hedgehog_weights()
        lax.fori_loop(0, 2, layer, 0)
        for c in range(NCH):
            out_copy(c).wait()

    scratch = [
        pltpu.VMEM((G, D // 2, 3 * PW), jnp.uint32),
        pltpu.VMEM((H * DH, D), BF16),
        pltpu.VMEM((NBUF, 3 * PW, D), BF16),
        pltpu.VMEM((NBUF, XC // SEG, SEG, D), BF16),
        pltpu.VMEM((NPRE, PRE, D), BF16),
        pltpu.VMEM((NPRE * PRE, D), BF16),
        pltpu.VMEM((G, NPRE * PRE, 3 * PW), F32),
        pltpu.VMEM((S, D), BF16),
        pltpu.VMEM((S, D), F32),
        pltpu.VMEM((L, D), F32),
        pltpu.VMEM((D, 3 * D), BF16),
        pltpu.VMEM((FR, D), F32),
        pltpu.VMEM((3, D, D), BF16),
        pltpu.VMEM((D, D), BF16),
        pltpu.VMEM((NG, GR + SUB, 2 * GR), F32),
        pltpu.SemaphoreType.DMA((NBUF, 4)),
        pltpu.SemaphoreType.DMA((G,)),
        pltpu.SemaphoreType.DMA((3,)),
        pltpu.SemaphoreType.DMA((NCH,)),
    ]
    return kernel, scratch


@functools.partial(jax.jit, static_argnames=("A_seg_len",))
def pallas_interleave_layers__memory_aug_recurrent_mem_tr__linear_kernel_hedgehog__prompt_kernel(
    A_x: jax.Array,
    A_mem0: jax.Array,
    A_Wq: jax.Array,
    A_Wk: jax.Array,
    A_Wv: jax.Array,
    A_Wo: jax.Array,
    A_seg_len: int,
    B_x: jax.Array,
    B_wqkv: jax.Array,
    B_w_phi: jax.Array,
    B_wo: jax.Array,
):
    del B_x
    B, S, D = A_x.shape
    M = A_mem0.shape[1]
    _, H, DH = A_Wq.shape
    HB = B_w_phi.shape[0]
    assert B == 1

    kernel, scratch = _make_kernel(S, D, H, DH, M, A_seg_len, HB,
                                   HG=2, TB=512, NBUF=4, NPRE=44, UNROLL=2, UNROLL_PRE=2)

    def head_major(w):
        return w.transpose(1, 2, 0).reshape(H * DH, D)

    hbm = pl.BlockSpec(memory_space=pltpu.HBM)
    vmem = pl.BlockSpec(memory_space=pltpu.VMEM)
    out = pl.pallas_call(
        kernel,
        out_shape=jax.ShapeDtypeStruct((S, D), A_x.dtype),
        in_specs=[hbm, vmem, hbm, hbm, hbm, hbm, hbm, vmem, hbm],
        out_specs=hbm,
        scratch_shapes=scratch,
        compiler_params=pltpu.CompilerParams(vmem_limit_bytes=110 * 1024 * 1024,
                                             disable_bounds_checks=True),
    )(
        A_x.reshape(S // A_seg_len, A_seg_len, D), A_mem0.reshape(M, D),
        head_major(A_Wq), head_major(A_Wk), head_major(A_Wv), A_Wo.reshape(H * DH, D),
        B_wqkv, B_w_phi.transpose(1, 2, 0), B_wo,
    )
    return out.reshape(B, S, D)
```

```python
import functools

import jax
import jax.numpy as jnp
from jax import lax
import jax.experimental.pallas as pl
import jax.experimental.pallas.tpu as pltpu

F32 = jnp.float32
BF16 = jnp.bfloat16
LANES = 128
SUB = 8


def _dot(a, b):
    return lax.dot_general(a, b, (((1,), (0,)), ((), ())), preferred_element_type=F32)


def _dot_nt(a, b):
    return lax.dot_general(a, b, (((1,), (1,)), ((), ())), preferred_element_type=F32)


def _layernorm_parts(x):
    inv_n = 1.0 / x.shape[-1]
    c = x - jnp.sum(x, axis=-1, keepdims=True) * inv_n
    var = jnp.sum(c * c, axis=-1, keepdims=True) * inv_n
    return c, lax.rsqrt(var + 1e-5)


def _layernorm(x):
    c, inv_std = _layernorm_parts(x)
    return c * inv_std


def _iota(shape, dim):
    return lax.broadcasted_iota(jnp.int32, shape, dim)


def _div20(n):
    return (n * 3277) >> 16


def _make_kernel(S, D, H, DH, M, SEG, HB, *, HG, TB, NBUF, NPRE, UNROLL, UNROLL_PRE):
    L = M + SEG
    G = H // 2
    PW = 2 * DH
    NSEG = S // SEG
    XC = S // G
    PRE = SUB
    DB = D // HB
    NG = HB // HG
    GR = DB * HG
    FR = 4 * DB
    LOG_HG = HG.bit_length() - 1
    NCH = S // TB
    scale = DH ** -0.5
    assert PW == 3 * LANES and 2 * L <= LANES and DB == 20 and D < 1024
    assert L % SUB == 0 and M % SUB == 0 and GR % SUB == 0 and HG == 2
    assert S % TB == 0 and S % G == 0 and NPRE <= NSEG and NBUF < G and G >= 14
    assert NSEG % UNROLL == 0 and NPRE % UNROLL == 0 and NPRE % UNROLL_PRE == 0

    def kernel(x_hbm, mem_ref, wq_hbm, wk_hbm, wv_hbm, wo_hbm, bw_hbm, phi_ref, bwo_hbm,
               out_hbm,
               w_ref, wo_ref, stage_ref, xin_ref, xp_ref, hp_ref, pre_ref,
               xb_ref, x_ref, h_ref,
               bw_ref, phi_rows_ref, bt_ref, bwo_ref, kv_ref,
               stage_sem, wo_sem, misc_sem, out_sem):

        def stage_copies(g):
            slot = g % NBUF
            rows = pl.ds(pl.multiple_of(g * PW, PW), PW)
            copies = [
                pltpu.make_async_copy(src.at[rows, :],
                                      stage_ref.at[slot, pl.ds(j * PW, PW), :],
                                      stage_sem.at[slot, j])
                for j, src in enumerate((wq_hbm, wk_hbm, wv_hbm))]
            copies.append(pltpu.make_async_copy(
                x_hbm.at[pl.ds(g * (XC // SEG), XC // SEG)], xin_ref.at[slot],
                stage_sem.at[slot, 3]))
            return copies

        xp_copy = pltpu.make_async_copy(
            x_hbm.at[pl.ds(0, NPRE), pl.ds(SEG - PRE, PRE), :], xp_ref, misc_sem.at[0])
        bw_copy = pltpu.make_async_copy(bw_hbm, bw_ref, misc_sem.at[1])
        bwo_copy = pltpu.make_async_copy(bwo_hbm, bwo_ref, misc_sem.at[2])

        def wo_copy(g):
            rows = pl.ds(pl.multiple_of(g * PW, PW), PW)
            return pltpu.make_async_copy(wo_hbm.at[rows, :], wo_ref.at[rows, :], wo_sem.at[g])

        xp_copy.start()
        for cp in stage_copies(0):
            cp.start()

        eh = _iota((HB, D), 0) * DB
        ec = _iota((HB, D), 1)
        phi_flat = None
        for d in range(DB):
            t = _dot(phi_ref[d], jnp.where(ec == eh + d, 1.0, 0.0).astype(BF16))
            phi_flat = t if phi_flat is None else phi_flat + t
        nf = _iota((FR, DB), 0) >> LOG_HG
        sel = jnp.where(nf - DB * _div20(nf) == _iota((FR, DB), 1), 1.0, 0.0)
        phi_rows_ref[...] = _dot(sel.astype(BF16), phi_flat.astype(BF16))

        xp_copy.wait()
        for g in range(1, NBUF):
            for cp in stage_copies(g):
                cp.start()
        hp_ref[...] = _layernorm(
            xp_ref[...].astype(F32).reshape(NPRE * PRE, D)).astype(BF16)

        def load_body(g, carry):
            slot = g % NBUF
            for cp in stage_copies(g):
                cp.wait()
            pre_ref[g] = _dot_nt(hp_ref[...], stage_ref[slot])
            w_ref[g] = pltpu.bitcast(stage_ref[slot].T, jnp.uint32)
            rows = pl.ds(pl.multiple_of(g * XC, XC), XC)
            x_ref[rows, :] = xin_ref[slot].astype(F32).reshape(XC, D)

            @pl.when(g + NBUF < G)
            def _():
                for cp in stage_copies(g + NBUF):
                    cp.start()
                wo_copy(g).start()

            @pl.when(g + NBUF == G)
            def _():
                for k in range(G - NBUF, G):
                    wo_copy(k).start()

            return carry

        lax.fori_loop(0, G, load_body, 0)
        bw_copy.start()
        bwo_copy.start()

        def layer_a(start, stop, pre, unroll, lag):
            row = _iota((L, 2 * L), 0)
            col = _iota((L, 2 * L), 1)
            first = col < L
            visible = (row < M) | (row >= jnp.where(first, col, col - L))
            low = _iota((L, LANES), 1) < DH - LANES
            zero = jnp.zeros((L, LANES), F32)

            def block_diag(t):
                t0, t1, t2 = t[:, :LANES], t[:, LANES:2 * LANES], t[:, 2 * LANES:]
                top = jnp.concatenate([t0, jnp.where(low, t1, 0.0), zero], axis=1)
                bot = jnp.concatenate([zero, jnp.where(low, 0.0, t1), t2], axis=1)
                return jnp.concatenate([top, bot], axis=0).astype(BF16)

            def step(s, h):
                rows = seg_rows(s)
                chained = h is not None
                if not chained:
                    h = h_ref[...]
                if pre:
                    h = h[:L - PRE].astype(BF16)
                st = {}
                acc = [None]

                def project(g):
                    w = pltpu.bitcast(w_ref[g], BF16)
                    if g == 0 and chained:
                        qkv = functools.reduce(jnp.add, [
                            _dot(h[:, k:k + LANES], w[k:k + LANES])
                            for k in range(0, D, LANES)])
                    else:
                        qkv = _dot(h, w)
                    if pre:
                        qkv = jnp.concatenate(
                            [qkv, pre_ref[g, pl.ds(pl.multiple_of(s * PRE, PRE), PRE), :]],
                            axis=0)
                    st[g] = [qkv[:, :PW], block_diag(qkv[:, PW:2 * PW]),
                             block_diag(qkv[:, 2 * PW:])]

                def attend(g, after):
                    fill = -1e9
                    if after is not None:
                        fill = jnp.concatenate(
                            [jnp.full((M, 1), fill, F32), jnp.minimum(after, fill)], axis=0)
                    sc = jnp.where(visible, _dot_nt(st[g][0], st[g][1]) * scale, fill)
                    m0 = jnp.max(jnp.where(first, sc, -jnp.inf), axis=1, keepdims=True)
                    m1 = jnp.max(jnp.where(first, -jnp.inf, sc), axis=1, keepdims=True)
                    e = jnp.exp(sc - jnp.where(first, m0, m1))
                    s0 = jnp.sum(jnp.where(first, e, 0.0), axis=1, keepdims=True)
                    s1 = jnp.sum(jnp.where(first, 0.0, e), axis=1, keepdims=True)
                    st[g][0] = e / jnp.where(first, s0, s1)

                def mix(g):
                    st[g] = _dot(st[g][0], st[g][2])

                def out_proj(g0, g1):
                    o = jnp.concatenate([st[g] for g in range(g0, g1)], axis=1)
                    r = _dot(o, wo_ref[g0 * PW:g1 * PW, :])
                    acc[0] = r if acc[0] is None else acc[0] + r

                done = 0
                for i in range(G + 2):
                    if i < G:
                        project(i)
                    while done < (i - lag if i < G else G - 4 * (G + 2 - i)):
                        out_proj(done, done + 1)
                        done += 1
                    after = None
                    if i == 3:
                        prev = seg_rows(jnp.maximum(s - 1, 0))
                        c, after = _layernorm_parts(x_ref[prev, :])
                        xb_ref[prev, :] = (c * after).astype(BF16)
                    if i == 6:
                        c, after = _layernorm_parts(
                            x_ref[seg_rows(jnp.minimum(s + 1, NSEG - 1)), :])
                        xn_next = c * after
                    if 0 <= i - 1 < G:
                        attend(i - 1, None if pre else after)
                    if 0 <= i - 2 < G:
                        mix(i - 2)
                o = jnp.concatenate([st[g] for g in range(G - 4, G)], axis=1)
                y = jnp.concatenate([
                    acc[0][:, c:c + LANES]
                    + _dot(o, wo_ref[(G - 4) * PW:G * PW, c:c + LANES])
                    for c in range(0, D, LANES)], axis=1)
                x_ref[rows, :] = x_ref[rows, :] + y[M:L]
                return jnp.concatenate([y[0:M], xn_next], axis=0)

            def steps(i, carry):
                h = None
                for u in range(unroll):
                    h = step(i * unroll + u, h)
                h_ref[...] = h
                return carry

            lax.fori_loop(start // unroll, stop // unroll, steps, 0)

        def seg_rows(s):
            return pl.ds(s * SEG if isinstance(s, int) else pl.multiple_of(s * SEG, SEG), SEG)

        def normalise_output(s):
            xb_ref[seg_rows(s), :] = _layernorm(x_ref[seg_rows(s), :]).astype(BF16)

        def reset_memory():
            h_ref[0:M, :] = mem_ref[...].astype(F32)
            h_ref[M:L, :] = _layernorm(x_ref[0:SEG, :])

        def fold_hedgehog_weights():
            bw_copy.wait()
            bwo_copy.wait()
            bt_ref[2] = bw_ref[:, 2 * D:3 * D].T
            for r0 in range(0, D, FR):
                c0 = r0 // LANES * LANES
                c1 = pl.cdiv(r0 + FR, LANES) * LANES
                n = _iota((FR, c1 - c0), 0) + r0
                c = _iota((FR, c1 - c0), 1) + c0
                grp = _div20(n >> LOG_HG)
                head = (grp << LOG_HG) + (n & (HG - 1))
                fold = jnp.where(_div20(c) == head, phi_rows_ref[:, c0:c1], 0.0).astype(BF16)
                for j in range(2):
                    bt_ref[j, r0:r0 + FR, :] = _dot_nt(
                        fold, bw_ref[:, j * D + c0:j * D + c1]).astype(BF16)

        def over_features(op, p):
            r = p[0:SUB]
            for i in range(1, GR // SUB):
                r = op(r, p[i * SUB:(i + 1) * SUB])
            shift = SUB // 2
            while shift >= HG:
                r = op(r, pltpu.roll(r, shift, 0))
                shift //= 2
            return r

        def spread(r):
            return jnp.concatenate([r] * (GR // SUB), axis=0)

        def features(p):
            ep = jnp.exp(p - spread(over_features(jnp.maximum, p)))
            en = jnp.exp(spread(over_features(jnp.minimum, p)) - p)
            fp = ep * spread(1.0 / over_features(jnp.add, ep))
            fn = en * spread(1.0 / over_features(jnp.add, en))
            return jnp.concatenate([fp, fn], axis=0).astype(BF16)

        def out_copy(c):
            rows = pl.ds(pl.multiple_of(c * TB, TB), TB)
            return pltpu.make_async_copy(xb_ref.at[rows, :], out_hbm.at[rows, :], out_sem.at[c])

        def layer_b(last):
            kv_ref[...] = jnp.zeros(kv_ref.shape, F32)

            def keys(c, carry):
                rows = pl.ds(pl.multiple_of(c * TB, TB), TB)
                pk = _dot_nt(bt_ref[1], xb_ref[rows, :])
                v = _dot_nt(bt_ref[2], xb_ref[rows, :])
                ones = jnp.ones((SUB, TB), F32)
                for j in range(NG):
                    vj = jnp.concatenate([v[j * GR:(j + 1) * GR], ones], axis=0)
                    kv_ref[j] += _dot_nt(vj, features(pk[j * GR:(j + 1) * GR]))
                return carry

            lax.fori_loop(0, NCH, keys, 0)

            shape = (GR + SUB, 2 * GR)
            r = _iota(shape, 0)
            second = ((r >= DB) & (r < GR)) | (r >= GR + SUB // 2)
            same_head = second.astype(jnp.int32) == (_iota(shape, 1) & 1)
            for j in range(NG):
                kv_ref[j] = jnp.where(same_head, kv_ref[j], 0.0)

            def queries(c, carry):
                rows = pl.ds(pl.multiple_of(c * TB, TB), TB)
                pq = _dot_nt(bt_ref[0], xb_ref[rows, :])
                top = _iota((SUB, TB), 0) < SUB // 2
                o = []
                for j in range(NG):
                    nd = _dot(kv_ref[j], features(pq[j * GR:(j + 1) * GR]))
                    inv = 1.0 / (nd[GR:] + 1e-6)
                    swapped = pltpu.roll(inv, SUB // 2, 0)
                    inv0, inv1 = jnp.where(top, inv, swapped), jnp.where(top, swapped, inv)
                    o.append(nd[:GR] * jnp.concatenate([inv0, inv0, inv, inv1, inv1], axis=0))
                o = jnp.concatenate(o, axis=0).astype(BF16).T
                x = x_ref[rows, :] + _dot(o, bwo_ref[...])
                if last:
                    xb_ref[rows, :] = x.astype(BF16)
                    out_copy(c).start()
                else:
                    x_ref[rows, :] = x
                return carry

            lax.fori_loop(0, NCH, queries, 0)

        reset_memory()
        for g in range(G):
            wo_copy(g).wait()
        layer_a(0, NPRE, pre=True, unroll=UNROLL_PRE, lag=9)
        fold_hedgehog_weights()
        layer_a(NPRE, NSEG, pre=False, unroll=UNROLL_PRE, lag=99)
        normalise_output(NSEG - 1)
        layer_b(last=False)
        reset_memory()
        layer_a(0, NSEG, pre=False, unroll=UNROLL, lag=99)
        normalise_output(NSEG - 1)
        layer_b(last=True)
        for c in range(NCH):
            out_copy(c).wait()

    scratch = [
        pltpu.VMEM((G, D // 2, 3 * PW), jnp.uint32),
        pltpu.VMEM((H * DH, D), BF16),
        pltpu.VMEM((NBUF, 3 * PW, D), BF16),
        pltpu.VMEM((NBUF, XC // SEG, SEG, D), BF16),
        pltpu.VMEM((NPRE, PRE, D), BF16),
        pltpu.VMEM((NPRE * PRE, D), BF16),
        pltpu.VMEM((G, NPRE * PRE, 3 * PW), F32),
        pltpu.VMEM((S, D), BF16),
        pltpu.VMEM((S, D), F32),
        pltpu.VMEM((L, D), F32),
        pltpu.VMEM((D, 3 * D), BF16),
        pltpu.VMEM((FR, D), F32),
        pltpu.VMEM((3, D, D), BF16),
        pltpu.VMEM((D, D), BF16),
        pltpu.VMEM((NG, GR + SUB, 2 * GR), F32),
        pltpu.SemaphoreType.DMA((NBUF, 4)),
        pltpu.SemaphoreType.DMA((G,)),
        pltpu.SemaphoreType.DMA((3,)),
        pltpu.SemaphoreType.DMA((NCH,)),
    ]
    return kernel, scratch


@functools.partial(jax.jit, static_argnames=("A_seg_len",))
def pallas_interleave_layers__memory_aug_recurrent_mem_tr__linear_kernel_hedgehog__prompt_kernel(
    A_x: jax.Array,
    A_mem0: jax.Array,
    A_Wq: jax.Array,
    A_Wk: jax.Array,
    A_Wv: jax.Array,
    A_Wo: jax.Array,
    A_seg_len: int,
    B_x: jax.Array,
    B_wqkv: jax.Array,
    B_w_phi: jax.Array,
    B_wo: jax.Array,
):
    del B_x
    B, S, D = A_x.shape
    M = A_mem0.shape[1]
    _, H, DH = A_Wq.shape
    HB = B_w_phi.shape[0]
    assert B == 1

    kernel, scratch = _make_kernel(S, D, H, DH, M, A_seg_len, HB,
                                   HG=2, TB=512, NBUF=4, NPRE=44, UNROLL=4, UNROLL_PRE=2)

    def head_major(w):
        return w.transpose(1, 2, 0).reshape(H * DH, D)

    hbm = pl.BlockSpec(memory_space=pltpu.HBM)
    vmem = pl.BlockSpec(memory_space=pltpu.VMEM)
    out = pl.pallas_call(
        kernel,
        out_shape=jax.ShapeDtypeStruct((S, D), A_x.dtype),
        in_specs=[hbm, vmem, hbm, hbm, hbm, hbm, hbm, vmem, hbm],
        out_specs=hbm,
        scratch_shapes=scratch,
        compiler_params=pltpu.CompilerParams(vmem_limit_bytes=110 * 1024 * 1024,
                                             disable_bounds_checks=True),
    )(
        A_x.reshape(S // A_seg_len, A_seg_len, D), A_mem0.reshape(M, D),
        head_major(A_Wq), head_major(A_Wk), head_major(A_Wv), A_Wo.reshape(H * DH, D),
        B_wqkv, B_w_phi.transpose(1, 2, 0), B_wo,
    )
    return out.reshape(B, S, D)
```

```python
import functools

import jax
import jax.numpy as jnp
from jax import lax
import jax.experimental.pallas as pl
import jax.experimental.pallas.tpu as pltpu

F32 = jnp.float32
BF16 = jnp.bfloat16
LANES = 128
SUB = 8


def _dot(a, b):
    return lax.dot_general(a, b, (((1,), (0,)), ((), ())), preferred_element_type=F32)


def _dot_nt(a, b):
    return lax.dot_general(a, b, (((1,), (1,)), ((), ())), preferred_element_type=F32)


def _layernorm_parts(x):
    inv_n = 1.0 / x.shape[-1]
    c = x - jnp.sum(x, axis=-1, keepdims=True) * inv_n
    var = jnp.sum(c * c, axis=-1, keepdims=True) * inv_n
    return c, lax.rsqrt(var + 1e-5)


def _layernorm(x):
    c, inv_std = _layernorm_parts(x)
    return c * inv_std


def _iota(shape, dim):
    return lax.broadcasted_iota(jnp.int32, shape, dim)


def _div20(n):
    return (n * 3277) >> 16


def _make_kernel(S, D, H, DH, M, SEG, HB, *, HG, TB, NBUF, UNROLL):
    L = M + SEG
    G = H // 2
    PW = 2 * DH
    NSEG = S // SEG
    XC = S // G
    PRE = SUB
    DB = D // HB
    NG = HB // HG
    GR = DB * HG
    FR = 4 * DB
    LOG_HG = HG.bit_length() - 1
    NCH = S // TB
    scale = DH ** -0.5
    assert PW == 3 * LANES and 2 * L <= LANES and DB == 20 and D < 1024
    assert L % SUB == 0 and M % SUB == 0 and GR % SUB == 0 and HG == 2
    assert S % TB == 0 and S % G == 0 and NBUF < G and G >= 14
    assert NSEG % UNROLL == 0

    def kernel(x_hbm, mem_ref, wq_hbm, wk_hbm, wv_hbm, wo_hbm, bw_hbm, phi_ref, bwo_hbm,
               out_hbm,
               w_ref, wo_ref, stage_ref, xin_ref, xp_ref, hp_ref, pre_ref,
               xb_ref, x_ref, h_ref,
               bw_ref, phi_rows_ref, bt_ref, bwo_ref, kv_ref,
               stage_sem, wo_sem, misc_sem, out_sem):

        def stage_copies(g):
            slot = g % NBUF
            rows = pl.ds(pl.multiple_of(g * PW, PW), PW)
            copies = [
                pltpu.make_async_copy(src.at[rows, :],
                                      stage_ref.at[slot, pl.ds(j * PW, PW), :],
                                      stage_sem.at[slot, j])
                for j, src in enumerate((wq_hbm, wk_hbm, wv_hbm))]
            copies.append(pltpu.make_async_copy(
                x_hbm.at[pl.ds(g * (XC // SEG), XC // SEG)], xin_ref.at[slot],
                stage_sem.at[slot, 3]))
            return copies

        xp_copy = pltpu.make_async_copy(
            x_hbm.at[:, pl.ds(SEG - PRE, PRE), :], xp_ref, misc_sem.at[0])
        bw_copy = pltpu.make_async_copy(bw_hbm, bw_ref, misc_sem.at[1])
        bwo_copy = pltpu.make_async_copy(bwo_hbm, bwo_ref, misc_sem.at[2])

        def wo_copy(g):
            rows = pl.ds(pl.multiple_of(g * PW, PW), PW)
            return pltpu.make_async_copy(wo_hbm.at[rows, :], wo_ref.at[rows, :], wo_sem.at[g])

        xp_copy.start()
        for cp in stage_copies(0):
            cp.start()

        eh = _iota((HB, D), 0) * DB
        ec = _iota((HB, D), 1)
        phi_flat = None
        for d in range(DB):
            t = _dot(phi_ref[d], jnp.where(ec == eh + d, 1.0, 0.0).astype(BF16))
            phi_flat = t if phi_flat is None else phi_flat + t
        nf = _iota((FR, DB), 0) >> LOG_HG
        sel = jnp.where(nf - DB * _div20(nf) == _iota((FR, DB), 1), 1.0, 0.0)
        phi_rows_ref[...] = _dot(sel.astype(BF16), phi_flat.astype(BF16))

        xp_copy.wait()
        for g in range(1, NBUF):
            for cp in stage_copies(g):
                cp.start()
        hp_ref[...] = _layernorm(
            xp_ref[...].astype(F32).reshape(NSEG * PRE, D)).astype(BF16)

        def load_body(g, carry):
            slot = g % NBUF
            for cp in stage_copies(g):
                cp.wait()
            pre_ref[g] = _dot_nt(hp_ref[...], stage_ref[slot, PW:, :])
            w_ref[g] = pltpu.bitcast(stage_ref[slot].T, jnp.uint32)
            rows = pl.ds(pl.multiple_of(g * XC, XC), XC)
            x_ref[rows, :] = xin_ref[slot].astype(F32).reshape(XC, D)

            @pl.when(g + NBUF < G)
            def _():
                for cp in stage_copies(g + NBUF):
                    cp.start()
                wo_copy(g).start()

            @pl.when(g + NBUF == G)
            def _():
                for k in range(G - NBUF, G):
                    wo_copy(k).start()

            return carry

        lax.fori_loop(0, G, load_body, 0)
        bw_copy.start()
        bwo_copy.start()

        def layer_a(start, stop, pre, unroll, lag):
            row = _iota((L, 2 * L), 0)
            col = _iota((L, 2 * L), 1)
            first = col < L
            visible = (row < M) | (row >= jnp.where(first, col, col - L))
            low = _iota((L, LANES), 1) < DH - LANES
            zero = jnp.zeros((L, LANES), F32)

            def block_diag(t):
                t0, t1, t2 = t[:, :LANES], t[:, LANES:2 * LANES], t[:, 2 * LANES:]
                top = jnp.concatenate([t0, jnp.where(low, t1, 0.0), zero], axis=1)
                bot = jnp.concatenate([zero, jnp.where(low, 0.0, t1), t2], axis=1)
                return jnp.concatenate([top, bot], axis=0).astype(BF16)

            def step(s, h):
                rows = seg_rows(s)
                chained = h is not None
                if not chained:
                    h = h_ref[...]
                h_kv = h[:L - PRE].astype(BF16) if pre else h
                st = {}
                acc = [None]

                def project(g):
                    def times(c0, c1):
                        return [
                            _dot(lhs[:, c0:c1], pltpu.bitcast(
                                w_ref[g, c0 // 2:c1 // 2, j * PW:(j + 1) * PW], BF16))
                            for lhs, j in ((h_kv, 1), (h, 0), (h_kv, 2))]

                    if g == 0 and chained:
                        parts = [times(c, c + LANES) for c in range(0, D, LANES)]
                        k, q, v = [functools.reduce(jnp.add, t) for t in zip(*parts)]
                    else:
                        k, q, v = times(0, D)
                    if pre:
                        done = pre_ref[g, pl.ds(pl.multiple_of(s * PRE, PRE), PRE), :]
                        k = jnp.concatenate([k, done[:, :PW]], axis=0)
                        v = jnp.concatenate([v, done[:, PW:]], axis=0)
                    st[g] = [q, block_diag(k), block_diag(v)]

                def attend(g, after):
                    fill = -1e9
                    if after is not None:
                        fill = jnp.concatenate(
                            [jnp.full((M, 1), fill, F32), jnp.minimum(after, fill)], axis=0)
                    sc = jnp.where(visible, _dot_nt(st[g][0], st[g][1]) * scale, fill)
                    m0 = jnp.max(jnp.where(first, sc, -jnp.inf), axis=1, keepdims=True)
                    m1 = jnp.max(jnp.where(first, -jnp.inf, sc), axis=1, keepdims=True)
                    e = jnp.exp(sc - jnp.where(first, m0, m1))
                    s0 = jnp.sum(jnp.where(first, e, 0.0), axis=1, keepdims=True)
                    s1 = jnp.sum(jnp.where(first, 0.0, e), axis=1, keepdims=True)
                    st[g][0] = e / jnp.where(first, s0, s1)

                def mix(g):
                    st[g] = _dot(st[g][0], st[g][2])

                def out_proj(g0, g1):
                    o = jnp.concatenate([st[g] for g in range(g0, g1)], axis=1)
                    r = _dot(o, wo_ref[g0 * PW:g1 * PW, :])
                    acc[0] = r if acc[0] is None else acc[0] + r

                done = 0
                for i in range(G + 2):
                    if i < G:
                        project(i)
                    while done < (i - lag if i < G else G - 4 * (G + 2 - i)):
                        out_proj(done, done + 1)
                        done += 1
                    after = None
                    if i == 3:
                        prev = seg_rows(jnp.maximum(s - 1, 0))
                        c, after = _layernorm_parts(x_ref[prev, :])
                        xb_ref[prev, :] = (c * after).astype(BF16)
                    if i == 6:
                        c, after = _layernorm_parts(
                            x_ref[seg_rows(jnp.minimum(s + 1, NSEG - 1)), :])
                        xn_next = c * after
                    if 0 <= i - 1 < G:
                        attend(i - 1, after)
                    if 0 <= i - 2 < G:
                        mix(i - 2)
                o = jnp.concatenate([st[g] for g in range(G - 4, G)], axis=1)
                y = jnp.concatenate([
                    acc[0][:, c:c + LANES]
                    + _dot(o, wo_ref[(G - 4) * PW:G * PW, c:c + LANES])
                    for c in range(0, D, LANES)], axis=1)
                x_ref[rows, :] = x_ref[rows, :] + y[M:L]
                return jnp.concatenate([y[0:M], xn_next], axis=0)

            def steps(i, carry):
                h = None
                for u in range(unroll):
                    h = step(i * unroll + u, h)
                h_ref[...] = h
                return carry

            lax.fori_loop(start // unroll, stop // unroll, steps, 0)

        def seg_rows(s):
            return pl.ds(s * SEG if isinstance(s, int) else pl.multiple_of(s * SEG, SEG), SEG)

        def normalise_output(s):
            xb_ref[seg_rows(s), :] = _layernorm(x_ref[seg_rows(s), :]).astype(BF16)

        def reset_memory():
            h_ref[0:M, :] = mem_ref[...].astype(F32)
            h_ref[M:L, :] = _layernorm(x_ref[0:SEG, :])

        def fold_hedgehog_weights():
            bw_copy.wait()
            bwo_copy.wait()
            bt_ref[2] = bw_ref[:, 2 * D:3 * D].T
            for r0 in range(0, D, FR):
                c0 = r0 // LANES * LANES
                c1 = pl.cdiv(r0 + FR, LANES) * LANES
                n = _iota((FR, c1 - c0), 0) + r0
                c = _iota((FR, c1 - c0), 1) + c0
                grp = _div20(n >> LOG_HG)
                head = (grp << LOG_HG) + (n & (HG - 1))
                fold = jnp.where(_div20(c) == head, phi_rows_ref[:, c0:c1], 0.0).astype(BF16)
                for j in range(2):
                    bt_ref[j, r0:r0 + FR, :] = _dot_nt(
                        fold, bw_ref[:, j * D + c0:j * D + c1]).astype(BF16)

        def over_features(op, p):
            r = p[0:SUB]
            for i in range(1, GR // SUB):
                r = op(r, p[i * SUB:(i + 1) * SUB])
            shift = SUB // 2
            while shift >= HG:
                r = op(r, pltpu.roll(r, shift, 0))
                shift //= 2
            return r

        def spread(r):
            return jnp.concatenate([r] * (GR // SUB), axis=0)

        def features(p):
            ep = jnp.exp(p - spread(over_features(jnp.maximum, p)))
            en = jnp.exp(spread(over_features(jnp.minimum, p)) - p)
            fp = ep * spread(1.0 / over_features(jnp.add, ep))
            fn = en * spread(1.0 / over_features(jnp.add, en))
            return jnp.concatenate([fp, fn], axis=0).astype(BF16)

        def out_copy(c):
            rows = pl.ds(pl.multiple_of(c * TB, TB), TB)
            return pltpu.make_async_copy(xb_ref.at[rows, :], out_hbm.at[rows, :], out_sem.at[c])

        def layer_b(last):
            kv_ref[...] = jnp.zeros(kv_ref.shape, F32)

            def keys(c, carry):
                rows = pl.ds(pl.multiple_of(c * TB, TB), TB)
                pk = _dot_nt(bt_ref[1], xb_ref[rows, :])
                v = _dot_nt(bt_ref[2], xb_ref[rows, :])
                ones = jnp.ones((SUB, TB), F32)
                for j in range(NG):
                    vj = jnp.concatenate([v[j * GR:(j + 1) * GR], ones], axis=0)
                    kv_ref[j] += _dot_nt(vj, features(pk[j * GR:(j + 1) * GR]))
                return carry

            lax.fori_loop(0, NCH, keys, 0)

            shape = (GR + SUB, 2 * GR)
            r = _iota(shape, 0)
            second = ((r >= DB) & (r < GR)) | (r >= GR + SUB // 2)
            same_head = second.astype(jnp.int32) == (_iota(shape, 1) & 1)
            for j in range(NG):
                kv_ref[j] = jnp.where(same_head, kv_ref[j], 0.0)

            def queries(c, carry):
                rows = pl.ds(pl.multiple_of(c * TB, TB), TB)
                pq = _dot_nt(bt_ref[0], xb_ref[rows, :])
                top = _iota((SUB, TB), 0) < SUB // 2
                o = []
                for j in range(NG):
                    nd = _dot(kv_ref[j], features(pq[j * GR:(j + 1) * GR]))
                    inv = 1.0 / (nd[GR:] + 1e-6)
                    swapped = pltpu.roll(inv, SUB // 2, 0)
                    inv0, inv1 = jnp.where(top, inv, swapped), jnp.where(top, swapped, inv)
                    o.append(nd[:GR] * jnp.concatenate([inv0, inv0, inv, inv1, inv1], axis=0))
                o = jnp.concatenate(o, axis=0).astype(BF16).T
                x = x_ref[rows, :] + _dot(o, bwo_ref[...])
                if last:
                    xb_ref[rows, :] = x.astype(BF16)
                    out_copy(c).start()
                else:
                    x_ref[rows, :] = x
                return carry

            lax.fori_loop(0, NCH, queries, 0)

        reset_memory()
        for g in range(G):
            wo_copy(g).wait()
        layer_a(0, NSEG, pre=True, unroll=UNROLL, lag=99)
        normalise_output(NSEG - 1)
        fold_hedgehog_weights()
        layer_b(last=False)
        reset_memory()
        layer_a(0, NSEG, pre=False, unroll=UNROLL, lag=99)
        normalise_output(NSEG - 1)
        layer_b(last=True)
        for c in range(NCH):
            out_copy(c).wait()

    scratch = [
        pltpu.VMEM((G, D // 2, 3 * PW), jnp.uint32),
        pltpu.VMEM((H * DH, D), BF16),
        pltpu.VMEM((NBUF, 3 * PW, D), BF16),
        pltpu.VMEM((NBUF, XC // SEG, SEG, D), BF16),
        pltpu.VMEM((NSEG, PRE, D), BF16),
        pltpu.VMEM((NSEG * PRE, D), BF16),
        pltpu.VMEM((G, NSEG * PRE, 2 * PW), F32),
        pltpu.VMEM((S, D), BF16),
        pltpu.VMEM((S, D), F32),
        pltpu.VMEM((L, D), F32),
        pltpu.VMEM((D, 3 * D), BF16),
        pltpu.VMEM((FR, D), F32),
        pltpu.VMEM((3, D, D), BF16),
        pltpu.VMEM((D, D), BF16),
        pltpu.VMEM((NG, GR + SUB, 2 * GR), F32),
        pltpu.SemaphoreType.DMA((NBUF, 4)),
        pltpu.SemaphoreType.DMA((G,)),
        pltpu.SemaphoreType.DMA((3,)),
        pltpu.SemaphoreType.DMA((NCH,)),
    ]
    return kernel, scratch


@functools.partial(jax.jit, static_argnames=("A_seg_len",))
def pallas_interleave_layers__memory_aug_recurrent_mem_tr__linear_kernel_hedgehog__prompt_kernel(
    A_x: jax.Array,
    A_mem0: jax.Array,
    A_Wq: jax.Array,
    A_Wk: jax.Array,
    A_Wv: jax.Array,
    A_Wo: jax.Array,
    A_seg_len: int,
    B_x: jax.Array,
    B_wqkv: jax.Array,
    B_w_phi: jax.Array,
    B_wo: jax.Array,
):
    del B_x
    B, S, D = A_x.shape
    M = A_mem0.shape[1]
    _, H, DH = A_Wq.shape
    HB = B_w_phi.shape[0]
    assert B == 1

    kernel, scratch = _make_kernel(S, D, H, DH, M, A_seg_len, HB,
                                   HG=2, TB=512, NBUF=4, UNROLL=4)

    def head_major(w):
        return w.transpose(1, 2, 0).reshape(H * DH, D)

    hbm = pl.BlockSpec(memory_space=pltpu.HBM)
    vmem = pl.BlockSpec(memory_space=pltpu.VMEM)
    out = pl.pallas_call(
        kernel,
        out_shape=jax.ShapeDtypeStruct((S, D), A_x.dtype),
        in_specs=[hbm, vmem, hbm, hbm, hbm, hbm, hbm, vmem, hbm],
        out_specs=hbm,
        scratch_shapes=scratch,
        compiler_params=pltpu.CompilerParams(vmem_limit_bytes=110 * 1024 * 1024,
                                             disable_bounds_checks=True),
    )(
        A_x.reshape(S // A_seg_len, A_seg_len, D), A_mem0.reshape(M, D),
        head_major(A_Wq), head_major(A_Wk), head_major(A_Wv), A_Wo.reshape(H * DH, D),
        B_wqkv, B_w_phi.transpose(1, 2, 0), B_wo,
    )
    return out.reshape(B, S, D)
```

```python
import functools

import jax
import jax.numpy as jnp
from jax import lax
import jax.experimental.pallas as pl
import jax.experimental.pallas.tpu as pltpu

F32 = jnp.float32
BF16 = jnp.bfloat16
LANES = 128
SUB = 8
LOG2E = 1.4426950408889634


def _dot(a, b):
    return lax.dot_general(a, b, (((1,), (0,)), ((), ())), preferred_element_type=F32)


def _dot_nt(a, b):
    return lax.dot_general(a, b, (((1,), (1,)), ((), ())), preferred_element_type=F32)


def _layernorm_parts(x):
    inv_n = 1.0 / x.shape[-1]
    c = x - jnp.sum(x, axis=-1, keepdims=True) * inv_n
    var = jnp.sum(c * c, axis=-1, keepdims=True) * inv_n
    return c, lax.rsqrt(var + 1e-5)


def _layernorm(x):
    c, inv_std = _layernorm_parts(x)
    return c * inv_std


def _recip(x):
    r = pl.reciprocal(x, approx=True)
    return r * (2.0 - x * r)


def _iota(shape, dim):
    return lax.broadcasted_iota(jnp.int32, shape, dim)


def _div20(n):
    return (n * 3277) >> 16


def _make_kernel(S, D, H, DH, M, SEG, HB, *, HG, TB, NBUF, UNROLL):
    L = M + SEG
    G = H // 2
    PW = 2 * DH
    NSEG = S // SEG
    XC = S // G
    PRE = SUB
    DB = D // HB
    NG = HB // HG
    GR = DB * HG
    FR = 4 * DB
    LOG_HG = HG.bit_length() - 1
    NCH = S // TB
    scale = DH ** -0.5
    assert PW == 3 * LANES and 2 * L <= LANES and DB == 20 and D < 1024
    assert L % SUB == 0 and M % SUB == 0 and GR % SUB == 0 and HG == 2
    assert S % TB == 0 and S % G == 0 and NBUF < G and G >= 14
    assert NSEG % UNROLL == 0

    def kernel(x_hbm, mem_ref, wq_hbm, wk_hbm, wv_hbm, wo_hbm, bw_hbm, phi_ref, bwo_hbm,
               out_hbm,
               w_ref, wo_ref, stage_ref, xin_ref, xp_ref, hp_ref, pre_ref,
               xb_ref, x_ref, h_ref,
               bw_ref, phi_rows_ref, bt_ref, bwo_ref, kv_ref,
               stage_sem, wo_sem, misc_sem, out_sem):

        def stage_copies(g):
            slot = g % NBUF
            rows = pl.ds(pl.multiple_of(g * PW, PW), PW)
            copies = [
                pltpu.make_async_copy(src.at[rows, :],
                                      stage_ref.at[slot, pl.ds(j * PW, PW), :],
                                      stage_sem.at[slot, j])
                for j, src in enumerate((wq_hbm, wk_hbm, wv_hbm))]
            copies.append(pltpu.make_async_copy(
                x_hbm.at[pl.ds(g * (XC // SEG), XC // SEG)], xin_ref.at[slot],
                stage_sem.at[slot, 3]))
            return copies

        xp_copy = pltpu.make_async_copy(
            x_hbm.at[:, pl.ds(SEG - PRE, PRE), :], xp_ref, misc_sem.at[0])
        bw_copy = pltpu.make_async_copy(bw_hbm, bw_ref, misc_sem.at[1])
        bwo_copy = pltpu.make_async_copy(bwo_hbm, bwo_ref, misc_sem.at[2])

        def wo_copy(g):
            rows = pl.ds(pl.multiple_of(g * PW, PW), PW)
            return pltpu.make_async_copy(wo_hbm.at[rows, :], wo_ref.at[rows, :], wo_sem.at[g])

        xp_copy.start()
        for cp in stage_copies(0):
            cp.start()

        eh = _iota((HB, D), 0) * DB
        ec = _iota((HB, D), 1)
        phi_flat = None
        for d in range(DB):
            t = _dot(phi_ref[d], jnp.where(ec == eh + d, 1.0, 0.0).astype(BF16))
            phi_flat = t if phi_flat is None else phi_flat + t
        nf = _iota((FR, DB), 0) >> LOG_HG
        sel = jnp.where(nf - DB * _div20(nf) == _iota((FR, DB), 1), 1.0, 0.0)
        phi_rows_ref[...] = _dot(sel.astype(BF16), phi_flat.astype(BF16))

        xp_copy.wait()
        for g in range(1, NBUF):
            for cp in stage_copies(g):
                cp.start()
        hp_ref[...] = _layernorm(
            xp_ref[...].astype(F32).reshape(NSEG * PRE, D)).astype(BF16)

        def load_body(g, carry):
            slot = g % NBUF
            for cp in stage_copies(g):
                cp.wait()
            pre_ref[g] = _dot_nt(hp_ref[...], stage_ref[slot, PW:, :])
            w_ref[g] = pltpu.bitcast(stage_ref[slot].T, jnp.uint32)
            rows = pl.ds(pl.multiple_of(g * XC, XC), XC)
            x_ref[rows, :] = xin_ref[slot].astype(F32).reshape(XC, D)

            @pl.when(g + NBUF < G)
            def _():
                for cp in stage_copies(g + NBUF):
                    cp.start()
                wo_copy(g).start()

            @pl.when(g + NBUF == G)
            def _():
                for k in range(G - NBUF, G):
                    wo_copy(k).start()

            return carry

        lax.fori_loop(0, G, load_body, 0)
        bw_copy.start()
        bwo_copy.start()

        def layer_a(start, stop, pre, unroll, lag):
            row = _iota((L, 2 * L), 0)
            col = _iota((L, 2 * L), 1)
            first = col < L
            visible = (row < M) | (row >= jnp.where(first, col, col - L))
            low = _iota((L, LANES), 1) < DH - LANES
            zero = jnp.zeros((L, LANES), F32)

            def block_diag(t):
                t0, t1, t2 = t[:, :LANES], t[:, LANES:2 * LANES], t[:, 2 * LANES:]
                top = jnp.concatenate([t0, jnp.where(low, t1, 0.0), zero], axis=1)
                bot = jnp.concatenate([zero, jnp.where(low, 0.0, t1), t2], axis=1)
                return jnp.concatenate([top, bot], axis=0).astype(BF16)

            def step(s, h):
                rows = seg_rows(s)
                chained = h is not None
                if not chained:
                    h = h_ref[...]
                h_kv = h[:L - PRE].astype(BF16) if pre else h
                st = {}
                acc = [None]

                def project(g):
                    def times(c0, c1):
                        return [
                            _dot(lhs[:, c0:c1], pltpu.bitcast(
                                w_ref[g, c0 // 2:c1 // 2, j * PW:(j + 1) * PW], BF16))
                            for lhs, j in ((h_kv, 1), (h, 0), (h_kv, 2))]

                    if g == 0 and chained:
                        parts = [times(c, c + LANES) for c in range(0, D, LANES)]
                        k, q, v = [functools.reduce(jnp.add, t) for t in zip(*parts)]
                    else:
                        k, q, v = times(0, D)
                    if pre:
                        done = pre_ref[g, pl.ds(pl.multiple_of(s * PRE, PRE), PRE), :]
                        k = jnp.concatenate([k, done[:, :PW]], axis=0)
                        v = jnp.concatenate([v, done[:, PW:]], axis=0)
                    st[g] = [q, block_diag(k), block_diag(v)]

                def attend(g, after):
                    fill = -1e9
                    if after is not None:
                        fill = jnp.concatenate(
                            [jnp.full((M, 1), fill, F32), jnp.minimum(after, fill)], axis=0)
                    sc = jnp.where(visible, _dot_nt(st[g][0], st[g][1]) * scale, fill)
                    m0 = jnp.max(jnp.where(first, sc, -jnp.inf), axis=1, keepdims=True)
                    m1 = jnp.max(jnp.where(first, -jnp.inf, sc), axis=1, keepdims=True)
                    e = jnp.exp(sc - jnp.where(first, m0, m1))
                    s0 = jnp.sum(jnp.where(first, e, 0.0), axis=1, keepdims=True)
                    s1 = jnp.sum(jnp.where(first, 0.0, e), axis=1, keepdims=True)
                    st[g][0] = e / jnp.where(first, s0, s1)

                def mix(g):
                    st[g] = _dot(st[g][0], st[g][2])

                def out_proj(g0, g1):
                    o = jnp.concatenate([st[g] for g in range(g0, g1)], axis=1)
                    r = _dot(o, wo_ref[g0 * PW:g1 * PW, :])
                    acc[0] = r if acc[0] is None else acc[0] + r

                done = 0
                for i in range(G + 2):
                    if i < G:
                        project(i)
                    while done < (i - lag if i < G else G - 4 * (G + 2 - i)):
                        out_proj(done, done + 1)
                        done += 1
                    after = None
                    if i == 3:
                        prev = seg_rows(jnp.maximum(s - 1, 0))
                        c, after = _layernorm_parts(x_ref[prev, :])
                        xb_ref[prev, :] = (c * after).astype(BF16)
                    if i == 6:
                        c, after = _layernorm_parts(
                            x_ref[seg_rows(jnp.minimum(s + 1, NSEG - 1)), :])
                        xn_next = c * after
                    if 0 <= i - 1 < G:
                        attend(i - 1, after)
                    if 0 <= i - 2 < G:
                        mix(i - 2)
                o = jnp.concatenate([st[g] for g in range(G - 4, G)], axis=1)
                y = jnp.concatenate([
                    acc[0][:, c:c + LANES]
                    + _dot(o, wo_ref[(G - 4) * PW:G * PW, c:c + LANES])
                    for c in range(0, D, LANES)], axis=1)
                x_ref[rows, :] = x_ref[rows, :] + y[M:L]
                return jnp.concatenate([y[0:M], xn_next], axis=0)

            def steps(i, carry):
                h = None
                for u in range(unroll):
                    h = step(i * unroll + u, h)
                h_ref[...] = h
                return carry

            lax.fori_loop(start // unroll, stop // unroll, steps, 0)

        def seg_rows(s):
            return pl.ds(s * SEG if isinstance(s, int) else pl.multiple_of(s * SEG, SEG), SEG)

        def normalise_output(s):
            xb_ref[seg_rows(s), :] = _layernorm(x_ref[seg_rows(s), :]).astype(BF16)

        def reset_memory():
            h_ref[0:M, :] = mem_ref[...].astype(F32)
            h_ref[M:L, :] = _layernorm(x_ref[0:SEG, :])

        def fold_hedgehog_weights():
            bw_copy.wait()
            bwo_copy.wait()
            bt_ref[2] = bw_ref[:, 2 * D:3 * D].T
            for r0 in range(0, D, FR):
                c0 = r0 // LANES * LANES
                c1 = pl.cdiv(r0 + FR, LANES) * LANES
                n = _iota((FR, c1 - c0), 0) + r0
                c = _iota((FR, c1 - c0), 1) + c0
                grp = _div20(n >> LOG_HG)
                head = (grp << LOG_HG) + (n & (HG - 1))
                fold = jnp.where(_div20(c) == head, phi_rows_ref[:, c0:c1], 0.0).astype(BF16)
                for j in range(2):
                    bt_ref[j, r0:r0 + FR, :] = (LOG2E * _dot_nt(
                        fold, bw_ref[:, j * D + c0:j * D + c1])).astype(BF16)

        def over_features(op, p):
            r = p[0:SUB]
            for i in range(1, GR // SUB):
                r = op(r, p[i * SUB:(i + 1) * SUB])
            shift = SUB // 2
            while shift >= HG:
                r = op(r, pltpu.roll(r, shift, 0))
                shift //= 2
            return r

        def spread(r):
            return jnp.concatenate([r] * (GR // SUB), axis=0)

        def features(p):
            ep = jnp.exp2(p - spread(over_features(jnp.maximum, p)))
            en = jnp.exp2(spread(over_features(jnp.minimum, p)) - p)
            fp = ep * spread(_recip(over_features(jnp.add, ep)))
            fn = en * spread(_recip(over_features(jnp.add, en)))
            return jnp.concatenate([fp, fn], axis=0).astype(BF16)

        def out_copy(c):
            rows = pl.ds(pl.multiple_of(c * TB, TB), TB)
            return pltpu.make_async_copy(xb_ref.at[rows, :], out_hbm.at[rows, :], out_sem.at[c])

        def layer_b(last):
            kv_ref[...] = jnp.zeros(kv_ref.shape, F32)

            def keys(c, carry):
                rows = pl.ds(pl.multiple_of(c * TB, TB), TB)
                pk = _dot_nt(bt_ref[1], xb_ref[rows, :])
                v = _dot_nt(bt_ref[2], xb_ref[rows, :])
                ones = jnp.ones((SUB, TB), F32)
                for j in range(NG):
                    vj = jnp.concatenate([v[j * GR:(j + 1) * GR], ones], axis=0)
                    kv_ref[j] += _dot_nt(vj, features(pk[j * GR:(j + 1) * GR]))
                return carry

            lax.fori_loop(0, NCH, keys, 0)

            shape = (GR + SUB, 2 * GR)
            r = _iota(shape, 0)
            second = ((r >= DB) & (r < GR)) | (r >= GR + SUB // 2)
            same_head = second.astype(jnp.int32) == (_iota(shape, 1) & 1)
            for j in range(NG):
                kv_ref[j] = jnp.where(same_head, kv_ref[j], 0.0)

            def queries(c, carry):
                half = TB // 2
                parts = [pl.ds(pl.multiple_of(c * TB + i * half, half), half) for i in range(2)]
                top = _iota((SUB, half), 0) < SUB // 2

                def attend(pq):
                    o = []
                    for j in range(NG):
                        nd = _dot(kv_ref[j], features(pq[j * GR:(j + 1) * GR]))
                        inv = _recip(nd[GR:] + 1e-6)
                        swapped = pltpu.roll(inv, SUB // 2, 0)
                        inv0, inv1 = jnp.where(top, inv, swapped), jnp.where(top, swapped, inv)
                        o.append(nd[:GR] * jnp.concatenate(
                            [inv0, inv0, inv, inv1, inv1], axis=0))
                    return jnp.concatenate(o, axis=0).astype(BF16).T

                pqs = [_dot_nt(bt_ref[0], xb_ref[rows, :]) for rows in parts]
                outs = [attend(pq) for pq in pqs]
                for rows, o in zip(parts, outs):
                    x = x_ref[rows, :] + _dot(o, bwo_ref[...])
                    if last:
                        xb_ref[rows, :] = x.astype(BF16)
                    else:
                        x_ref[rows, :] = x
                if last:
                    out_copy(c).start()
                return carry

            lax.fori_loop(0, NCH, queries, 0)

        reset_memory()
        for g in range(G):
            wo_copy(g).wait()
        layer_a(0, NSEG, pre=True, unroll=UNROLL, lag=99)
        normalise_output(NSEG - 1)
        fold_hedgehog_weights()
        layer_b(last=False)
        reset_memory()
        layer_a(0, NSEG, pre=False, unroll=UNROLL, lag=99)
        normalise_output(NSEG - 1)
        layer_b(last=True)
        for c in range(NCH):
            out_copy(c).wait()

    scratch = [
        pltpu.VMEM((G, D // 2, 3 * PW), jnp.uint32),
        pltpu.VMEM((H * DH, D), BF16),
        pltpu.VMEM((NBUF, 3 * PW, D), BF16),
        pltpu.VMEM((NBUF, XC // SEG, SEG, D), BF16),
        pltpu.VMEM((NSEG, PRE, D), BF16),
        pltpu.VMEM((NSEG * PRE, D), BF16),
        pltpu.VMEM((G, NSEG * PRE, 2 * PW), F32),
        pltpu.VMEM((S, D), BF16),
        pltpu.VMEM((S, D), F32),
        pltpu.VMEM((L, D), F32),
        pltpu.VMEM((D, 3 * D), BF16),
        pltpu.VMEM((FR, D), F32),
        pltpu.VMEM((3, D, D), BF16),
        pltpu.VMEM((D, D), BF16),
        pltpu.VMEM((NG, GR + SUB, 2 * GR), F32),
        pltpu.SemaphoreType.DMA((NBUF, 4)),
        pltpu.SemaphoreType.DMA((G,)),
        pltpu.SemaphoreType.DMA((3,)),
        pltpu.SemaphoreType.DMA((NCH,)),
    ]
    return kernel, scratch


@functools.partial(jax.jit, static_argnames=("A_seg_len",))
def pallas_interleave_layers__memory_aug_recurrent_mem_tr__linear_kernel_hedgehog__prompt_kernel(
    A_x: jax.Array,
    A_mem0: jax.Array,
    A_Wq: jax.Array,
    A_Wk: jax.Array,
    A_Wv: jax.Array,
    A_Wo: jax.Array,
    A_seg_len: int,
    B_x: jax.Array,
    B_wqkv: jax.Array,
    B_w_phi: jax.Array,
    B_wo: jax.Array,
):
    del B_x
    B, S, D = A_x.shape
    M = A_mem0.shape[1]
    _, H, DH = A_Wq.shape
    HB = B_w_phi.shape[0]
    assert B == 1

    kernel, scratch = _make_kernel(S, D, H, DH, M, A_seg_len, HB,
                                   HG=2, TB=512, NBUF=4, UNROLL=4)

    def head_major(w):
        return w.transpose(1, 2, 0).reshape(H * DH, D)

    hbm = pl.BlockSpec(memory_space=pltpu.HBM)
    vmem = pl.BlockSpec(memory_space=pltpu.VMEM)
    out = pl.pallas_call(
        kernel,
        out_shape=jax.ShapeDtypeStruct((S, D), A_x.dtype),
        in_specs=[hbm, vmem, hbm, hbm, hbm, hbm, hbm, vmem, hbm],
        out_specs=hbm,
        scratch_shapes=scratch,
        compiler_params=pltpu.CompilerParams(vmem_limit_bytes=110 * 1024 * 1024,
                                             disable_bounds_checks=True),
    )(
        A_x.reshape(S // A_seg_len, A_seg_len, D), A_mem0.reshape(M, D),
        head_major(A_Wq), head_major(A_Wk), head_major(A_Wv), A_Wo.reshape(H * DH, D),
        B_wqkv, B_w_phi.transpose(1, 2, 0), B_wo,
    )
    return out.reshape(B, S, D)
```

```python
import functools

import jax
import jax.numpy as jnp
from jax import lax
import jax.experimental.pallas as pl
import jax.experimental.pallas.tpu as pltpu

F32 = jnp.float32
BF16 = jnp.bfloat16
LANES = 128
SUB = 8
LOG2E = 1.4426950408889634


def _dot(a, b):
    return lax.dot_general(a, b, (((1,), (0,)), ((), ())), preferred_element_type=F32)


def _dot_nt(a, b):
    return lax.dot_general(a, b, (((1,), (1,)), ((), ())), preferred_element_type=F32)


def _layernorm_parts(x):
    inv_n = 1.0 / x.shape[-1]
    c = x - jnp.sum(x, axis=-1, keepdims=True) * inv_n
    var = jnp.sum(c * c, axis=-1, keepdims=True) * inv_n
    return c, lax.rsqrt(var + 1e-5)


def _layernorm(x):
    c, inv_std = _layernorm_parts(x)
    return c * inv_std


def _recip(x):
    r = pl.reciprocal(x, approx=True)
    return r * (2.0 - x * r)


def _iota(shape, dim):
    return lax.broadcasted_iota(jnp.int32, shape, dim)


def _div20(n):
    return (n * 3277) >> 16


def _make_kernel(S, D, H, DH, M, SEG, HB, *, HG, TB, NBUF, UNROLL):
    L = M + SEG
    G = H // 2
    PW = 2 * DH
    NSEG = S // SEG
    XC = S // G
    PRE = SUB
    DB = D // HB
    NG = HB // HG
    GR = DB * HG
    FR = 4 * DB
    LOG_HG = HG.bit_length() - 1
    NCH = S // TB
    scale = DH ** -0.5
    assert PW == 3 * LANES and 2 * L <= LANES and DB == 20 and D < 1024
    assert L % SUB == 0 and M % SUB == 0 and GR % SUB == 0 and HG == 2
    assert S % TB == 0 and S % G == 0 and NBUF < G and G >= 14
    assert NSEG % UNROLL == 0

    def kernel(x_hbm, mem_ref, wq_hbm, wk_hbm, wv_hbm, wo_hbm, bw_hbm, phi_ref, bwo_hbm,
               out_hbm,
               w_ref, wo_ref, stage_ref, xin_ref, xp_ref, hp_ref, pre_ref,
               xb_ref, x_ref, h_ref,
               bw_ref, phi_rows_ref, bt_ref, bwo_ref, kv_ref, z_ref,
               stage_sem, wo_sem, misc_sem, out_sem):

        def stage_copies(g):
            slot = g % NBUF
            rows = pl.ds(pl.multiple_of(g * PW, PW), PW)
            copies = [
                pltpu.make_async_copy(src.at[rows, :],
                                      stage_ref.at[slot, pl.ds(j * PW, PW), :],
                                      stage_sem.at[slot, j])
                for j, src in enumerate((wq_hbm, wk_hbm, wv_hbm))]
            copies.append(pltpu.make_async_copy(
                x_hbm.at[pl.ds(g * (XC // SEG), XC // SEG)], xin_ref.at[slot],
                stage_sem.at[slot, 3]))
            return copies

        xp_copy = pltpu.make_async_copy(
            x_hbm.at[:, pl.ds(SEG - PRE, PRE), :], xp_ref, misc_sem.at[0])
        bw_copy = pltpu.make_async_copy(bw_hbm, bw_ref, misc_sem.at[1])
        bwo_copy = pltpu.make_async_copy(bwo_hbm, bwo_ref, misc_sem.at[2])

        def wo_copy(g):
            rows = pl.ds(pl.multiple_of(g * PW, PW), PW)
            return pltpu.make_async_copy(wo_hbm.at[rows, :], wo_ref.at[rows, :], wo_sem.at[g])

        xp_copy.start()
        for cp in stage_copies(0):
            cp.start()

        eh = _iota((HB, D), 0) * DB
        ec = _iota((HB, D), 1)
        phi_flat = None
        for d in range(DB):
            t = _dot(phi_ref[d], jnp.where(ec == eh + d, 1.0, 0.0).astype(BF16))
            phi_flat = t if phi_flat is None else phi_flat + t
        nf = _iota((FR, DB), 0) >> LOG_HG
        sel = jnp.where(nf - DB * _div20(nf) == _iota((FR, DB), 1), 1.0, 0.0)
        phi_rows_ref[...] = _dot(sel.astype(BF16), phi_flat.astype(BF16))

        xp_copy.wait()
        for g in range(1, NBUF):
            for cp in stage_copies(g):
                cp.start()
        hp_ref[...] = _layernorm(
            xp_ref[...].astype(F32).reshape(NSEG * PRE, D)).astype(BF16)

        def load_body(g, carry):
            slot = g % NBUF
            for cp in stage_copies(g):
                cp.wait()
            pre_ref[g] = _dot_nt(hp_ref[...], stage_ref[slot, PW:, :])
            w_ref[g] = pltpu.bitcast(stage_ref[slot].T, jnp.uint32)
            rows = pl.ds(pl.multiple_of(g * XC, XC), XC)
            x_ref[rows, :] = xin_ref[slot].astype(F32).reshape(XC, D)

            @pl.when(g + NBUF < G)
            def _():
                for cp in stage_copies(g + NBUF):
                    cp.start()
                wo_copy(g).start()

            @pl.when(g + NBUF == G)
            def _():
                for k in range(G - NBUF, G):
                    wo_copy(k).start()

            return carry

        lax.fori_loop(0, G, load_body, 0)
        bw_copy.start()
        bwo_copy.start()

        def layer_a(start, stop, pre, unroll, lag):
            row = _iota((L, 2 * L), 0)
            col = _iota((L, 2 * L), 1)
            first = col < L
            visible = (row < M) | (row >= jnp.where(first, col, col - L))
            low = _iota((L, LANES), 1) < DH - LANES
            zero = jnp.zeros((L, LANES), F32)

            def block_diag(t):
                t0, t1, t2 = t[:, :LANES], t[:, LANES:2 * LANES], t[:, 2 * LANES:]
                top = jnp.concatenate([t0, jnp.where(low, t1, 0.0), zero], axis=1)
                bot = jnp.concatenate([zero, jnp.where(low, 0.0, t1), t2], axis=1)
                return jnp.concatenate([top, bot], axis=0).astype(BF16)

            def step(s, h):
                rows = seg_rows(s)
                chained = h is not None
                if not chained:
                    h = h_ref[...]
                h_kv = h[:L - PRE].astype(BF16) if pre else h
                st = {}
                acc = [None]

                def project(g):
                    def times(c0, c1):
                        return [
                            _dot(lhs[:, c0:c1], pltpu.bitcast(
                                w_ref[g, c0 // 2:c1 // 2, j * PW:(j + 1) * PW], BF16))
                            for lhs, j in ((h_kv, 1), (h, 0), (h_kv, 2))]

                    if g == 0 and chained:
                        parts = [times(c, c + LANES) for c in range(0, D, LANES)]
                        k, q, v = [functools.reduce(jnp.add, t) for t in zip(*parts)]
                    else:
                        k, q, v = times(0, D)
                    if pre:
                        done = pre_ref[g, pl.ds(pl.multiple_of(s * PRE, PRE), PRE), :]
                        k = jnp.concatenate([k, done[:, :PW]], axis=0)
                        v = jnp.concatenate([v, done[:, PW:]], axis=0)
                    st[g] = [q, block_diag(k), block_diag(v)]

                def attend(g, after):
                    fill = -1e9
                    if after is not None:
                        fill = jnp.concatenate(
                            [jnp.full((M, 1), fill, F32), jnp.minimum(after, fill)], axis=0)
                    sc = jnp.where(visible, _dot_nt(st[g][0], st[g][1]) * scale, fill)
                    m0 = jnp.max(jnp.where(first, sc, -jnp.inf), axis=1, keepdims=True)
                    m1 = jnp.max(jnp.where(first, -jnp.inf, sc), axis=1, keepdims=True)
                    e = jnp.exp(sc - jnp.where(first, m0, m1))
                    s0 = jnp.sum(jnp.where(first, e, 0.0), axis=1, keepdims=True)
                    s1 = jnp.sum(jnp.where(first, 0.0, e), axis=1, keepdims=True)
                    st[g][0] = e / jnp.where(first, s0, s1)

                def mix(g):
                    st[g] = _dot(st[g][0], st[g][2])

                def out_proj(g0, g1):
                    o = jnp.concatenate([st[g] for g in range(g0, g1)], axis=1)
                    r = _dot(o, wo_ref[g0 * PW:g1 * PW, :])
                    acc[0] = r if acc[0] is None else acc[0] + r

                done = 0
                for i in range(G + 2):
                    if i < G:
                        project(i)
                    while done < (i - lag if i < G else G - 4 * (G + 2 - i)):
                        out_proj(done, done + 1)
                        done += 1
                    after = None
                    if i == 3:
                        prev = seg_rows(jnp.maximum(s - 1, 0))
                        c, after = _layernorm_parts(x_ref[prev, :])
                        xb_ref[prev, :] = (c * after).astype(BF16)
                    if i == 6:
                        c, after = _layernorm_parts(
                            x_ref[seg_rows(jnp.minimum(s + 1, NSEG - 1)), :])
                        xn_next = c * after
                    if 0 <= i - 1 < G:
                        attend(i - 1, after)
                    if 0 <= i - 2 < G:
                        mix(i - 2)
                o = jnp.concatenate([st[g] for g in range(G - 4, G)], axis=1)
                y = jnp.concatenate([
                    acc[0][:, c:c + LANES]
                    + _dot(o, wo_ref[(G - 4) * PW:G * PW, c:c + LANES])
                    for c in range(0, D, LANES)], axis=1)
                x_ref[rows, :] = x_ref[rows, :] + y[M:L]
                return jnp.concatenate([y[0:M], xn_next], axis=0)

            def steps(i, carry):
                h = None
                for u in range(unroll):
                    h = step(i * unroll + u, h)
                h_ref[...] = h
                return carry

            lax.fori_loop(start // unroll, stop // unroll, steps, 0)

        def seg_rows(s):
            return pl.ds(s * SEG if isinstance(s, int) else pl.multiple_of(s * SEG, SEG), SEG)

        def normalise_output(s):
            xb_ref[seg_rows(s), :] = _layernorm(x_ref[seg_rows(s), :]).astype(BF16)

        def reset_memory():
            h_ref[0:M, :] = mem_ref[...].astype(F32)
            h_ref[M:L, :] = _layernorm(x_ref[0:SEG, :])

        def fold_hedgehog_weights():
            bw_copy.wait()
            bwo_copy.wait()
            bt_ref[2] = bw_ref[:, 2 * D:3 * D].T
            for r0 in range(0, D, FR):
                c0 = r0 // LANES * LANES
                c1 = pl.cdiv(r0 + FR, LANES) * LANES
                n = _iota((FR, c1 - c0), 0) + r0
                c = _iota((FR, c1 - c0), 1) + c0
                grp = _div20(n >> LOG_HG)
                head = (grp << LOG_HG) + (n & (HG - 1))
                fold = jnp.where(_div20(c) == head, phi_rows_ref[:, c0:c1], 0.0).astype(BF16)
                for j in range(2):
                    bt_ref[j, r0:r0 + FR, :] = (LOG2E * _dot_nt(
                        fold, bw_ref[:, j * D + c0:j * D + c1])).astype(BF16)

        def over_features(op, p):
            r = p[0:SUB]
            for i in range(1, p.shape[0] // SUB):
                r = op(r, p[i * SUB:(i + 1) * SUB])
            shift = SUB // 2
            while shift >= HG:
                r = op(r, pltpu.roll(r, shift, 0))
                shift //= 2
            return r

        def spread(r):
            return jnp.concatenate([r] * (GR // SUB), axis=0)

        def features(p):
            ep = jnp.exp2(p - spread(over_features(jnp.maximum, p)))
            en = jnp.exp2(spread(over_features(jnp.minimum, p)) - p)
            fp = ep * spread(_recip(over_features(jnp.add, ep)))
            fn = en * spread(_recip(over_features(jnp.add, en)))
            return jnp.concatenate([fp, fn], axis=0)

        def out_copy(i):
            rows = pl.ds(pl.multiple_of(i * (TB // 2), TB // 2), TB // 2)
            return pltpu.make_async_copy(xb_ref.at[rows, :], out_hbm.at[rows, :], out_sem.at[i])

        def layer_b(last):
            kv_ref[...] = jnp.zeros(kv_ref.shape, F32)
            z_ref[...] = jnp.zeros(z_ref.shape, F32)

            def keys(c, carry):
                rows = pl.ds(pl.multiple_of(c * TB, TB), TB)
                pk = _dot_nt(bt_ref[1], xb_ref[rows, :])
                v = _dot_nt(bt_ref[2], xb_ref[rows, :])
                for j in range(NG):
                    phi = features(pk[j * GR:(j + 1) * GR])
                    kv_ref[j] += _dot_nt(v[j * GR:(j + 1) * GR], phi.astype(BF16))
                    z_ref[j] += functools.reduce(
                        jnp.add, [phi[:, t:t + LANES] for t in range(0, TB, LANES)])
                return carry

            lax.fori_loop(0, NCH, keys, 0)

            shape = (GR, 2 * GR)
            same_head = (_iota(shape, 0) >= DB).astype(jnp.int32) == (_iota(shape, 1) & 1)
            for j in range(NG):
                kv_ref[j] = jnp.where(same_head, kv_ref[j], 0.0)
                z_ref[j] = jnp.broadcast_to(
                    jnp.sum(z_ref[j], axis=1, keepdims=True), z_ref.shape[1:])

            def queries(c, carry):
                half = TB // 2
                parts = [pl.ds(pl.multiple_of(c * TB + i * half, half), half) for i in range(2)]
                sublane = _iota((SUB, half), 0)
                even = (sublane & 1) == 0

                def attend(pq):
                    o = []
                    for j in range(NG):
                        phi = features(pq[j * GR:(j + 1) * GR])
                        z = jnp.concatenate([z_ref[j]] * (half // LANES), axis=1)
                        inv = _recip(over_features(jnp.add, phi * z) + 1e-6)
                        swapped = pltpu.roll(inv, 1, 0)
                        inv0, inv1 = jnp.where(even, inv, swapped), jnp.where(even, swapped, inv)
                        both = jnp.where(sublane < SUB // 2, inv0, inv1)
                        o.append(_dot(kv_ref[j], phi.astype(BF16)) * jnp.concatenate(
                            [inv0, inv0, both, inv1, inv1], axis=0))
                    return jnp.concatenate(o, axis=0).astype(BF16).T

                pqs = [_dot_nt(bt_ref[0], xb_ref[rows, :]) for rows in parts]
                outs = [attend(pq) for pq in pqs]
                for i, (rows, o) in enumerate(zip(parts, outs)):
                    x = x_ref[rows, :] + _dot(o, bwo_ref[...])
                    if last:
                        xb_ref[rows, :] = x.astype(BF16)
                        out_copy(2 * c + i).start()
                    else:
                        x_ref[rows, :] = x
                return carry

            lax.fori_loop(0, NCH, queries, 0)

        reset_memory()
        for g in range(G):
            wo_copy(g).wait()
        layer_a(0, NSEG, pre=True, unroll=UNROLL, lag=99)
        normalise_output(NSEG - 1)
        fold_hedgehog_weights()
        layer_b(last=False)
        reset_memory()
        layer_a(0, NSEG, pre=False, unroll=UNROLL, lag=99)
        normalise_output(NSEG - 1)
        layer_b(last=True)
        for i in range(2 * NCH):
            out_copy(i).wait()

    scratch = [
        pltpu.VMEM((G, D // 2, 3 * PW), jnp.uint32),
        pltpu.VMEM((H * DH, D), BF16),
        pltpu.VMEM((NBUF, 3 * PW, D), BF16),
        pltpu.VMEM((NBUF, XC // SEG, SEG, D), BF16),
        pltpu.VMEM((NSEG, PRE, D), BF16),
        pltpu.VMEM((NSEG * PRE, D), BF16),
        pltpu.VMEM((G, NSEG * PRE, 2 * PW), F32),
        pltpu.VMEM((S, D), BF16),
        pltpu.VMEM((S, D), F32),
        pltpu.VMEM((L, D), F32),
        pltpu.VMEM((D, 3 * D), BF16),
        pltpu.VMEM((FR, D), F32),
        pltpu.VMEM((3, D, D), BF16),
        pltpu.VMEM((D, D), BF16),
        pltpu.VMEM((NG, GR, 2 * GR), F32),
        pltpu.VMEM((NG, 2 * GR, LANES), F32),
        pltpu.SemaphoreType.DMA((NBUF, 4)),
        pltpu.SemaphoreType.DMA((G,)),
        pltpu.SemaphoreType.DMA((3,)),
        pltpu.SemaphoreType.DMA((2 * NCH,)),
    ]
    return kernel, scratch


@functools.partial(jax.jit, static_argnames=("A_seg_len",))
def pallas_interleave_layers__memory_aug_recurrent_mem_tr__linear_kernel_hedgehog__prompt_kernel(
    A_x: jax.Array,
    A_mem0: jax.Array,
    A_Wq: jax.Array,
    A_Wk: jax.Array,
    A_Wv: jax.Array,
    A_Wo: jax.Array,
    A_seg_len: int,
    B_x: jax.Array,
    B_wqkv: jax.Array,
    B_w_phi: jax.Array,
    B_wo: jax.Array,
):
    del B_x
    B, S, D = A_x.shape
    M = A_mem0.shape[1]
    _, H, DH = A_Wq.shape
    HB = B_w_phi.shape[0]
    assert B == 1

    kernel, scratch = _make_kernel(S, D, H, DH, M, A_seg_len, HB,
                                   HG=2, TB=512, NBUF=4, UNROLL=4)

    def head_major(w):
        return w.transpose(1, 2, 0).reshape(H * DH, D)

    hbm = pl.BlockSpec(memory_space=pltpu.HBM)
    vmem = pl.BlockSpec(memory_space=pltpu.VMEM)
    out = pl.pallas_call(
        kernel,
        out_shape=jax.ShapeDtypeStruct((S, D), A_x.dtype),
        in_specs=[hbm, vmem, hbm, hbm, hbm, hbm, hbm, vmem, hbm],
        out_specs=hbm,
        scratch_shapes=scratch,
        compiler_params=pltpu.CompilerParams(vmem_limit_bytes=110 * 1024 * 1024,
                                             disable_bounds_checks=True),
    )(
        A_x.reshape(S // A_seg_len, A_seg_len, D), A_mem0.reshape(M, D),
        head_major(A_Wq), head_major(A_Wk), head_major(A_Wv), A_Wo.reshape(H * DH, D),
        B_wqkv, B_w_phi.transpose(1, 2, 0), B_wo,
    )
    return out.reshape(B, S, D)
```

```python
import functools

import jax
import jax.numpy as jnp
from jax import lax
import jax.experimental.pallas as pl
import jax.experimental.pallas.tpu as pltpu

F32 = jnp.float32
BF16 = jnp.bfloat16
LANES = 128
SUB = 8
LOG2E = 1.4426950408889634


def _dot(a, b):
    return lax.dot_general(a, b, (((1,), (0,)), ((), ())), preferred_element_type=F32)


def _dot_nt(a, b):
    return lax.dot_general(a, b, (((1,), (1,)), ((), ())), preferred_element_type=F32)


def _layernorm_parts(x):
    inv_n = 1.0 / x.shape[-1]
    c = x - jnp.sum(x, axis=-1, keepdims=True) * inv_n
    var = jnp.sum(c * c, axis=-1, keepdims=True) * inv_n
    return c, lax.rsqrt(var + 1e-5)


def _layernorm(x):
    c, inv_std = _layernorm_parts(x)
    return c * inv_std


def _recip(x):
    r = pl.reciprocal(x, approx=True)
    return r * (2.0 - x * r)


def _iota(shape, dim):
    return lax.broadcasted_iota(jnp.int32, shape, dim)


def _div20(n):
    return (n * 3277) >> 16


def _make_kernel(S, D, H, DH, M, SEG, HB, *, HG, TB, NBUF, UNROLL):
    L = M + SEG
    G = H // 2
    PW = 2 * DH
    NSEG = S // SEG
    PRE = SUB
    DB = D // HB
    NG = HB // HG
    GR = DB * HG
    FR = 4 * DB
    LOG_HG = HG.bit_length() - 1
    NCH = S // TB
    scale = DH ** -0.5
    assert PW == 3 * LANES and 2 * L <= LANES and DB == 20 and D < 1024
    assert L % SUB == 0 and M % SUB == 0 and GR % SUB == 0 and HG == 2
    assert S % TB == 0 and NBUF < G and G >= 14
    assert NSEG % UNROLL == 0

    def kernel(x_hbm, mem_ref, wq_hbm, wk_hbm, wv_hbm, wo_hbm, bw_hbm, phi_ref, bwo_hbm,
               out_hbm,
               w_ref, wo_ref, stage_ref, xin_ref, xp_ref, hp_ref, pre_ref,
               xb_ref, x_ref, h_ref,
               bw_ref, phi_rows_ref, bt_ref, bwo_ref, kv_ref, z_ref,
               stage_sem, wo_sem, misc_sem, out_sem):

        def stage_copies(g):
            slot = g % NBUF
            rows = pl.ds(pl.multiple_of(g * PW, PW), PW)
            return [
                pltpu.make_async_copy(src.at[rows, :],
                                      stage_ref.at[slot, pl.ds(j * PW, PW), :],
                                      stage_sem.at[slot, j])
                for j, src in enumerate((wq_hbm, wk_hbm, wv_hbm))]

        xp_copy = pltpu.make_async_copy(
            x_hbm.at[:, pl.ds(SEG - PRE, PRE), :], xp_ref, misc_sem.at[0])
        bw_copy = pltpu.make_async_copy(bw_hbm, bw_ref, misc_sem.at[1])
        bwo_copy = pltpu.make_async_copy(bwo_hbm, bwo_ref, misc_sem.at[2])

        head, rest = pl.ds(0, 2 * UNROLL), pl.ds(2 * UNROLL, NSEG - 2 * UNROLL)
        x_head_copy = pltpu.make_async_copy(x_hbm.at[head], xin_ref.at[head], misc_sem.at[3])
        x_rest_copy = pltpu.make_async_copy(x_hbm.at[rest], xin_ref.at[rest], misc_sem.at[4])

        def wo_copy(g):
            rows = pl.ds(pl.multiple_of(g * PW, PW), PW)
            return pltpu.make_async_copy(wo_hbm.at[rows, :], wo_ref.at[rows, :], wo_sem.at[g])

        xp_copy.start()
        for cp in stage_copies(0):
            cp.start()

        eh = _iota((HB, D), 0) * DB
        ec = _iota((HB, D), 1)
        phi_flat = None
        for d in range(DB):
            t = _dot(phi_ref[d], jnp.where(ec == eh + d, 1.0, 0.0).astype(BF16))
            phi_flat = t if phi_flat is None else phi_flat + t
        nf = _iota((FR, DB), 0) >> LOG_HG
        sel = jnp.where(nf - DB * _div20(nf) == _iota((FR, DB), 1), 1.0, 0.0)
        phi_rows_ref[...] = _dot(sel.astype(BF16), phi_flat.astype(BF16))

        xp_copy.wait()
        hp_ref[...] = _layernorm(
            xp_ref[...].astype(F32).reshape(NSEG * PRE, D)).astype(BF16)
        for cp in stage_copies(1):
            cp.start()
        for cp in stage_copies(0):
            cp.wait()
        for g in range(2, NBUF):
            for cp in stage_copies(g):
                cp.start()

        def load_body(g, carry):
            slot = g % NBUF
            pre_ref[g] = _dot_nt(hp_ref[...], stage_ref[slot, PW:, :])
            w_ref[g] = pltpu.bitcast(stage_ref[slot].T, jnp.uint32)

            @pl.when(g + NBUF < G)
            def _():
                for cp in stage_copies(g + NBUF):
                    cp.start()
                wo_copy(g).start()

            @pl.when(g + NBUF == G)
            def _():
                x_head_copy.start()
                for k in range(G - NBUF, G):
                    wo_copy(k).start()

            @pl.when(g + 1 < G)
            def _():
                for cp in stage_copies(g + 1):
                    cp.wait()

            return carry

        lax.fori_loop(0, G, load_body, 0)

        def layer_a(start, stop, pre, unroll, lag):
            row = _iota((L, 2 * L), 0)
            col = _iota((L, 2 * L), 1)
            first = col < L
            visible = (row < M) | (row >= jnp.where(first, col, col - L))
            low = _iota((L, LANES), 1) < DH - LANES
            zero = jnp.zeros((L, LANES), F32)

            def block_diag(t):
                t0, t1, t2 = t[:, :LANES], t[:, LANES:2 * LANES], t[:, 2 * LANES:]
                top = jnp.concatenate([t0, jnp.where(low, t1, 0.0), zero], axis=1)
                bot = jnp.concatenate([zero, jnp.where(low, 0.0, t1), t2], axis=1)
                return jnp.concatenate([top, bot], axis=0).astype(BF16)

            def step(s, h):
                rows = seg_rows(s)
                chained = h is not None
                if not chained:
                    h = h_ref[...]
                h_kv = h[:L - PRE].astype(BF16) if pre else h
                st = {}
                acc = [None]

                def project(g):
                    def times(c0, c1):
                        return [
                            _dot(lhs[:, c0:c1], pltpu.bitcast(
                                w_ref[g, c0 // 2:c1 // 2, j * PW:(j + 1) * PW], BF16))
                            for lhs, j in ((h_kv, 1), (h, 0), (h_kv, 2))]

                    if g == 0 and chained:
                        parts = [times(c, c + LANES) for c in range(0, D, LANES)]
                        k, q, v = [functools.reduce(jnp.add, t) for t in zip(*parts)]
                    else:
                        k, q, v = times(0, D)
                    if pre:
                        done = pre_ref[g, pl.ds(pl.multiple_of(s * PRE, PRE), PRE), :]
                        k = jnp.concatenate([k, done[:, :PW]], axis=0)
                        v = jnp.concatenate([v, done[:, PW:]], axis=0)
                    st[g] = [q, block_diag(k), block_diag(v)]

                def attend(g, after):
                    fill = -1e9
                    if after is not None:
                        fill = jnp.concatenate(
                            [jnp.full((M, 1), fill, F32), jnp.minimum(after, fill)], axis=0)
                    sc = jnp.where(visible, _dot_nt(st[g][0], st[g][1]) * scale, fill)
                    m0 = jnp.max(jnp.where(first, sc, -jnp.inf), axis=1, keepdims=True)
                    m1 = jnp.max(jnp.where(first, -jnp.inf, sc), axis=1, keepdims=True)
                    e = jnp.exp(sc - jnp.where(first, m0, m1))
                    s0 = jnp.sum(jnp.where(first, e, 0.0), axis=1, keepdims=True)
                    s1 = jnp.sum(jnp.where(first, 0.0, e), axis=1, keepdims=True)
                    st[g][0] = e / jnp.where(first, s0, s1)

                def mix(g):
                    st[g] = _dot(st[g][0], st[g][2])

                def out_proj(g0, g1):
                    o = jnp.concatenate([st[g] for g in range(g0, g1)], axis=1)
                    r = _dot(o, wo_ref[g0 * PW:g1 * PW, :])
                    acc[0] = r if acc[0] is None else acc[0] + r

                done = 0
                for i in range(G + 2):
                    if i < G:
                        project(i)
                    while done < (i - lag if i < G else G - 4 * (G + 2 - i)):
                        out_proj(done, done + 1)
                        done += 1
                    after = None
                    if i == 3:
                        prev = seg_rows(jnp.maximum(s - 1, 0))
                        c, after = _layernorm_parts(x_ref[prev, :])
                        xb_ref[prev, :] = (c * after).astype(BF16)
                    if i == 6:
                        c, after = _layernorm_parts(tokens(jnp.minimum(s + 1, NSEG - 1), pre))
                        xn_next = c * after
                    if 0 <= i - 1 < G:
                        attend(i - 1, after)
                    if 0 <= i - 2 < G:
                        mix(i - 2)
                o = jnp.concatenate([st[g] for g in range(G - 4, G)], axis=1)
                y = jnp.concatenate([
                    acc[0][:, c:c + LANES]
                    + _dot(o, wo_ref[(G - 4) * PW:G * PW, c:c + LANES])
                    for c in range(0, D, LANES)], axis=1)
                x_ref[rows, :] = tokens(s, pre) + y[M:L]
                return jnp.concatenate([y[0:M], xn_next], axis=0)

            def steps(i, carry):
                if pre:
                    pl.when(i == 1)(x_rest_copy.wait)
                h = None
                for u in range(unroll):
                    h = step(i * unroll + u, h)
                h_ref[...] = h
                return carry

            lax.fori_loop(start // unroll, stop // unroll, steps, 0)

        def seg_rows(s):
            return pl.ds(s * SEG if isinstance(s, int) else pl.multiple_of(s * SEG, SEG), SEG)

        def normalise_output(s):
            xb_ref[seg_rows(s), :] = _layernorm(x_ref[seg_rows(s), :]).astype(BF16)

        def tokens(s, from_input):
            return xin_ref[s].astype(F32) if from_input else x_ref[seg_rows(s), :]

        def reset_memory(from_input):
            h_ref[0:M, :] = mem_ref[...].astype(F32)
            h_ref[M:L, :] = _layernorm(tokens(0, from_input))

        def fold_hedgehog_weights():
            bw_copy.wait()
            bwo_copy.wait()
            bt_ref[2] = bw_ref[:, 2 * D:3 * D].T
            for r0 in range(0, D, FR):
                c0 = r0 // LANES * LANES
                c1 = pl.cdiv(r0 + FR, LANES) * LANES
                n = _iota((FR, c1 - c0), 0) + r0
                c = _iota((FR, c1 - c0), 1) + c0
                grp = _div20(n >> LOG_HG)
                head = (grp << LOG_HG) + (n & (HG - 1))
                fold = jnp.where(_div20(c) == head, phi_rows_ref[:, c0:c1], 0.0).astype(BF16)
                for j in range(2):
                    bt_ref[j, r0:r0 + FR, :] = (LOG2E * _dot_nt(
                        fold, bw_ref[:, j * D + c0:j * D + c1])).astype(BF16)

        def over_features(op, p):
            r = p[0:SUB]
            for i in range(1, p.shape[0] // SUB):
                r = op(r, p[i * SUB:(i + 1) * SUB])
            shift = SUB // 2
            while shift >= HG:
                r = op(r, pltpu.roll(r, shift, 0))
                shift //= 2
            return r

        def spread(r):
            return jnp.concatenate([r] * (GR // SUB), axis=0)

        def features(p):
            ep = jnp.exp2(p - spread(over_features(jnp.maximum, p)))
            en = jnp.exp2(spread(over_features(jnp.minimum, p)) - p)
            fp = ep * spread(_recip(over_features(jnp.add, ep)))
            fn = en * spread(_recip(over_features(jnp.add, en)))
            return jnp.concatenate([fp, fn], axis=0)

        def out_copy(i):
            rows = pl.ds(pl.multiple_of(i * (TB // 2), TB // 2), TB // 2)
            return pltpu.make_async_copy(xb_ref.at[rows, :], out_hbm.at[rows, :], out_sem.at[i])

        def layer_b(last):
            kv_ref[...] = jnp.zeros(kv_ref.shape, F32)
            z_ref[...] = jnp.zeros(z_ref.shape, F32)

            def keys(c, carry):
                rows = pl.ds(pl.multiple_of(c * TB, TB), TB)
                pk = _dot_nt(bt_ref[1], xb_ref[rows, :])
                v = _dot_nt(bt_ref[2], xb_ref[rows, :])
                for j in range(NG):
                    phi = features(pk[j * GR:(j + 1) * GR])
                    kv_ref[j] += _dot_nt(v[j * GR:(j + 1) * GR], phi.astype(BF16))
                    z_ref[j] += functools.reduce(
                        jnp.add, [phi[:, t:t + LANES] for t in range(0, TB, LANES)])
                return carry

            lax.fori_loop(0, NCH, keys, 0)

            shape = (GR, 2 * GR)
            same_head = (_iota(shape, 0) >= DB).astype(jnp.int32) == (_iota(shape, 1) & 1)
            for j in range(NG):
                kv_ref[j] = jnp.where(same_head, kv_ref[j], 0.0)
                z_ref[j] = jnp.broadcast_to(
                    jnp.sum(z_ref[j], axis=1, keepdims=True), z_ref.shape[1:])

            def queries(c, carry):
                half = TB // 2
                parts = [pl.ds(pl.multiple_of(c * TB + i * half, half), half) for i in range(2)]
                sublane = _iota((SUB, half), 0)
                even = (sublane & 1) == 0

                def attend(pq):
                    o = []
                    for j in range(NG):
                        phi = features(pq[j * GR:(j + 1) * GR])
                        z = jnp.concatenate([z_ref[j]] * (half // LANES), axis=1)
                        inv = _recip(over_features(jnp.add, phi * z) + 1e-6)
                        swapped = pltpu.roll(inv, 1, 0)
                        inv0, inv1 = jnp.where(even, inv, swapped), jnp.where(even, swapped, inv)
                        both = jnp.where(sublane < SUB // 2, inv0, inv1)
                        o.append(_dot(kv_ref[j], phi.astype(BF16)) * jnp.concatenate(
                            [inv0, inv0, both, inv1, inv1], axis=0))
                    return jnp.concatenate(o, axis=0).astype(BF16).T

                pqs = [_dot_nt(bt_ref[0], xb_ref[rows, :]) for rows in parts]
                outs = [attend(pq) for pq in pqs]
                for i, (rows, o) in enumerate(zip(parts, outs)):
                    x = x_ref[rows, :] + _dot(o, bwo_ref[...])
                    if last:
                        xb_ref[rows, :] = x.astype(BF16)
                        out_copy(2 * c + i).start()
                    else:
                        x_ref[rows, :] = x
                return carry

            lax.fori_loop(0, NCH, queries, 0)

        x_head_copy.wait()
        x_ref[seg_rows(0), :] = tokens(0, True)
        reset_memory(True)
        for g in range(G):
            wo_copy(g).wait()
        x_rest_copy.start()
        bw_copy.start()
        bwo_copy.start()
        layer_a(0, NSEG, pre=True, unroll=UNROLL, lag=99)
        normalise_output(NSEG - 1)
        fold_hedgehog_weights()
        layer_b(last=False)
        reset_memory(False)
        layer_a(0, NSEG, pre=False, unroll=UNROLL, lag=99)
        normalise_output(NSEG - 1)
        layer_b(last=True)
        for i in range(2 * NCH):
            out_copy(i).wait()

    scratch = [
        pltpu.VMEM((G, D // 2, 3 * PW), jnp.uint32),
        pltpu.VMEM((H * DH, D), BF16),
        pltpu.VMEM((NBUF, 3 * PW, D), BF16),
        pltpu.VMEM((NSEG, SEG, D), BF16),
        pltpu.VMEM((NSEG, PRE, D), BF16),
        pltpu.VMEM((NSEG * PRE, D), BF16),
        pltpu.VMEM((G, NSEG * PRE, 2 * PW), F32),
        pltpu.VMEM((S, D), BF16),
        pltpu.VMEM((S, D), F32),
        pltpu.VMEM((L, D), F32),
        pltpu.VMEM((D, 3 * D), BF16),
        pltpu.VMEM((FR, D), F32),
        pltpu.VMEM((3, D, D), BF16),
        pltpu.VMEM((D, D), BF16),
        pltpu.VMEM((NG, GR, 2 * GR), F32),
        pltpu.VMEM((NG, 2 * GR, LANES), F32),
        pltpu.SemaphoreType.DMA((NBUF, 3)),
        pltpu.SemaphoreType.DMA((G,)),
        pltpu.SemaphoreType.DMA((5,)),
        pltpu.SemaphoreType.DMA((2 * NCH,)),
    ]
    return kernel, scratch


@functools.partial(jax.jit, static_argnames=("A_seg_len",))
def pallas_interleave_layers__memory_aug_recurrent_mem_tr__linear_kernel_hedgehog__prompt_kernel(
    A_x: jax.Array,
    A_mem0: jax.Array,
    A_Wq: jax.Array,
    A_Wk: jax.Array,
    A_Wv: jax.Array,
    A_Wo: jax.Array,
    A_seg_len: int,
    B_x: jax.Array,
    B_wqkv: jax.Array,
    B_w_phi: jax.Array,
    B_wo: jax.Array,
):
    del B_x
    B, S, D = A_x.shape
    M = A_mem0.shape[1]
    _, H, DH = A_Wq.shape
    HB = B_w_phi.shape[0]
    assert B == 1

    kernel, scratch = _make_kernel(S, D, H, DH, M, A_seg_len, HB,
                                   HG=2, TB=512, NBUF=3, UNROLL=4)

    def head_major(w):
        return w.transpose(1, 2, 0).reshape(H * DH, D)

    hbm = pl.BlockSpec(memory_space=pltpu.HBM)
    vmem = pl.BlockSpec(memory_space=pltpu.VMEM)
    out = pl.pallas_call(
        kernel,
        out_shape=jax.ShapeDtypeStruct((S, D), A_x.dtype),
        in_specs=[hbm, vmem, hbm, hbm, hbm, hbm, hbm, vmem, hbm],
        out_specs=hbm,
        scratch_shapes=scratch,
        compiler_params=pltpu.CompilerParams(vmem_limit_bytes=110 * 1024 * 1024),
    )(
        A_x.reshape(S // A_seg_len, A_seg_len, D), A_mem0.reshape(M, D),
        head_major(A_Wq), head_major(A_Wk), head_major(A_Wv), A_Wo.reshape(H * DH, D),
        B_wqkv, B_w_phi.transpose(1, 2, 0), B_wo,
    )
    return out.reshape(B, S, D)
```

```python
import functools

import jax
import jax.numpy as jnp
from jax import lax
import jax.experimental.pallas as pl
import jax.experimental.pallas.tpu as pltpu

F32 = jnp.float32
BF16 = jnp.bfloat16
LANES = 128
SUB = 8
LOG2E = 1.4426950408889634


def _dot(a, b):
    return lax.dot_general(a, b, (((1,), (0,)), ((), ())), preferred_element_type=F32)


def _dot_nt(a, b):
    return lax.dot_general(a, b, (((1,), (1,)), ((), ())), preferred_element_type=F32)


def _layernorm_parts(x):
    inv_n = 1.0 / x.shape[-1]
    c = x - jnp.sum(x, axis=-1, keepdims=True) * inv_n
    var = jnp.sum(c * c, axis=-1, keepdims=True) * inv_n
    return c, lax.rsqrt(var + 1e-5)


def _layernorm(x):
    c, inv_std = _layernorm_parts(x)
    return c * inv_std


def _recip(x):
    r = pl.reciprocal(x, approx=True)
    return r * (2.0 - x * r)


def _iota(shape, dim):
    return lax.broadcasted_iota(jnp.int32, shape, dim)


def _div20(n):
    return (n * 3277) >> 16


def _make_kernel(S, D, H, DH, M, SEG, HB, *, HG, TB, NBUF, UNROLL):
    L = M + SEG
    G = H // 2
    PW = 2 * DH
    NSEG = S // SEG
    PRE = SUB
    ATTEND_LAG, MIX_LAG, TAIL = 1, 3, 8
    DB = D // HB
    NG = HB // HG
    GR = DB * HG
    FR = 4 * DB
    LOG_HG = HG.bit_length() - 1
    NCH = S // TB
    scale = DH ** -0.5
    assert PW == 3 * LANES and 2 * L <= LANES and DB == 20 and D < 1024
    assert L % SUB == 0 and M % SUB == 0 and GR % SUB == 0 and HG == 2
    assert S % TB == 0 and NBUF < G and G >= 14
    assert NSEG % UNROLL == 0

    def kernel(x_hbm, mem_ref, wq_hbm, wk_hbm, wv_hbm, wo_hbm, bw_hbm, phi_ref, bwo_hbm,
               out_hbm,
               w_ref, wo_ref, stage_ref, xin_ref, xp_ref, hp_ref, pre_ref,
               xb_ref, x_ref, h_ref,
               bw_ref, phi_rows_ref, bt_ref, bwo_ref, kv_ref, z_ref,
               stage_sem, wo_sem, misc_sem, out_sem):

        def stage_copies(g):
            slot = g % NBUF
            rows = pl.ds(pl.multiple_of(g * PW, PW), PW)
            return [
                pltpu.make_async_copy(src.at[rows, :],
                                      stage_ref.at[slot, pl.ds(j * PW, PW), :],
                                      stage_sem.at[slot, j])
                for j, src in enumerate((wq_hbm, wk_hbm, wv_hbm))]

        xp_copy = pltpu.make_async_copy(
            x_hbm.at[:, pl.ds(SEG - PRE, PRE), :], xp_ref, misc_sem.at[0])
        bw_copy = pltpu.make_async_copy(bw_hbm, bw_ref, misc_sem.at[1])
        bwo_copy = pltpu.make_async_copy(bwo_hbm, bwo_ref, misc_sem.at[2])

        head, rest = pl.ds(0, 2 * UNROLL), pl.ds(2 * UNROLL, NSEG - 2 * UNROLL)
        x_head_copy = pltpu.make_async_copy(x_hbm.at[head], xin_ref.at[head], misc_sem.at[3])
        x_rest_copy = pltpu.make_async_copy(x_hbm.at[rest], xin_ref.at[rest], misc_sem.at[4])

        def wo_copy(g):
            rows = pl.ds(pl.multiple_of(g * PW, PW), PW)
            return pltpu.make_async_copy(wo_hbm.at[rows, :], wo_ref.at[rows, :], wo_sem.at[g])

        xp_copy.start()
        for cp in stage_copies(0):
            cp.start()

        eh = _iota((HB, D), 0) * DB
        ec = _iota((HB, D), 1)
        phi_flat = None
        for d in range(DB):
            t = _dot(phi_ref[d], jnp.where(ec == eh + d, 1.0, 0.0).astype(BF16))
            phi_flat = t if phi_flat is None else phi_flat + t
        nf = _iota((FR, DB), 0) >> LOG_HG
        sel = jnp.where(nf - DB * _div20(nf) == _iota((FR, DB), 1), 1.0, 0.0)
        phi_rows_ref[...] = _dot(sel.astype(BF16), phi_flat.astype(BF16))

        xp_copy.wait()
        hp_ref[...] = _layernorm(
            xp_ref[...].astype(F32).reshape(NSEG * PRE, D)).astype(BF16)
        for cp in stage_copies(1):
            cp.start()
        for cp in stage_copies(0):
            cp.wait()
        for g in range(2, NBUF):
            for cp in stage_copies(g):
                cp.start()

        def load_body(g, carry):
            slot = g % NBUF
            pre_ref[g] = _dot_nt(hp_ref[...], stage_ref[slot, PW:, :])
            w_ref[g] = pltpu.bitcast(stage_ref[slot].T, jnp.uint32)

            @pl.when(g + NBUF < G)
            def _():
                for cp in stage_copies(g + NBUF):
                    cp.start()
                wo_copy(g).start()

            @pl.when(g + NBUF == G)
            def _():
                x_head_copy.start()
                for k in range(G - NBUF, G):
                    wo_copy(k).start()

            @pl.when(g + 1 < G)
            def _():
                for cp in stage_copies(g + 1):
                    cp.wait()

            return carry

        lax.fori_loop(0, G, load_body, 0)

        def layer_a(pre):
            row = _iota((L, 2 * L), 0)
            col = _iota((L, 2 * L), 1)
            first = col < L
            visible = (row < M) | (row >= jnp.where(first, col, col - L))
            low = _iota((L, LANES), 1) < DH - LANES
            zero = jnp.zeros((L, LANES), F32)

            def block_diag(t):
                t0, t1, t2 = t[:, :LANES], t[:, LANES:2 * LANES], t[:, 2 * LANES:]
                top = jnp.concatenate([t0, jnp.where(low, t1, 0.0), zero], axis=1)
                bot = jnp.concatenate([zero, jnp.where(low, 0.0, t1), t2], axis=1)
                return jnp.concatenate([top, bot], axis=0).astype(BF16)

            def step(s, h):
                rows = seg_rows(s)
                chained = h is not None
                if not chained:
                    h = h_ref[...]
                h_kv = h[:L - PRE].astype(BF16) if pre else h
                st = {}
                acc = [None]

                def project(g):
                    def times(c0, c1):
                        return [
                            _dot(lhs[:, c0:c1], pltpu.bitcast(
                                w_ref[g, c0 // 2:c1 // 2, j * PW:(j + 1) * PW], BF16))
                            for lhs, j in ((h_kv, 1), (h, 0), (h_kv, 2))]

                    if g == 0 and chained:
                        parts = [times(c, c + LANES) for c in range(0, D, LANES)]
                        k, q, v = [functools.reduce(jnp.add, t) for t in zip(*parts)]
                    else:
                        k, q, v = times(0, D)
                    if pre:
                        done = pre_ref[g, pl.ds(pl.multiple_of(s * PRE, PRE), PRE), :]
                        k = jnp.concatenate([k, done[:, :PW]], axis=0)
                        v = jnp.concatenate([v, done[:, PW:]], axis=0)
                    st[g] = [q, block_diag(k), block_diag(v)]

                def attend(g, after):
                    fill = -1e9
                    if after is not None:
                        fill = jnp.concatenate(
                            [jnp.full((M, 1), fill, F32), jnp.minimum(after, fill)], axis=0)
                    sc = jnp.where(visible, _dot_nt(st[g][0], st[g][1]) * scale, fill)
                    m0 = jnp.max(jnp.where(first, sc, -jnp.inf), axis=1, keepdims=True)
                    m1 = jnp.max(jnp.where(first, -jnp.inf, sc), axis=1, keepdims=True)
                    e = jnp.exp(sc - jnp.where(first, m0, m1))
                    s0 = jnp.sum(jnp.where(first, e, 0.0), axis=1, keepdims=True)
                    s1 = jnp.sum(jnp.where(first, 0.0, e), axis=1, keepdims=True)
                    st[g][0] = e / jnp.where(first, s0, s1)

                def mix(g):
                    st[g] = _dot(st[g][0], st[g][2])

                def out_proj(g):
                    r = _dot(st[g], wo_ref[g * PW:(g + 1) * PW, :])
                    acc[0] = r if acc[0] is None else acc[0] + r

                for i in range(G + MIX_LAG):
                    if i < G:
                        project(i)
                    else:
                        for g in range((G - TAIL) * (i - G) // MIX_LAG,
                                       (G - TAIL) * (i - G + 1) // MIX_LAG):
                            out_proj(g)
                    after = None
                    if i == 3:
                        prev = seg_rows(jnp.maximum(s - 1, 0))
                        c, after = _layernorm_parts(x_ref[prev, :])
                        xb_ref[prev, :] = (c * after).astype(BF16)
                    if i == 6:
                        c, after = _layernorm_parts(tokens(jnp.minimum(s + 1, NSEG - 1), pre))
                        xn_next = c * after
                    if 0 <= i - ATTEND_LAG < G:
                        attend(i - ATTEND_LAG, after)
                    if 0 <= i - MIX_LAG < G:
                        mix(i - MIX_LAG)
                o = jnp.concatenate([st[g] for g in range(G - TAIL, G)], axis=1)
                y = jnp.concatenate([
                    acc[0][:, c:c + LANES]
                    + _dot(o, wo_ref[(G - TAIL) * PW:G * PW, c:c + LANES])
                    for c in range(0, D, LANES)], axis=1)
                x_ref[rows, :] = tokens(s, pre) + y[M:L]
                return jnp.concatenate([y[0:M], xn_next], axis=0)

            def steps(i, carry):
                if pre:
                    pl.when(i == 1)(x_rest_copy.wait)
                h = None
                for u in range(UNROLL):
                    h = step(i * UNROLL + u, h)
                h_ref[...] = h
                return carry

            lax.fori_loop(0, NSEG // UNROLL, steps, 0)

        def seg_rows(s):
            return pl.ds(s * SEG if isinstance(s, int) else pl.multiple_of(s * SEG, SEG), SEG)

        def normalise_output(s):
            xb_ref[seg_rows(s), :] = _layernorm(x_ref[seg_rows(s), :]).astype(BF16)

        def tokens(s, from_input):
            return xin_ref[s].astype(F32) if from_input else x_ref[seg_rows(s), :]

        def reset_memory(from_input):
            h_ref[0:M, :] = mem_ref[...].astype(F32)
            h_ref[M:L, :] = _layernorm(tokens(0, from_input))

        def fold_hedgehog_weights():
            bw_copy.wait()
            bwo_copy.wait()
            bt_ref[2] = bw_ref[:, 2 * D:3 * D].T
            for r0 in range(0, D, FR):
                c0 = r0 // LANES * LANES
                c1 = pl.cdiv(r0 + FR, LANES) * LANES
                n = _iota((FR, c1 - c0), 0) + r0
                c = _iota((FR, c1 - c0), 1) + c0
                grp = _div20(n >> LOG_HG)
                head = (grp << LOG_HG) + (n & (HG - 1))
                fold = jnp.where(_div20(c) == head, phi_rows_ref[:, c0:c1], 0.0).astype(BF16)
                for j in range(2):
                    bt_ref[j, r0:r0 + FR, :] = (LOG2E * _dot_nt(
                        fold, bw_ref[:, j * D + c0:j * D + c1])).astype(BF16)

        def over_features(op, p):
            r = p[0:SUB]
            for i in range(1, p.shape[0] // SUB):
                r = op(r, p[i * SUB:(i + 1) * SUB])
            shift = SUB // 2
            while shift >= HG:
                r = op(r, pltpu.roll(r, shift, 0))
                shift //= 2
            return r

        def spread(r):
            return jnp.concatenate([r] * (GR // SUB), axis=0)

        def features(p):
            ep = jnp.exp2(p - spread(over_features(jnp.maximum, p)))
            en = jnp.exp2(spread(over_features(jnp.minimum, p)) - p)
            fp = ep * spread(_recip(over_features(jnp.add, ep)))
            fn = en * spread(_recip(over_features(jnp.add, en)))
            return jnp.concatenate([fp, fn], axis=0)

        def out_copy(i):
            rows = pl.ds(pl.multiple_of(i * (TB // 2), TB // 2), TB // 2)
            return pltpu.make_async_copy(xb_ref.at[rows, :], out_hbm.at[rows, :], out_sem.at[i])

        def layer_b(last):
            kv_ref[...] = jnp.zeros(kv_ref.shape, F32)
            z_ref[...] = jnp.zeros(z_ref.shape, F32)

            def keys(c, carry):
                rows = pl.ds(pl.multiple_of(c * TB, TB), TB)
                pk = _dot_nt(bt_ref[1], xb_ref[rows, :])
                v = _dot_nt(bt_ref[2], xb_ref[rows, :])
                for j in range(NG):
                    phi = features(pk[j * GR:(j + 1) * GR])
                    kv_ref[j] += _dot_nt(v[j * GR:(j + 1) * GR], phi.astype(BF16))
                    z_ref[j] += functools.reduce(
                        jnp.add, [phi[:, t:t + LANES] for t in range(0, TB, LANES)])
                return carry

            lax.fori_loop(0, NCH, keys, 0)

            shape = (GR, 2 * GR)
            same_head = (_iota(shape, 0) >= DB).astype(jnp.int32) == (_iota(shape, 1) & 1)
            for j in range(NG):
                kv_ref[j] = jnp.where(same_head, kv_ref[j], 0.0)
                z_ref[j] = jnp.broadcast_to(
                    jnp.sum(z_ref[j], axis=1, keepdims=True), z_ref.shape[1:])

            def queries(c, carry):
                half = TB // 2
                parts = [pl.ds(pl.multiple_of(c * TB + i * half, half), half) for i in range(2)]
                sublane = _iota((SUB, half), 0)
                even = (sublane & 1) == 0

                def attend(pq):
                    o = []
                    for j in range(NG):
                        phi = features(pq[j * GR:(j + 1) * GR])
                        z = jnp.concatenate([z_ref[j]] * (half // LANES), axis=1)
                        inv = _recip(over_features(jnp.add, phi * z) + 1e-6)
                        swapped = pltpu.roll(inv, 1, 0)
                        inv0, inv1 = jnp.where(even, inv, swapped), jnp.where(even, swapped, inv)
                        both = jnp.where(sublane < SUB // 2, inv0, inv1)
                        o.append(_dot(kv_ref[j], phi.astype(BF16)) * jnp.concatenate(
                            [inv0, inv0, both, inv1, inv1], axis=0))
                    return jnp.concatenate(o, axis=0).astype(BF16).T

                pqs = [_dot_nt(bt_ref[0], xb_ref[rows, :]) for rows in parts]
                outs = [attend(pq) for pq in pqs]
                for i, (rows, o) in enumerate(zip(parts, outs)):
                    x = x_ref[rows, :] + _dot(o, bwo_ref[...])
                    if last:
                        xb_ref[rows, :] = x.astype(BF16)
                        out_copy(2 * c + i).start()
                    else:
                        x_ref[rows, :] = x
                return carry

            lax.fori_loop(0, NCH, queries, 0)

        x_head_copy.wait()
        x_ref[seg_rows(0), :] = tokens(0, True)
        reset_memory(True)
        for g in range(G):
            wo_copy(g).wait()
        x_rest_copy.start()
        bw_copy.start()
        bwo_copy.start()
        layer_a(pre=True)
        normalise_output(NSEG - 1)
        fold_hedgehog_weights()
        layer_b(last=False)
        reset_memory(False)
        layer_a(pre=False)
        normalise_output(NSEG - 1)
        layer_b(last=True)
        for i in range(2 * NCH):
            out_copy(i).wait()

    scratch = [
        pltpu.VMEM((G, D // 2, 3 * PW), jnp.uint32),
        pltpu.VMEM((H * DH, D), BF16),
        pltpu.VMEM((NBUF, 3 * PW, D), BF16),
        pltpu.VMEM((NSEG, SEG, D), BF16),
        pltpu.VMEM((NSEG, PRE, D), BF16),
        pltpu.VMEM((NSEG * PRE, D), BF16),
        pltpu.VMEM((G, NSEG * PRE, 2 * PW), F32),
        pltpu.VMEM((S, D), BF16),
        pltpu.VMEM((S, D), F32),
        pltpu.VMEM((L, D), F32),
        pltpu.VMEM((D, 3 * D), BF16),
        pltpu.VMEM((FR, D), F32),
        pltpu.VMEM((3, D, D), BF16),
        pltpu.VMEM((D, D), BF16),
        pltpu.VMEM((NG, GR, 2 * GR), F32),
        pltpu.VMEM((NG, 2 * GR, LANES), F32),
        pltpu.SemaphoreType.DMA((NBUF, 3)),
        pltpu.SemaphoreType.DMA((G,)),
        pltpu.SemaphoreType.DMA((5,)),
        pltpu.SemaphoreType.DMA((2 * NCH,)),
    ]
    return kernel, scratch


@functools.partial(jax.jit, static_argnames=("A_seg_len",))
def pallas_interleave_layers__memory_aug_recurrent_mem_tr__linear_kernel_hedgehog__prompt_kernel(
    A_x: jax.Array,
    A_mem0: jax.Array,
    A_Wq: jax.Array,
    A_Wk: jax.Array,
    A_Wv: jax.Array,
    A_Wo: jax.Array,
    A_seg_len: int,
    B_x: jax.Array,
    B_wqkv: jax.Array,
    B_w_phi: jax.Array,
    B_wo: jax.Array,
):
    del B_x
    B, S, D = A_x.shape
    M = A_mem0.shape[1]
    _, H, DH = A_Wq.shape
    HB = B_w_phi.shape[0]
    assert B == 1

    kernel, scratch = _make_kernel(S, D, H, DH, M, A_seg_len, HB,
                                   HG=2, TB=512, NBUF=4, UNROLL=4)

    def head_major(w):
        return w.transpose(1, 2, 0).reshape(H * DH, D)

    hbm = pl.BlockSpec(memory_space=pltpu.HBM)
    vmem = pl.BlockSpec(memory_space=pltpu.VMEM)
    out = pl.pallas_call(
        kernel,
        out_shape=jax.ShapeDtypeStruct((S, D), A_x.dtype),
        in_specs=[hbm, vmem, hbm, hbm, hbm, hbm, hbm, vmem, hbm],
        out_specs=hbm,
        scratch_shapes=scratch,
        compiler_params=pltpu.CompilerParams(vmem_limit_bytes=110 * 1024 * 1024),
    )(
        A_x.reshape(S // A_seg_len, A_seg_len, D), A_mem0.reshape(M, D),
        head_major(A_Wq), head_major(A_Wk), head_major(A_Wv), A_Wo.reshape(H * DH, D),
        B_wqkv, B_w_phi.transpose(1, 2, 0), B_wo,
    )
    return out.reshape(B, S, D)
```

```python
import functools

import jax
import jax.numpy as jnp
from jax import lax
import jax.experimental.pallas as pl
import jax.experimental.pallas.tpu as pltpu

F32 = jnp.float32
BF16 = jnp.bfloat16
LANES = 128
SUB = 8
LOG2E = 1.4426950408889634


def _dot(a, b):
    return lax.dot_general(a, b, (((1,), (0,)), ((), ())), preferred_element_type=F32)


def _dot_nt(a, b):
    return lax.dot_general(a, b, (((1,), (1,)), ((), ())), preferred_element_type=F32)


def _layernorm_parts(x):
    inv_n = 1.0 / x.shape[-1]
    c = x - jnp.sum(x, axis=-1, keepdims=True) * inv_n
    var = jnp.sum(c * c, axis=-1, keepdims=True) * inv_n
    return c, lax.rsqrt(var + 1e-5)


def _layernorm(x):
    c, inv_std = _layernorm_parts(x)
    return c * inv_std


def _recip(x):
    r = pl.reciprocal(x, approx=True)
    return r * (2.0 - x * r)


def _iota(shape, dim):
    return lax.broadcasted_iota(jnp.int32, shape, dim)


def _div20(n):
    return (n * 3277) >> 16


def _make_kernel(S, D, H, DH, M, SEG, HB):
    L = M + SEG
    G = H // 2
    PW = 2 * DH
    NSEG = S // SEG
    PRE = SUB
    UNROLL = 4
    ATTEND_LAG, MIX_LAG, TAIL = 1, 3, 8
    NBUF = 4
    DB = D // HB
    NG = HB // 2
    GR = 2 * DB
    FR = 2 * GR
    TB = 512
    NCH = S // TB
    scale = DH ** -0.5
    assert PW == 3 * LANES and 2 * L <= LANES and M == SUB and SEG % (2 * SUB) == 0
    assert DB == 20 and D < 1024 and D % LANES == 0 and D % FR == 0 and S % TB == 0
    assert max(NBUF, TAIL) < G and NSEG % UNROLL == 0 and NSEG > 2 * UNROLL

    def kernel(x_hbm, mem_ref, wq_hbm, wk_hbm, wv_hbm, wo_hbm, bw_hbm, phi_ref, bwo_hbm,
               out_hbm,
               w_ref, wo_ref, stage_ref, xin_ref, xp_ref, hp_ref, pre_ref,
               xb_ref, x_ref, h_ref,
               bw_ref, phi_rows_ref, bt_ref, bwo_ref, kv_ref, z_ref,
               stage_sem, wo_sem, misc_sem, out_sem):

        def stage_copies(g):
            slot = g % NBUF
            rows = pl.ds(pl.multiple_of(g * PW, PW), PW)
            return [
                pltpu.make_async_copy(src.at[rows, :],
                                      stage_ref.at[slot, pl.ds(j * PW, PW), :],
                                      stage_sem.at[slot, j])
                for j, src in enumerate((wq_hbm, wk_hbm, wv_hbm))]

        xp_copy = pltpu.make_async_copy(
            x_hbm.at[:, pl.ds(SEG - PRE, PRE), :], xp_ref, misc_sem.at[0])
        bw_copy = pltpu.make_async_copy(bw_hbm, bw_ref, misc_sem.at[1])
        bwo_copy = pltpu.make_async_copy(bwo_hbm, bwo_ref, misc_sem.at[2])

        head, rest = pl.ds(0, 2 * UNROLL), pl.ds(2 * UNROLL, NSEG - 2 * UNROLL)
        x_head_copy = pltpu.make_async_copy(x_hbm.at[head], xin_ref.at[head], misc_sem.at[3])
        x_rest_copy = pltpu.make_async_copy(x_hbm.at[rest], xin_ref.at[rest], misc_sem.at[4])

        def wo_copy(g):
            rows = pl.ds(pl.multiple_of(g * PW, PW), PW)
            return pltpu.make_async_copy(wo_hbm.at[rows, :], wo_ref.at[rows, :], wo_sem.at[g])

        xp_copy.start()
        for cp in stage_copies(0):
            cp.start()

        eh = _iota((HB, D), 0) * DB
        ec = _iota((HB, D), 1)
        phi_flat = None
        for d in range(DB):
            t = _dot(phi_ref[d], jnp.where(ec == eh + d, 1.0, 0.0).astype(BF16))
            phi_flat = t if phi_flat is None else phi_flat + t
        nf = _iota((FR, DB), 0) >> 1
        sel = jnp.where(nf - DB * _div20(nf) == _iota((FR, DB), 1), 1.0, 0.0)
        phi_rows_ref[...] = _dot(sel.astype(BF16), phi_flat.astype(BF16))

        xp_copy.wait()
        hp_ref[...] = _layernorm(
            xp_ref[...].astype(F32).reshape(NSEG * PRE, D)).astype(BF16)
        for cp in stage_copies(1):
            cp.start()
        for cp in stage_copies(0):
            cp.wait()
        for g in range(2, NBUF):
            for cp in stage_copies(g):
                cp.start()

        def load_body(g, carry):
            slot = g % NBUF
            pre_ref[g] = _dot_nt(hp_ref[...], stage_ref[slot, PW:, :])
            w_ref[g] = pltpu.bitcast(stage_ref[slot].T, jnp.uint32)

            @pl.when(g + NBUF < G)
            def _():
                for cp in stage_copies(g + NBUF):
                    cp.start()
                wo_copy(g).start()

            @pl.when(g + NBUF == G)
            def _():
                x_head_copy.start()
                for k in range(G - NBUF, G):
                    wo_copy(k).start()

            @pl.when(g + 1 < G)
            def _():
                for cp in stage_copies(g + 1):
                    cp.wait()

            return carry

        lax.fori_loop(0, G, load_body, 0)

        def layer_a(pre):
            row = _iota((L, 2 * L), 0)
            col = _iota((L, 2 * L), 1)
            first = col < L
            visible = (row < M) | (row >= jnp.where(first, col, col - L))
            low = _iota((L, LANES), 1) < DH - LANES
            zero = jnp.zeros((L, LANES), F32)

            def block_diag(t):
                t0, t1, t2 = t[:, :LANES], t[:, LANES:2 * LANES], t[:, 2 * LANES:]
                top = jnp.concatenate([t0, jnp.where(low, t1, 0.0), zero], axis=1)
                bot = jnp.concatenate([zero, jnp.where(low, 0.0, t1), t2], axis=1)
                return jnp.concatenate([top, bot], axis=0).astype(BF16)

            def step(s, h):
                rows = seg_rows(s)
                chained = h is not None
                if not chained:
                    h = h_ref[...]
                h_kv = h[:L - PRE].astype(BF16) if pre else h
                st = {}
                acc = [None]

                def project(g):
                    def times(c0, c1):
                        return [
                            _dot(lhs[:, c0:c1], pltpu.bitcast(
                                w_ref[g, c0 // 2:c1 // 2, j * PW:(j + 1) * PW], BF16))
                            for lhs, j in ((h_kv, 1), (h, 0), (h_kv, 2))]

                    if g == 0 and chained:
                        parts = [times(c, c + LANES) for c in range(0, D, LANES)]
                        k, q, v = [functools.reduce(jnp.add, t) for t in zip(*parts)]
                    else:
                        k, q, v = times(0, D)
                    if pre:
                        done = pre_ref[g, pl.ds(pl.multiple_of(s * PRE, PRE), PRE), :]
                        k = jnp.concatenate([k, done[:, :PW]], axis=0)
                        v = jnp.concatenate([v, done[:, PW:]], axis=0)
                    st[g] = [q, block_diag(k), block_diag(v)]

                def attend(g, after):
                    fill = -1e9
                    if after is not None:
                        fill = jnp.concatenate(
                            [jnp.full((M, 1), fill, F32), jnp.minimum(after, fill)], axis=0)
                    sc = jnp.where(visible, _dot_nt(st[g][0], st[g][1]) * scale, fill)
                    m0 = jnp.max(jnp.where(first, sc, -jnp.inf), axis=1, keepdims=True)
                    m1 = jnp.max(jnp.where(first, -jnp.inf, sc), axis=1, keepdims=True)
                    e = jnp.exp(sc - jnp.where(first, m0, m1))
                    s0 = jnp.sum(jnp.where(first, e, 0.0), axis=1, keepdims=True)
                    s1 = jnp.sum(jnp.where(first, 0.0, e), axis=1, keepdims=True)
                    st[g][0] = e / jnp.where(first, s0, s1)

                def mix(g):
                    st[g] = _dot(st[g][0], st[g][2])

                def out_proj(g):
                    r = _dot(st[g], wo_ref[g * PW:(g + 1) * PW, :])
                    acc[0] = r if acc[0] is None else acc[0] + r

                for i in range(G + MIX_LAG):
                    if i < G:
                        project(i)
                    else:
                        for g in range((G - TAIL) * (i - G) // MIX_LAG,
                                       (G - TAIL) * (i - G + 1) // MIX_LAG):
                            out_proj(g)
                    after = None
                    if i == 3:
                        prev = seg_rows(jnp.maximum(s - 1, 0))
                        c, after = _layernorm_parts(x_ref[prev, :])
                        xb_ref[prev, :] = (c * after).astype(BF16)
                    if i == 6:
                        c, after = _layernorm_parts(tokens(jnp.minimum(s + 1, NSEG - 1), pre))
                        xn_next = c * after
                    if 0 <= i - ATTEND_LAG < G:
                        attend(i - ATTEND_LAG, after)
                    if 0 <= i - MIX_LAG < G:
                        mix(i - MIX_LAG)
                o = jnp.concatenate([st[g] for g in range(G - TAIL, G)], axis=1)
                y = jnp.concatenate([
                    acc[0][:, c:c + LANES]
                    + _dot(o, wo_ref[(G - TAIL) * PW:G * PW, c:c + LANES])
                    for c in range(0, D, LANES)], axis=1)
                x_ref[rows, :] = tokens(s, pre) + y[M:L]
                return jnp.concatenate([y[0:M], xn_next], axis=0)

            def steps(i, carry):
                if pre:
                    pl.when(i == 1)(x_rest_copy.wait)
                h = None
                for u in range(UNROLL):
                    h = step(i * UNROLL + u, h)
                h_ref[...] = h
                return carry

            lax.fori_loop(0, NSEG // UNROLL, steps, 0)

        def seg_rows(s):
            return pl.ds(s * SEG if isinstance(s, int) else pl.multiple_of(s * SEG, SEG), SEG)

        def normalise_output(s):
            xb_ref[seg_rows(s), :] = _layernorm(x_ref[seg_rows(s), :]).astype(BF16)

        def tokens(s, from_input):
            return xin_ref[s].astype(F32) if from_input else x_ref[seg_rows(s), :]

        def reset_memory(from_input):
            h_ref[0:M, :] = mem_ref[...].astype(F32)
            h_ref[M:L, :] = _layernorm(tokens(0, from_input))

        def fold_hedgehog_weights():
            bw_copy.wait()
            bwo_copy.wait()
            bt_ref[2] = bw_ref[:, 2 * D:3 * D].T
            for r0 in range(0, D, FR):
                c0 = r0 // LANES * LANES
                c1 = pl.cdiv(r0 + FR, LANES) * LANES
                n = _iota((FR, c1 - c0), 0) + r0
                c = _iota((FR, c1 - c0), 1) + c0
                head = 2 * _div20(n >> 1) + (n & 1)
                fold = jnp.where(_div20(c) == head, phi_rows_ref[:, c0:c1], 0.0).astype(BF16)
                for j in range(2):
                    bt_ref[j, r0:r0 + FR, :] = (LOG2E * _dot_nt(
                        fold, bw_ref[:, j * D + c0:j * D + c1])).astype(BF16)

        def over_features(op, p):
            r = p[0:SUB]
            for i in range(1, p.shape[0] // SUB):
                r = op(r, p[i * SUB:(i + 1) * SUB])
            for shift in (4, 2):
                r = op(r, pltpu.roll(r, shift, 0))
            return r

        def spread(r):
            return jnp.concatenate([r] * (GR // SUB), axis=0)

        def features(p):
            ep = jnp.exp2(p - spread(over_features(jnp.maximum, p)))
            en = jnp.exp2(spread(over_features(jnp.minimum, p)) - p)
            fp = ep * spread(_recip(over_features(jnp.add, ep)))
            fn = en * spread(_recip(over_features(jnp.add, en)))
            return jnp.concatenate([fp, fn], axis=0)

        def out_copy(i):
            rows = pl.ds(pl.multiple_of(i * (TB // 2), TB // 2), TB // 2)
            return pltpu.make_async_copy(xb_ref.at[rows, :], out_hbm.at[rows, :], out_sem.at[i])

        def layer_b(last):
            kv_ref[...] = jnp.zeros(kv_ref.shape, F32)
            z_ref[...] = jnp.zeros(z_ref.shape, F32)

            def keys(c, carry):
                rows = pl.ds(pl.multiple_of(c * TB, TB), TB)
                pk = _dot_nt(bt_ref[1], xb_ref[rows, :])
                v = _dot_nt(bt_ref[2], xb_ref[rows, :])
                for j in range(NG):
                    phi = features(pk[j * GR:(j + 1) * GR])
                    kv_ref[j] += _dot_nt(v[j * GR:(j + 1) * GR], phi.astype(BF16))
                    z_ref[j] += functools.reduce(
                        jnp.add, [phi[:, t:t + LANES] for t in range(0, TB, LANES)])
                return carry

            lax.fori_loop(0, NCH, keys, 0)

            def queries(c, carry):
                half = TB // 2
                parts = [pl.ds(pl.multiple_of(c * TB + i * half, half), half) for i in range(2)]
                sublane = _iota((SUB, half), 0)
                even = (sublane & 1) == 0
                same_head = ((_iota((GR, 2 * GR), 0) >= DB).astype(jnp.int32)
                             == (_iota((GR, 2 * GR), 1) & 1))
                kv = [jnp.where(same_head, kv_ref[j], 0.0) for j in range(NG)]
                z = [jnp.sum(z_ref[j], axis=1, keepdims=True) for j in range(NG)]

                def attend(pq):
                    o = []
                    for j in range(NG):
                        phi = features(pq[j * GR:(j + 1) * GR])
                        inv = _recip(over_features(jnp.add, phi * z[j]) + 1e-6)
                        swapped = pltpu.roll(inv, 1, 0)
                        inv0, inv1 = jnp.where(even, inv, swapped), jnp.where(even, swapped, inv)
                        both = jnp.where(sublane < SUB // 2, inv0, inv1)
                        o.append(_dot(kv[j], phi.astype(BF16)) * jnp.concatenate(
                            [inv0, inv0, both, inv1, inv1], axis=0))
                    return jnp.concatenate(o, axis=0).astype(BF16).T

                pqs = [_dot_nt(bt_ref[0], xb_ref[rows, :]) for rows in parts]
                outs = [attend(pq) for pq in pqs]
                for i, (rows, o) in enumerate(zip(parts, outs)):
                    x = x_ref[rows, :] + _dot(o, bwo_ref[...])
                    if last:
                        xb_ref[rows, :] = x.astype(BF16)
                        out_copy(2 * c + i).start()
                    else:
                        x_ref[rows, :] = x
                return carry

            lax.fori_loop(0, NCH, queries, 0)

        x_head_copy.wait()
        x_ref[seg_rows(0), :] = tokens(0, True)
        reset_memory(True)
        for g in range(G):
            wo_copy(g).wait()
        x_rest_copy.start()
        bw_copy.start()
        bwo_copy.start()
        layer_a(pre=True)
        normalise_output(NSEG - 1)
        fold_hedgehog_weights()
        layer_b(last=False)
        reset_memory(False)
        layer_a(pre=False)
        normalise_output(NSEG - 1)
        layer_b(last=True)
        for i in range(2 * NCH):
            out_copy(i).wait()

    scratch = [
        pltpu.VMEM((G, D // 2, 3 * PW), jnp.uint32),
        pltpu.VMEM((H * DH, D), BF16),
        pltpu.VMEM((NBUF, 3 * PW, D), BF16),
        pltpu.VMEM((NSEG, SEG, D), BF16),
        pltpu.VMEM((NSEG, PRE, D), BF16),
        pltpu.VMEM((NSEG * PRE, D), BF16),
        pltpu.VMEM((G, NSEG * PRE, 2 * PW), F32),
        pltpu.VMEM((S, D), BF16),
        pltpu.VMEM((S, D), F32),
        pltpu.VMEM((L, D), F32),
        pltpu.VMEM((D, 3 * D), BF16),
        pltpu.VMEM((FR, D), F32),
        pltpu.VMEM((3, D, D), BF16),
        pltpu.VMEM((D, D), BF16),
        pltpu.VMEM((NG, GR, 2 * GR), F32),
        pltpu.VMEM((NG, 2 * GR, LANES), F32),
        pltpu.SemaphoreType.DMA((NBUF, 3)),
        pltpu.SemaphoreType.DMA((G,)),
        pltpu.SemaphoreType.DMA((5,)),
        pltpu.SemaphoreType.DMA((2 * NCH,)),
    ]
    return kernel, scratch


@functools.partial(jax.jit, static_argnames=("A_seg_len",))
def pallas_interleave_layers__memory_aug_recurrent_mem_tr__linear_kernel_hedgehog__prompt_kernel(
    A_x: jax.Array,
    A_mem0: jax.Array,
    A_Wq: jax.Array,
    A_Wk: jax.Array,
    A_Wv: jax.Array,
    A_Wo: jax.Array,
    A_seg_len: int,
    B_x: jax.Array,
    B_wqkv: jax.Array,
    B_w_phi: jax.Array,
    B_wo: jax.Array,
):
    del B_x
    B, S, D = A_x.shape
    M = A_mem0.shape[1]
    _, H, DH = A_Wq.shape
    HB = B_w_phi.shape[0]
    assert B == 1

    kernel, scratch = _make_kernel(S, D, H, DH, M, A_seg_len, HB)

    def head_major(w):
        return w.transpose(1, 2, 0).reshape(H * DH, D)

    hbm = pl.BlockSpec(memory_space=pltpu.HBM)
    vmem = pl.BlockSpec(memory_space=pltpu.VMEM)
    out = pl.pallas_call(
        kernel,
        out_shape=jax.ShapeDtypeStruct((S, D), A_x.dtype),
        in_specs=[hbm, vmem, hbm, hbm, hbm, hbm, hbm, vmem, hbm],
        out_specs=hbm,
        scratch_shapes=scratch,
        compiler_params=pltpu.CompilerParams(vmem_limit_bytes=110 * 1024 * 1024),
    )(
        A_x.reshape(S // A_seg_len, A_seg_len, D), A_mem0.reshape(M, D),
        head_major(A_Wq), head_major(A_Wk), head_major(A_Wv), A_Wo.reshape(H * DH, D),
        B_wqkv, B_w_phi.transpose(1, 2, 0), B_wo,
    )
    return out.reshape(B, S, D)
```
